```python
import jax
import jax.numpy as jnp

def _softmax(x, axis=-1):
    return jax.nn.softmax(x, axis=axis)

def _gelu(x):
    return jax.nn.gelu(x, approximate=True)

def _silu(x):
    return jax.nn.silu(x)

def _sigmoid(x):
    return jax.nn.sigmoid(x)

def _layernorm(x, axis=-1, eps=1e-05):
    m = jnp.mean(x, axis=axis, keepdims=True)
    v = jnp.var(x, axis=axis, keepdims=True)
    return (x - m) / jnp.sqrt(v + eps)

def _scatter_add(tgt, idx, src, axis=0):
    return tgt.at[idx].add(src)

def _segment_sum(src, seg, n):
    return jax.ops.segment_sum(src, seg, n)

class _Rng:

    def __init__(self, key):
        self._k = key

    def _next(self):
        self._k, sub = jax.random.split(self._k)
        return sub

    def normal(self, shape):
        return jax.random.normal(self._next(), shape, dtype=jnp.bfloat16)

    def randint(self, lo, hi, shape):
        return jax.random.randint(self._next(), shape, lo, hi, dtype=jnp.int32)

    def uniform(self, shape, lo=0.0, hi=1.0):
        return jax.random.uniform(self._next(), shape, jnp.bfloat16, lo, hi)

    def permutation(self, n):
        return jax.random.permutation(self._next(), n)
kernel_name = 'concat_heads__memory_aug_recurrent_mem_tr__compressed_kv_cla__prompt'

def setup_inputs():
    _rng = _Rng(jax.random.key(int.from_bytes(__import__("os").urandom(4), "little")))
    _w = lambda a: (lambda t: t.astype(jnp.bfloat16) if jnp.issubdtype(t.dtype, jnp.floating) else t)(jnp.asarray(a))

    def _A_setup():
        B, S, Dm = (1, 2048, 448)
        H, Dh = (16, 256)
        M, seg = (8, 32)
        seg = min(seg, S)
        S = S // seg * seg
        return {'x': _w((lambda *s: _rng.normal(s) * 0.05)(B, S, Dm)), 'mem0': _w((lambda *s: _rng.normal(s) * 0.05)(B, M, Dm)), 'Wq': _w((lambda *s: _rng.normal(s) * 0.05)(Dm, H, Dh) * Dm ** (-0.5)), 'Wk': _w((lambda *s: _rng.normal(s) * 0.05)(Dm, H, Dh) * Dm ** (-0.5)), 'Wv': _w((lambda *s: _rng.normal(s) * 0.05)(Dm, H, Dh) * Dm ** (-0.5)), 'Wo': _w((lambda *s: _rng.normal(s) * 0.05)(H, Dh, Dm) * (H * Dh) ** (-0.5)), 'seg_len': seg}
    _A_in = _A_setup()

    def _B_setup():
        B, H, Sq, Sk, D, M = (1, 16, 2048, 2048, 256, 448)
        Dc = 4 * D
        return {'x': _w((lambda *s: _rng.normal(s) * 0.05)(B, Sq, M)), 'c_kv': _w((lambda *s: _rng.normal(s) * 0.05)(B, Sk, Dc)), 'w_q': _w((lambda *s: _rng.normal(s) * 0.05)(M, H, D) * M ** (-0.5)), 'w_uk': _w((lambda *s: _rng.normal(s) * 0.05)(Dc, H, D) * Dc ** (-0.5)), 'w_uv': _w((lambda *s: _rng.normal(s) * 0.05)(Dc, H, D) * Dc ** (-0.5)), 'w_o': _w((lambda *s: _rng.normal(s) * 0.05)(H, D, M) * (H * D) ** (-0.5))}
    _B_in = _B_setup()
    return {'A_x': _A_in['x'], 'A_mem0': _A_in['mem0'], 'A_Wq': _A_in['Wq'], 'A_Wk': _A_in['Wk'], 'A_Wv': _A_in['Wv'], 'A_Wo': _A_in['Wo'], 'A_seg_len': _A_in['seg_len'], 'B_x': _B_in['x'], 'B_c_kv': _B_in['c_kv'], 'B_w_q': _B_in['w_q'], 'B_w_uk': _B_in['w_uk'], 'B_w_uv': _B_in['w_uv'], 'B_w_o': _B_in['w_o']}

def reference(A_x, A_mem0, A_Wq, A_Wk, A_Wv, A_Wo, A_seg_len, B_x, B_c_kv, B_w_q, B_w_uk, B_w_uv, B_w_o):

    def _A_ref(x, mem0, Wq, Wk, Wv, Wo, seg_len):
        B, S, Dm = x.shape
        H, Dh = (Wq.shape[1], Wq.shape[2])
        M = mem0.shape[1]
        scale = Dh ** (-0.5)
        n_seg = S // seg_len
        L = M + seg_len
        idx = jnp.arange(L)
        mask = (idx[:, None] < M) | (idx[:, None] >= idx[None, :])
        mem = mem0
        outs = []
        for s in range(n_seg):
            xs = x[:, s * seg_len:(s + 1) * seg_len, :].copy()
            h = jnp.concatenate([mem, xs], axis=1)
            q = jnp.einsum('btd,dhe->bhte', h, Wq)
            k = jnp.einsum('btd,dhe->bhte', h, Wk)
            v = jnp.einsum('btd,dhe->bhte', h, Wv)
            scores = jnp.einsum('bhqe,bhke->bhqk', q, k) * scale
            scores = jnp.where(mask[None, None], scores, -1000000000.0)
            p = _softmax(scores, axis=-1)
            o = jnp.einsum('bhqk,bhke->bhqe', p, v)
            o = jnp.einsum('bhte,hed->btd', o, Wo)
            mem = o[:, :M, :].copy()
            outs.append(o[:, M:, :])
        return jnp.concatenate(outs, axis=1)

    def _B_ref(x, c_kv, w_q, w_uk, w_uv, w_o):
        B, Sq, M = (x.shape[0], x.shape[1], x.shape[2])
        Sk = c_kv.shape[1]
        H, D = (w_q.shape[1], w_q.shape[2])
        q = jnp.einsum('bqm,mhd->bhqd', x, w_q)
        k = jnp.einsum('bkc,chd->bhkd', c_kv, w_uk)
        v = jnp.einsum('bkc,chd->bhkd', c_kv, w_uv)
        scores = jnp.einsum('bhqd,bhkd->bhqk', q, k) * D ** (-0.5)
        off = Sk - Sq
        qi = jnp.arange(Sq)[:, None]
        kj = jnp.arange(Sk)[None, :]
        cmask = kj <= qi + off
        scores = jnp.where(cmask[None, None], scores, -1000000000.0)
        p = _softmax(scores, axis=-1)
        ctx = jnp.einsum('bhqk,bhkd->bhqd', p, v)
        return jnp.einsum('bhqd,hdm->bqm', ctx, w_o)
    a = _A_ref(A_x, A_mem0, A_Wq, A_Wk, A_Wv, A_Wo, A_seg_len)
    b = _B_ref(B_x, B_c_kv, B_w_q, B_w_uk, B_w_uv, B_w_o)
    return jnp.concatenate([a, b], axis=-1)
```

```python
import functools

import jax
import jax.numpy as jnp
from jax import lax
import jax.experimental.pallas as pl
import jax.experimental.pallas.tpu as pltpu

BF = jnp.bfloat16
F32 = jnp.float32

S = 2048
DM = 448
H = 16
DH = 256
MEM = 8
SEG = 32
DC = 1024
LOG2E = 1.4426950408889634
SCALE = DH ** -0.5 * LOG2E
NEG = -1000000000.0 * LOG2E
T = 128
G = 48
PAIR = 2 * DM
BQ = 512
BO = 256
NPAIR = S // (2 * SEG)
WCH = DC // NPAIR
NSLOT = 3
_TRIPS = dict(pairs=NPAIR, heads=H)


def _dot(a, b):
    return jnp.dot(a, b, preferred_element_type=F32)


def _dot_nt(a, b):
    return lax.dot_general(a, b, (((1,), (1,)), ((), ())), preferred_element_type=F32)


def _seg_reduce_bcast(x, lane, fill, combine, reduce_fn):
    tiles = [x[:, t * T:(t + 1) * T] for t in range(3)]
    outs = [None, None, None]
    for g in range(8):
        parts = []
        for t in range(3):
            lo = max(G * g - T * t, 0)
            hi = min(G * g + G - T * t, T)
            if lo < hi:
                parts.append((t, (lane >= lo) & (lane < hi)))
        acc = None
        for t, msk in parts:
            sel = jnp.where(msk, tiles[t], fill)
            acc = sel if acc is None else combine(acc, sel)
        red = reduce_fn(acc, axis=1, keepdims=True)
        for t, msk in parts:
            if outs[t] is None:
                outs[t] = jnp.broadcast_to(red, tiles[t].shape)
            else:
                outs[t] = jnp.where(msk, red, outs[t])
    return jnp.concatenate(outs, axis=1)


def _seg_softmax(s, keep, fill, lane):
    s = jnp.where(keep, s, fill)
    m = _seg_reduce_bcast(s, lane, -jnp.inf, jnp.maximum, jnp.max)
    p = jnp.exp2(s - m)
    l = _seg_reduce_bcast(p, lane, 0.0, jnp.add, jnp.sum)
    return (p * (1.0 / l)).astype(BF)


def _stacks(slabs):
    ev = [jnp.concatenate([r[:, 0:384], r[:, 768:896]], axis=1) for r in slabs]
    od = [jnp.concatenate([r[:, 384:768], r[:, 768:896]], axis=1) for r in slabs]
    return jnp.concatenate(ev, axis=0), jnp.concatenate(od, axis=0)


def _rec_attention(qrows, kslabs, vslabs_fn, keep, fill, lane):
    lo = lane < 64
    tail = qrows[:, 384:512]
    zero = jnp.zeros_like(tail)
    q_e = jnp.concatenate([qrows[:, 0:384], jnp.where(lo, tail, zero)], axis=1)
    q_o = jnp.concatenate([qrows[:, 0:384], jnp.where(lo, zero, tail)], axis=1)
    k_e, k_o = _stacks(kslabs)
    s_e = _dot_nt(q_e, k_e)
    s_o = _dot_nt(q_o, k_o)
    vslabs = vslabs_fn()
    p_e = _seg_softmax(s_e, keep, fill, lane)
    p_o = _seg_softmax(s_o, keep, fill, lane)
    v_e, v_o = _stacks(vslabs)
    o_main = _dot(jnp.concatenate([p_e, p_o], axis=1),
                  jnp.concatenate([v_e[:, 0:384], v_o[:, 0:384]], axis=0))
    t = jnp.where(lo, _dot(p_e, v_e[:, 384:512]), _dot(p_o, v_o[:, 384:512]))
    t = t + pltpu.roll(t, 64, 1)
    return jnp.concatenate([o_main, t], axis=1), vslabs


def _attn_block(q_s, k_s, v_s, i, tri):
    r0 = i * BQ
    nt = BQ // T
    n0 = r0 + T
    s_main = _dot_nt(q_s[r0:r0 + BQ, :], k_s[0:n0, :])
    s_t = [None] + [_dot_nt(q_s[r0 + t * T:r0 + BQ, :], k_s[r0 + t * T:r0 + (t + 1) * T, :])
                    for t in range(1, nt)]
    p_main = []
    p_t = [[] for _ in range(nt)]
    ls = []
    for u in range(nt):
        rows = slice(u * T, (u + 1) * T)
        pieces = []
        if u == 0:
            if r0 > 0:
                pieces.append(s_main[rows, :r0])
            pieces.append(jnp.where(tri, s_main[rows, r0:], NEG))
        else:
            pieces.append(s_main[rows, :])
            for t in range(1, u + 1):
                blk = s_t[t][(u - t) * T:(u - t + 1) * T, :]
                pieces.append(jnp.where(tri, blk, NEG) if t == u else blk)
        s = jnp.concatenate(pieces, axis=1) if len(pieces) > 1 else pieces[0]
        m = jnp.max(s, axis=1, keepdims=True)
        p = jnp.exp2(s - m)
        ls.append(jnp.sum(p, axis=1, keepdims=True))
        p = p.astype(BF)
        p_main.append(p[:, :n0])
        for t in range(1, u + 1):
            p_t[t].append(p[:, n0 + (t - 1) * T:n0 + t * T])
    o = _dot(jnp.concatenate(p_main, axis=0), v_s[0:n0, :])
    os_ = [o[u * T:(u + 1) * T] for u in range(nt)]
    for t in range(1, nt):
        ot = _dot(jnp.concatenate(p_t[t], axis=0), v_s[r0 + t * T:r0 + (t + 1) * T, :])
        for u in range(t, nt):
            os_[u] = os_[u] + ot[(u - t) * T:(u - t + 1) * T]
    return jnp.concatenate([os_[u] * (1.0 / ls[u]) for u in range(nt)], axis=0)


def _kernel(xa_hbm, mem0_hbm, wq_hbm, wk_hbm, wv_hbm, wo_hbm,
            xb_hbm, c_hbm, bwq_hbm, bwk_hbm, bwv_hbm, bwo_hbm,
            out_hbm,
            xbt_s, c_s, bwq_raw, bwq_s, bwkv_s, bwo_s, stage_k, stage_v, out_s,
            sems, stage_sems, out_sems):

    def stage_copies(chunk, slot):
        rows = pl.ds(chunk * WCH, WCH)
        return (pltpu.make_async_copy(bwk_hbm.at[rows], stage_k.at[slot], stage_sems.at[0, slot]),
                pltpu.make_async_copy(bwv_hbm.at[rows], stage_v.at[slot], stage_sems.at[1, slot]))

    cp_xb = pltpu.make_async_copy(xb_hbm, xbt_s, sems.at[6])
    cp_c = pltpu.make_async_copy(c_hbm, c_s, sems.at[7])
    cp_bwq = pltpu.make_async_copy(bwq_hbm, bwq_raw, sems.at[8])
    cp_bwo = pltpu.make_async_copy(bwo_hbm, bwo_s, sems.at[9])

    def phase_a(xa_s, mem0_s, wq_raw, wk_raw, wv_raw, wo_s, wq_t, wk_t, wv_t,
                wck_s, wcv_s, xad_s):
        cp_wq = pltpu.make_async_copy(wq_hbm, wq_raw, sems.at[0])
        cp_wk = pltpu.make_async_copy(wk_hbm, wk_raw, sems.at[1])
        cp_wv = pltpu.make_async_copy(wv_hbm, wv_raw, sems.at[2])
        cp_wo = pltpu.make_async_copy(wo_hbm, wo_s, sems.at[3])
        cp_xa = pltpu.make_async_copy(xa_hbm, xa_s, sems.at[4])
        cp_m0 = pltpu.make_async_copy(mem0_hbm, mem0_s, sems.at[5])
        for cp in (cp_wq, cp_wk, cp_wv, cp_wo, cp_xa, cp_m0, cp_bwq):
            cp.start()
        for s0 in range(NSLOT - 1):
            for cp in stage_copies(s0, s0):
                cp.start()
        for cp in (cp_xb, cp_c, cp_bwo):
            cp.start()

        def relayout(src, dst):
            def body(t, carry):
                rows = pl.ds(pl.multiple_of(t * 64, 64), 64)
                dst[:, rows, :] = jnp.swapaxes(src[rows], 0, 1)
                return carry
            lax.fori_loop(0, DM // 64, body, 0)

        def pack_pair(e, o):
            return jnp.concatenate(
                [e[:, 0:384], o[:, 0:384], e[:, 384:448], o[:, 384:448]], axis=1).astype(BF)

        cp_wq.wait()
        relayout(wq_raw, wq_t)
        cp_wk.wait()
        relayout(wk_raw, wk_t)

        def ck_body(j, carry):
            e = _dot_nt(wk_t[2 * j], wq_t[2 * j]) * SCALE
            o = _dot_nt(wk_t[2 * j + 1], wq_t[2 * j + 1]) * SCALE
            wck_s[j] = pack_pair(e, o)
            return carry
        lax.fori_loop(0, H // 2, ck_body, 0)

        cp_wv.wait()
        relayout(wv_raw, wv_t)
        cp_wo.wait()

        def cv_body(j, carry):
            e = _dot_nt(wv_t[2 * j], wo_s[2 * j])
            o = _dot_nt(wv_t[2 * j + 1], wo_s[2 * j + 1])
            wcv_s[j] = pack_pair(e, o)
            return carry
        lax.fori_loop(0, H // 2, cv_body, 0)

        cp_xa.wait()
        cp_m0.wait()
        cp_bwq.wait()

        def dup_body(t, carry):
            rows = pl.ds(pl.multiple_of(t * 256, 256), 256)
            x = xa_s[:, rows]
            xad_s[rows, :] = jnp.concatenate([x, x[384:448, :]], axis=0).T
            return carry
        lax.fori_loop(0, S // 256, dup_body, 0)

        m0 = mem0_s[...].astype(F32)
        mem_init = jnp.concatenate([m0, m0[:, 384:448]], axis=1)

        def pair_body(i, mem):
            slot = lax.rem(i, NSLOT)
            for cp in stage_copies(i, slot):
                cp.wait()

            @pl.when(i + NSLOT - 1 < _TRIPS['pairs'])
            def _():
                nxt = i + NSLOT - 1
                for cp in stage_copies(nxt, lax.rem(nxt, NSLOT)):
                    cp.start()

            wrows = pl.ds(pl.multiple_of(i * WCH, WCH), WCH)
            bwkv_s[:, wrows, 0:DH] = jnp.swapaxes(stage_k[slot], 0, 1)
            bwkv_s[:, wrows, DH:2 * DH] = jnp.swapaxes(stage_v[slot], 0, 1)
            qrows = pl.ds(pl.multiple_of(jnp.minimum(i, DM // 16 - 1) * 16, 16), 16)
            bwq_s[:, qrows, :] = jnp.swapaxes(bwq_raw[qrows], 0, 1)

            lane = lax.broadcasted_iota(jnp.int32, (G, T), 1)
            r = lax.broadcasted_iota(jnp.int32, (G, 3 * T), 0)
            col = lax.broadcasted_iota(jnp.int32, (G, 3 * T), 1)
            kk = col - G * ((col * 1366) >> 16)
            valid_e = (kk < 32) | (kk >= 40)
            keep_e = valid_e & ((r >= 32) | (kk >= 40) | (kk <= r))
            fill_e = jnp.where(valid_e, NEG, -jnp.inf)
            valid_o = kk < 40
            kpos = jnp.where(kk < 24, kk + 8, kk - 32)
            qpos = jnp.where(r < 24, r + 8, r - 32)
            q_any = ((r >= 24) & (r < 32)) | (r >= 40)
            keep_o = valid_o & (q_any | ((kk >= 24) & (kk < 32)) | (kpos <= qpos))
            fill_o = jnp.where(valid_o, NEG, -jnp.inf)

            base = pl.multiple_of(i * 64, 64)
            xs = xad_s[pl.ds(base, 64), :]
            xs32 = xs[32:64, :].astype(F32)

            l1 = jnp.concatenate(
                [xs[0:32, :], jnp.concatenate([xs32[0:8, :], mem], axis=0).astype(BF)], axis=0)
            l1p = l1[:, 0:DM]
            k1 = [_dot(l1p, wck_s[j]).astype(BF) for j in range(H // 2)]
            o1, v1 = _rec_attention(
                l1, k1, lambda: [_dot(l1p, wcv_s[j]).astype(BF) for j in range(H // 2)],
                keep_e, fill_e, lane)

            l2 = jnp.concatenate([xs32[8:32, :], o1[40:48, :]], axis=0).astype(BF)
            l2p = l2[:, 0:DM]
            k2 = [jnp.concatenate([_dot(l2p, wck_s[j]).astype(BF), k1[j][32:48, :]], axis=0)
                  for j in range(H // 2)]
            o2, _ = _rec_attention(
                jnp.concatenate([l2, l1[32:48, :]], axis=0), k2,
                lambda: [jnp.concatenate([_dot(l2p, wcv_s[j]).astype(BF), v1[j][32:48, :]], axis=0)
                         for j in range(H // 2)],
                keep_o, fill_o, lane)

            res = jnp.concatenate([o1[0:32, :], o2[32:40, :], o2[0:24, :]], axis=0)
            out_s[pl.ds(base, 64), 0:512] = res.astype(BF)
            return o2[24:32, :]

        lax.fori_loop(0, _TRIPS['pairs'], pair_body, mem_init)

    pl.run_scoped(
        phase_a,
        pltpu.VMEM((DM, S), BF), pltpu.VMEM((MEM, DM), BF),
        pltpu.VMEM((DM, H, DH), BF), pltpu.VMEM((DM, H, DH), BF), pltpu.VMEM((DM, H, DH), BF),
        pltpu.VMEM((H, DM, DH), BF),
        pltpu.VMEM((H, DM, DH), BF), pltpu.VMEM((H, DM, DH), BF), pltpu.VMEM((H, DM, DH), BF),
        pltpu.VMEM((H // 2, DM, PAIR), BF), pltpu.VMEM((H // 2, DM, PAIR), BF),
        pltpu.VMEM((S, 512), BF),
    )

    def phase_b(q_s, k_s, v_s, o_s, xb_s):
        cp_xb.wait()
        cp_c.wait()
        cp_bwo.wait()

        def xt_body(t, carry):
            rows = pl.ds(pl.multiple_of(t * 256, 256), 256)
            x = xbt_s[:, rows]
            xb_s[rows, :] = jnp.concatenate([x, x[384:448, :]], axis=0).T
            return carry
        lax.fori_loop(0, S // 256, xt_body, 0)

        def head(h, carry):
            q_s[...] = (_dot(xb_s[:, 0:DM], bwq_s[h]) * SCALE).astype(BF)
            kv = _dot(c_s[...], bwkv_s[h])
            k_s[...] = kv[:, 0:DH].astype(BF)
            v_s[...] = kv[:, DH:2 * DH].astype(BF)
            row = lax.broadcasted_iota(jnp.int32, (T, T), 0)
            col = lax.broadcasted_iota(jnp.int32, (T, T), 1)
            tri = row >= col
            for i in reversed(range(S // BQ)):
                o_s[h, i * BQ:(i + 1) * BQ, :] = _attn_block(q_s, k_s, v_s, i, tri).astype(BF)
            return carry
        lax.fori_loop(0, _TRIPS['heads'], head, 0)

        def out_copy(t):
            rows = pl.ds(pl.multiple_of(t * BO, BO), BO)
            return pltpu.make_async_copy(out_s.at[rows], out_hbm.at[rows], out_sems.at[t])

        def oproj(t, carry):
            rows = pl.ds(pl.multiple_of(t * BO, BO), BO)
            ctx = jnp.concatenate([o_s[h, rows, :] for h in range(H)], axis=1)
            wo = jnp.concatenate([bwo_s[h] for h in range(H)], axis=1)
            out_s[rows, DM:2 * DM] = _dot_nt(ctx, wo).astype(BF)
            out_copy(t).start()
            return carry
        lax.fori_loop(0, S // BO, oproj, 0)
        for t in range(S // BO):
            out_copy(t).wait()

    pl.run_scoped(
        phase_b,
        pltpu.VMEM((S, DH), BF), pltpu.VMEM((S, DH), BF), pltpu.VMEM((S, DH), BF),
        pltpu.VMEM((H, S, DH), BF), pltpu.VMEM((S, 512), BF),
    )


@functools.partial(jax.jit, static_argnames=("A_seg_len",))
def pallas_concat_heads__memory_aug_recurrent_mem_tr__compressed_kv_cla__prompt_kernel(
    A_x: jax.Array,
    A_mem0: jax.Array,
    A_Wq: jax.Array,
    A_Wk: jax.Array,
    A_Wv: jax.Array,
    A_Wo: jax.Array,
    A_seg_len,
    B_x: jax.Array,
    B_c_kv: jax.Array,
    B_w_q: jax.Array,
    B_w_uk: jax.Array,
    B_w_uv: jax.Array,
    B_w_o: jax.Array,
):
    assert int(A_seg_len) == SEG
    assert A_x.shape == (1, S, DM) and A_mem0.shape == (1, MEM, DM)
    assert A_Wq.shape == (DM, H, DH) and A_Wo.shape == (H, DH, DM)
    assert B_x.shape == (1, S, DM) and B_c_kv.shape == (1, S, DC)
    assert B_w_uk.shape == (DC, H, DH) and B_w_o.shape == (H, DH, DM)

    any_spec = pl.BlockSpec(memory_space=pl.ANY)
    out = pl.pallas_call(
        _kernel,
        out_shape=jax.ShapeDtypeStruct((S, 2 * DM), BF),
        in_specs=[any_spec] * 12,
        out_specs=any_spec,
        scratch_shapes=[
            pltpu.VMEM((DM, S), BF),
            pltpu.VMEM((S, DC), BF),
            pltpu.VMEM((DM, H, DH), BF),
            pltpu.VMEM((H, DM, DH), BF),
            pltpu.VMEM((H, DC, 2 * DH), BF),
            pltpu.VMEM((H, DM, DH), BF),
            pltpu.VMEM((NSLOT, WCH, H, DH), BF),
            pltpu.VMEM((NSLOT, WCH, H, DH), BF),
            pltpu.VMEM((S, 2 * DM), BF),
            pltpu.SemaphoreType.DMA((10,)),
            pltpu.SemaphoreType.DMA((2, NSLOT)),
            pltpu.SemaphoreType.DMA((S // BO,)),
        ],
        compiler_params=pltpu.CompilerParams(vmem_limit_bytes=120 * 1024 * 1024),
    )(jnp.swapaxes(A_x, 1, 2).reshape(DM, S), A_mem0.reshape(MEM, DM), A_Wq, A_Wk, A_Wv,
      jnp.swapaxes(A_Wo, 1, 2),
      jnp.swapaxes(B_x, 1, 2).reshape(DM, S), B_c_kv.reshape(S, DC), B_w_q, B_w_uk, B_w_uv,
      jnp.swapaxes(B_w_o, 1, 2))
    return out.reshape(1, S, 2 * DM)
```

```python
import functools
import os

import jax
import jax.numpy as jnp
from jax import lax
import jax.experimental.pallas as pl
import jax.experimental.pallas.tpu as pltpu

BF = jnp.bfloat16
F32 = jnp.float32

S = 2048
DM = 448
H = 16
DH = 256
MEM = 8
SEG = 32
DC = 1024
LOG2E = 1.4426950408889634
SCALE = DH ** -0.5 * LOG2E
NEG = -1000000000.0 * LOG2E
T = 128
G = 48
PAIR = 2 * DM
BQ = 512
KC = 256
BO = 256
NPAIR = S // (2 * SEG)
WCH = DC // NPAIR
NSLOT = 3
RCH = 64
OPT = int(os.environ.get('OPT', '1'))
BO = int(os.environ.get('BO', '512'))
TIE_ROW = int(os.environ.get('TIE', '0'))
_TRIPS = dict(pairs=NPAIR, heads=H)


def _dot(a, b):
    return jnp.dot(a, b, preferred_element_type=F32)


def _dot_nt(a, b):
    return lax.dot_general(a, b, (((1,), (1,)), ((), ())), preferred_element_type=F32)


def _seg_reduce_bcast(x, lane, fill, combine, reduce_fn):
    tiles = [x[:, t * T:(t + 1) * T] for t in range(3)]
    outs = [None, None, None]
    for g in range(8):
        parts = []
        for t in range(3):
            lo = max(G * g - T * t, 0)
            hi = min(G * g + G - T * t, T)
            if lo < hi:
                parts.append((t, (lane >= lo) & (lane < hi)))
        acc = None
        for t, msk in parts:
            sel = jnp.where(msk, tiles[t], fill)
            acc = sel if acc is None else combine(acc, sel)
        red = reduce_fn(acc, axis=1, keepdims=True)
        for t, msk in parts:
            if outs[t] is None:
                outs[t] = jnp.broadcast_to(red, tiles[t].shape)
            else:
                outs[t] = jnp.where(msk, red, outs[t])
    return jnp.concatenate(outs, axis=1)


def _seg_softmax(s, keep, fill, lane):
    s = jnp.where(keep, s, fill)
    m = _seg_reduce_bcast(s, lane, -jnp.inf, jnp.maximum, jnp.max)
    p = jnp.exp2(s - m)
    l = _seg_reduce_bcast(p, lane, 0.0, jnp.add, jnp.sum)
    return (p * (1.0 / l)).astype(BF)


def _stacks(slabs):
    ev = [jnp.concatenate([r[:, 0:384], r[:, 768:896]], axis=1) for r in slabs]
    od = [jnp.concatenate([r[:, 384:768], r[:, 768:896]], axis=1) for r in slabs]
    return jnp.concatenate(ev, axis=0), jnp.concatenate(od, axis=0)


def _rec_attention(qrows, kslabs, vslab_fn, filler, keep, fill, lane):
    lo = lane < 64
    tail = qrows[:, 384:512]
    zero = jnp.zeros_like(tail)
    q_e = jnp.concatenate([qrows[:, 0:384], jnp.where(lo, tail, zero)], axis=1)
    q_o = jnp.concatenate([qrows[:, 0:384], jnp.where(lo, zero, tail)], axis=1)
    k_e, k_o = _stacks(kslabs)
    vslabs = [vslab_fn(0)]
    s_e = _dot_nt(q_e, k_e)
    s_o = _dot_nt(q_o, k_o)
    vslabs += [vslab_fn(j) for j in range(1, H // 2)]
    filler()
    p_e = _seg_softmax(s_e, keep, fill, lane)
    p_o = _seg_softmax(s_o, keep, fill, lane)
    v_e, v_o = _stacks(vslabs)
    o_main = _dot(jnp.concatenate([p_e, p_o], axis=1),
                  jnp.concatenate([v_e[:, 0:384], v_o[:, 0:384]], axis=0))
    t = jnp.where(lo, _dot(p_e, v_e[:, 384:512]), _dot(p_o, v_o[:, 384:512]))
    t = t + pltpu.roll(t, 64, 1)
    return jnp.concatenate([o_main, t], axis=1), vslabs


def _b_qk(q, k_s, r0):
    n0 = r0 + T
    s_main = _dot_nt(q, k_s[0:n0, :])
    s_t = [None] + [_dot_nt(q[t * T:, :], k_s[r0 + t * T:r0 + (t + 1) * T, :])
                    for t in range(1, BQ // T)]
    return s_main, s_t


def _b_softmax(scores, r0, tri):
    s_main, s_t = scores
    nt = BQ // T
    n0 = r0 + T
    p_main = []
    p_t = [[] for _ in range(nt)]
    ls = []
    for u in range(nt):
        rows = slice(u * T, (u + 1) * T)
        pieces = []
        if u == 0:
            if r0 > 0:
                pieces.append(s_main[rows, :r0])
            pieces.append(jnp.where(tri, s_main[rows, r0:], NEG))
        else:
            pieces.append(s_main[rows, :])
            for t in range(1, u + 1):
                blk = s_t[t][(u - t) * T:(u - t + 1) * T, :]
                pieces.append(jnp.where(tri, blk, NEG) if t == u else blk)
        s = jnp.concatenate(pieces, axis=1) if len(pieces) > 1 else pieces[0]
        m = jnp.max(s, axis=1, keepdims=True)
        p = jnp.exp2(s - m)
        ls.append(jnp.sum(p, axis=1, keepdims=True))
        p = p.astype(BF)
        p_main.append(p[:, :n0])
        for t in range(1, u + 1):
            p_t[t].append(p[:, n0 + (t - 1) * T:n0 + t * T])
    return p_main, p_t, ls


def _b_pv(probs, v_s, r0):
    p_main, p_t, ls = probs
    nt = BQ // T
    n0 = r0 + T
    pm = jnp.concatenate(p_main, axis=0)
    o = None
    for c0 in range(0, n0, KC):
        c1 = min(c0 + KC, n0)
        oc = _dot(pm[:, c0:c1], v_s[c0:c1, :])
        o = oc if o is None else o + oc
    os_ = [o[u * T:(u + 1) * T] for u in range(nt)]
    for t in range(1, nt):
        ot = _dot(jnp.concatenate(p_t[t], axis=0), v_s[r0 + t * T:r0 + (t + 1) * T, :])
        for u in range(t, nt):
            os_[u] = os_[u] + ot[(u - t) * T:(u - t + 1) * T]
    return jnp.concatenate([os_[u] * (1.0 / ls[u]) for u in range(nt)], axis=0)


def _kernel(xa_hbm, mem0_hbm, wq_hbm, wk_hbm, wv_hbm, wo_hbm,
            xb_hbm, c_hbm, bwq_hbm, bwk_hbm, bwv_hbm, bwo_hbm,
            out_hbm,
            c_s, q_s, bwkv_s, bwo_s, stage_k, stage_v, out_s,
            sems, w_sems, stage_sems, out_sems):

    def stage_copies(chunk, slot):
        rows = pl.ds(chunk * WCH, WCH)
        return (pltpu.make_async_copy(bwk_hbm.at[rows], stage_k.at[slot], stage_sems.at[0, slot]),
                pltpu.make_async_copy(bwv_hbm.at[rows], stage_v.at[slot], stage_sems.at[1, slot]))

    cp_c = pltpu.make_async_copy(c_hbm, c_s, sems.at[3])
    cp_bwo = pltpu.make_async_copy(bwo_hbm, bwo_s, sems.at[4])

    def phase_a(xat_s, xbt_s, mem0_s, wq_raw, wk_raw, wv_raw, bwq_raw, wo_s,
                wq_t, wk_t, wv_t, bwq_s, wck_s, wcv_s, xad_s, xb_s):
        def row_chunk(k, hbm, raw, t):
            rows = pl.ds(t * RCH, RCH)
            return pltpu.make_async_copy(hbm.at[rows], raw.at[rows], w_sems.at[k, t])

        def wo_chunk(j):
            heads = pl.ds(2 * j, 2)
            return pltpu.make_async_copy(wo_hbm.at[heads], wo_s.at[heads], w_sems.at[4, j])

        cp_xa = pltpu.make_async_copy(xa_hbm, xat_s, sems.at[0])
        cp_m0 = pltpu.make_async_copy(mem0_hbm, mem0_s, sems.at[1])
        cp_xb = pltpu.make_async_copy(xb_hbm, xbt_s, sems.at[2])
        for t in range(DM // RCH):
            row_chunk(0, wv_hbm, wv_raw, t).start()
        for j in range(H // 2):
            wo_chunk(j).start()
        for t in range(DM // RCH):
            row_chunk(1, wq_hbm, wq_raw, t).start()
        for t in range(DM // RCH):
            row_chunk(2, wk_hbm, wk_raw, t).start()
        cp_xa.start()
        cp_m0.start()
        for t in range(DM // RCH):
            row_chunk(3, bwq_hbm, bwq_raw, t).start()
        cp_xb.start()
        for s0 in range(NSLOT - 1):
            for cp in stage_copies(s0, s0):
                cp.start()
        for cp in (cp_c, cp_bwo):
            cp.start()

        def relayout(k, hbm, raw, store):
            def body(t, carry):
                row_chunk(k, hbm, raw, t).wait()
                rows = pl.ds(pl.multiple_of(t * RCH, RCH), RCH)
                store(rows, jnp.swapaxes(raw[rows], 0, 1))
                return carry
            lax.fori_loop(0, DM // RCH, body, 0)

        def store_to(dst):
            def store(rows, val):
                dst[:, rows, :] = val
            return store

        def store_bwq(rows, val):
            bwq_s[:, 0, rows, :] = val[:, :, 0:T]
            bwq_s[:, 1, rows, :] = val[:, :, T:2 * T]

        def pack_pair(e, o):
            w = jnp.concatenate(
                [e[:, 0:384], o[:, 0:384], e[:, 384:448], o[:, 384:448]], axis=1).astype(BF)
            return pltpu.bitcast(w, jnp.uint32)

        def transpose_x(src, dst):
            def body(t, carry):
                rows = pl.ds(pl.multiple_of(t * 256, 256), 256)
                x = src[:, rows]
                dst[rows, :] = jnp.concatenate([x, x[384:448, :]], axis=0).T
                return carry
            lax.fori_loop(0, S // 256, body, 0)

        relayout(0, wv_hbm, wv_raw, store_to(wv_t))

        def cv_body(j, carry):
            wo_chunk(j).wait()
            e = _dot_nt(wv_t[2 * j], wo_s[2 * j])
            o = _dot_nt(wv_t[2 * j + 1], wo_s[2 * j + 1])
            wcv_s[j] = pack_pair(e, o)
            return carry
        lax.fori_loop(0, H // 2, cv_body, 0)

        relayout(1, wq_hbm, wq_raw, store_to(wq_t))
        relayout(2, wk_hbm, wk_raw, store_to(wk_t))

        def ck_body(j, carry):
            e = _dot_nt(wk_t[2 * j], wq_t[2 * j]) * SCALE
            o = _dot_nt(wk_t[2 * j + 1], wq_t[2 * j + 1]) * SCALE
            wck_s[j] = pack_pair(e, o)
            return carry
        lax.fori_loop(0, H // 2, ck_body, 0)

        cp_xa.wait()
        cp_m0.wait()
        transpose_x(xat_s, xad_s)
        relayout(3, bwq_hbm, bwq_raw, store_bwq)
        cp_xb.wait()
        transpose_x(xbt_s, xb_s)

        m0 = mem0_s[...].astype(F32)
        mem_init = jnp.concatenate([m0, m0[:, 384:448]], axis=1)

        def pair_body(i, mem):
            slot = lax.rem(i, NSLOT)
            for cp in stage_copies(i, slot):
                cp.wait()

            @pl.when(i + NSLOT - 1 < _TRIPS['pairs'])
            def _():
                nxt = i + NSLOT - 1
                for cp in stage_copies(nxt, lax.rem(nxt, NSLOT)):
                    cp.start()

            zero_bits = jnp.full((8, T), i >> 20, jnp.int32).astype(jnp.uint32)

            def relayout_piece(n):
                part, src = n % 2, (stage_k, stage_v)[n // 2]
                wrows = pl.ds(pl.multiple_of(i * WCH + part * 16, 16), 16)
                c0 = (n // 2) * DH
                val = jnp.swapaxes(src[slot, part * 16:(part + 1) * 16], 0, 1)
                bwkv_s[:, wrows, c0:c0 + DH] = val
                bits = pltpu.bitcast(val.reshape(16 * 16, DH), jnp.uint32)
                acc = None
                for a in range(16):
                    for b in range(2):
                        x = bits[a * 8:(a + 1) * 8, b * T:(b + 1) * T]
                        acc = x if acc is None else (acc | x)
                return acc & zero_bits

            hq = i // 2
            half = lax.rem(i, 2)

            def q_fill(n):
                def run():
                    r0 = n * (S // 4)
                    rows = slice(r0, r0 + S // 4)
                    q = (_dot(xb_s[rows, 0:DM], bwq_s[hq, half]) * SCALE).astype(BF)
                    a = TIE_ROW
                    mid = pltpu.bitcast(
                        pltpu.bitcast(q[a:a + 16, :], jnp.uint32) | relayout_piece(n), BF)
                    parts = ([q[0:a, :]] if a else []) + [mid] + (
                        [q[a + 16:, :]] if a + 16 < S // 4 else [])
                    q_s[hq, half, rows, :] = jnp.concatenate(parts, axis=0)
                return run

            lane = lax.broadcasted_iota(jnp.int32, (G, T), 1)
            r = lax.broadcasted_iota(jnp.int32, (G, 3 * T), 0)
            col = lax.broadcasted_iota(jnp.int32, (G, 3 * T), 1)
            kk = col - G * ((col * 1366) >> 16)
            valid_e = (kk < 32) | (kk >= 40)
            keep_e = valid_e & ((r >= 32) | (kk >= 40) | (kk <= r))
            fill_e = jnp.where(valid_e, NEG, -jnp.inf)
            valid_o = kk < 40
            kpos = jnp.where(kk < 24, kk + 8, kk - 32)
            qpos = jnp.where(r < 24, r + 8, r - 32)
            q_any = ((r >= 24) & (r < 32)) | (r >= 40)
            keep_o = valid_o & (q_any | ((kk >= 24) & (kk < 32)) | (kpos <= qpos))
            fill_o = jnp.where(valid_o, NEG, -jnp.inf)

            base = pl.multiple_of(i * 64, 64)
            xs = xad_s[pl.ds(base, 64), :]
            xs32 = xs[32:64, :].astype(F32)

            l1 = jnp.concatenate(
                [xs[0:32, :], jnp.concatenate([xs32[0:8, :], mem], axis=0).astype(BF)], axis=0)
            l1p = l1[:, 0:DM]
            k1 = [_dot(l1p, pltpu.bitcast(wck_s[j], BF)).astype(BF) for j in range(H // 2)]
            o1, v1 = _rec_attention(
                l1, k1, lambda j: _dot(l1p, pltpu.bitcast(wcv_s[j], BF)).astype(BF), q_fill(0),
                keep_e, fill_e, lane)
            q_fill(1)()

            l2 = jnp.concatenate([xs32[8:32, :], o1[40:48, :]], axis=0).astype(BF)
            l2p = l2[:, 0:DM]
            k2 = [jnp.concatenate([_dot(l2p, pltpu.bitcast(wck_s[j], BF)).astype(BF), k1[j][32:48, :]], axis=0)
                  for j in range(H // 2)]
            o2, _ = _rec_attention(
                jnp.concatenate([l2, l1[32:48, :]], axis=0), k2,
                lambda j: jnp.concatenate(
                    [_dot(l2p, pltpu.bitcast(wcv_s[j], BF)).astype(BF), v1[j][32:48, :]], axis=0),
                q_fill(2), keep_o, fill_o, lane)
            q_fill(3)()

            res = jnp.concatenate([o1[0:32, :], o2[32:40, :], o2[0:24, :]], axis=0)
            out_s[pl.ds(base, 64), 0:512] = res.astype(BF)
            return o2[24:32, :]

        lax.fori_loop(0, _TRIPS['pairs'], pair_body, mem_init)

    pl.run_scoped(
        phase_a,
        pltpu.VMEM((DM, S), BF), pltpu.VMEM((DM, S), BF), pltpu.VMEM((MEM, DM), BF),
        pltpu.VMEM((DM, H, DH), BF), pltpu.VMEM((DM, H, DH), BF), pltpu.VMEM((DM, H, DH), BF),
        pltpu.VMEM((DM, H, DH), BF),
        pltpu.VMEM((H, DM, DH), BF),
        pltpu.VMEM((H, DM, DH), BF), pltpu.VMEM((H, DM, DH), BF), pltpu.VMEM((H, DM, DH), BF),
        pltpu.VMEM((H, 2, DM, T), BF),
        pltpu.VMEM((H // 2, DM // 2, PAIR), jnp.uint32),
        pltpu.VMEM((H // 2, DM // 2, PAIR), jnp.uint32),
        pltpu.VMEM((S, 512), BF), pltpu.VMEM((S, 512), BF),
    )

    def phase_b(k_s, v_s, o_s):
        cp_c.wait()
        cp_bwo.wait()

        def head(h, carry):
            k_s[...] = _dot(c_s[...], bwkv_s[h, :, 0:DH]).astype(BF)
            v_s[...] = _dot(c_s[...], bwkv_s[h, :, DH:2 * DH]).astype(BF)
            row = lax.broadcasted_iota(jnp.int32, (T, T), 0)
            col = lax.broadcasted_iota(jnp.int32, (T, T), 1)
            tri = row >= col

            def qk(r0):
                q = jnp.concatenate(
                    [q_s[h, 0, r0:r0 + BQ, :], q_s[h, 1, r0:r0 + BQ, :]], axis=1)
                return _b_qk(q, k_s, r0)

            starts = list(reversed(range(0, S, BQ)))
            scores = qk(starts[0])
            for n, r0 in enumerate(starts):
                nxt = qk(starts[n + 1]) if n + 1 < len(starts) else None
                probs = _b_softmax(scores, r0, tri)
                o_s[h, r0:r0 + BQ, :] = _b_pv(probs, v_s, r0).astype(BF)
                scores = nxt
            return carry
        lax.fori_loop(0, _TRIPS['heads'], head, 0)

        def out_copy(t):
            rows = pl.ds(pl.multiple_of(t * BO, BO), BO)
            return pltpu.make_async_copy(out_s.at[rows], out_hbm.at[rows], out_sems.at[t])

        def oproj(t, carry):
            rows = pl.ds(pl.multiple_of(t * BO, BO), BO)
            ctx = jnp.concatenate([o_s[h, rows, :] for h in range(H)], axis=1)
            wo = jnp.concatenate([bwo_s[h] for h in range(H)], axis=1)
            if OPT == 0:
                out_s[rows, DM:2 * DM] = _dot_nt(ctx, wo).astype(BF)
            else:
                bt = _dot_nt(wo, ctx)
                if OPT == 1:
                    bt = jnp.concatenate([jnp.zeros((64, BO), F32), bt], axis=0)
                    b = bt.T.astype(BF)
                else:
                    bt = jnp.concatenate([jnp.zeros((64, BO), BF), bt.astype(BF)], axis=0)
                    b = bt.T
                lo = lax.broadcasted_iota(jnp.int32, (BO, T), 1) < 64
                out_s[rows, 384:512] = jnp.where(lo, out_s[rows, 384:512], b[:, 0:T])
                out_s[rows, 512:896] = b[:, T:]
            out_copy(t).start()
            return carry
        lax.fori_loop(0, S // BO, oproj, 0)
        for t in range(S // BO):
            out_copy(t).wait()

    pl.run_scoped(
        phase_b,
        pltpu.VMEM((S, DH), BF), pltpu.VMEM((S, DH), BF),
        pltpu.VMEM((H, S, DH), BF),
    )


@functools.partial(jax.jit, static_argnames=("A_seg_len",))
def pallas_concat_heads__memory_aug_recurrent_mem_tr__compressed_kv_cla__prompt_kernel(
    A_x: jax.Array,
    A_mem0: jax.Array,
    A_Wq: jax.Array,
    A_Wk: jax.Array,
    A_Wv: jax.Array,
    A_Wo: jax.Array,
    A_seg_len,
    B_x: jax.Array,
    B_c_kv: jax.Array,
    B_w_q: jax.Array,
    B_w_uk: jax.Array,
    B_w_uv: jax.Array,
    B_w_o: jax.Array,
):
    assert int(A_seg_len) == SEG
    assert A_x.shape == (1, S, DM) and A_mem0.shape == (1, MEM, DM)
    assert A_Wq.shape == (DM, H, DH) and A_Wo.shape == (H, DH, DM)
    assert B_x.shape == (1, S, DM) and B_c_kv.shape == (1, S, DC)
    assert B_w_uk.shape == (DC, H, DH) and B_w_o.shape == (H, DH, DM)

    any_spec = pl.BlockSpec(memory_space=pl.ANY)
    out = pl.pallas_call(
        _kernel,
        out_shape=jax.ShapeDtypeStruct((S, 2 * DM), BF),
        in_specs=[any_spec] * 12,
        out_specs=any_spec,
        scratch_shapes=[
            pltpu.VMEM((S, DC), BF),
            pltpu.VMEM((H, 2, S, T), BF),
            pltpu.VMEM((H, DC, 2 * DH), BF),
            pltpu.VMEM((H, DM, DH), BF),
            pltpu.VMEM((NSLOT, WCH, H, DH), BF),
            pltpu.VMEM((NSLOT, WCH, H, DH), BF),
            pltpu.VMEM((S, 2 * DM), BF),
            pltpu.SemaphoreType.DMA((5,)),
            pltpu.SemaphoreType.DMA((5, 8)),
            pltpu.SemaphoreType.DMA((2, NSLOT)),
            pltpu.SemaphoreType.DMA((S // BO,)),
        ],
        compiler_params=pltpu.CompilerParams(vmem_limit_bytes=120 * 1024 * 1024),
    )(jnp.swapaxes(A_x, 1, 2).reshape(DM, S), A_mem0.reshape(MEM, DM), A_Wq, A_Wk, A_Wv,
      jnp.swapaxes(A_Wo, 1, 2),
      jnp.swapaxes(B_x, 1, 2).reshape(DM, S), B_c_kv.reshape(S, DC), B_w_q, B_w_uk, B_w_uv,
      jnp.swapaxes(B_w_o, 1, 2))
    return out.reshape(1, S, 2 * DM)
```

```python
import functools
import os

import jax
import jax.numpy as jnp
from jax import lax
import jax.experimental.pallas as pl
import jax.experimental.pallas.tpu as pltpu

BF = jnp.bfloat16
F32 = jnp.float32

S = 2048
DM = 448
H = 16
DH = 256
MEM = 8
SEG = 32
DC = 1024
LOG2E = 1.4426950408889634
SCALE = DH ** -0.5 * LOG2E
NEG = -1000000000.0 * LOG2E
T = 128
G = 48
PAIR = 2 * DM
BQ = 512
KC = 256
BO = 256
NPAIR = S // (2 * SEG)
WCH = DC // NPAIR
NSLOT = 3
FR = int(os.environ.get('FR', '256'))
UCD = int(os.environ.get('UCD', '1'))
UCH = int(os.environ.get('UCH', '1'))
UOP = int(os.environ.get('UOP', '1'))
RCH = 64
OPT = int(os.environ.get('OPT', '1'))
BO = int(os.environ.get('BO', '512'))
TIE_ROW = int(os.environ.get('TIE', '480'))
_TRIPS = dict(pairs=NPAIR, heads=H)


def _dot(a, b):
    return jnp.dot(a, b, preferred_element_type=F32)


def _dot_nt(a, b):
    return lax.dot_general(a, b, (((1,), (1,)), ((), ())), preferred_element_type=F32)


def _seg_reduce_bcast(x, lane, fill, combine, reduce_fn):
    tiles = [x[:, t * T:(t + 1) * T] for t in range(3)]
    outs = [None, None, None]
    for g in range(8):
        parts = []
        for t in range(3):
            lo = max(G * g - T * t, 0)
            hi = min(G * g + G - T * t, T)
            if lo < hi:
                parts.append((t, (lane >= lo) & (lane < hi)))
        acc = None
        for t, msk in parts:
            sel = jnp.where(msk, tiles[t], fill)
            acc = sel if acc is None else combine(acc, sel)
        red = reduce_fn(acc, axis=1, keepdims=True)
        for t, msk in parts:
            if outs[t] is None:
                outs[t] = jnp.broadcast_to(red, tiles[t].shape)
            else:
                outs[t] = jnp.where(msk, red, outs[t])
    return jnp.concatenate(outs, axis=1)


def _seg_softmax(s, keep, fill, lane):
    s = jnp.where(keep, s, fill)
    m = _seg_reduce_bcast(s, lane, -jnp.inf, jnp.maximum, jnp.max)
    p = jnp.exp2(s - m)
    l = _seg_reduce_bcast(p, lane, 0.0, jnp.add, jnp.sum)
    return (p * (1.0 / l)).astype(BF)


def _stacks(slabs):
    ev = [jnp.concatenate([r[:, 0:384], r[:, 768:896]], axis=1) for r in slabs]
    od = [jnp.concatenate([r[:, 384:768], r[:, 768:896]], axis=1) for r in slabs]
    return jnp.concatenate(ev, axis=0), jnp.concatenate(od, axis=0)


def _rec_attention(qrows, kslabs, vslab_fn, filler, keep, fill, lane):
    lo = lane < 64
    tail = qrows[:, 384:512]
    zero = jnp.zeros_like(tail)
    q_e = jnp.concatenate([qrows[:, 0:384], jnp.where(lo, tail, zero)], axis=1)
    q_o = jnp.concatenate([qrows[:, 0:384], jnp.where(lo, zero, tail)], axis=1)
    k_e, k_o = _stacks(kslabs)
    vslabs = [vslab_fn(0)]
    s_e = _dot_nt(q_e, k_e)
    s_o = _dot_nt(q_o, k_o)
    vslabs += [vslab_fn(j) for j in range(1, H // 2)]
    filler()
    p_e = _seg_softmax(s_e, keep, fill, lane)
    p_o = _seg_softmax(s_o, keep, fill, lane)
    v_e, v_o = _stacks(vslabs)
    o_main = _dot(jnp.concatenate([p_e, p_o], axis=1),
                  jnp.concatenate([v_e[:, 0:384], v_o[:, 0:384]], axis=0))
    t = jnp.where(lo, _dot(p_e, v_e[:, 384:512]), _dot(p_o, v_o[:, 384:512]))
    t = t + pltpu.roll(t, 64, 1)
    return jnp.concatenate([o_main, t], axis=1), vslabs


def _b_qk(q, k_s, r0):
    n0 = r0 + T
    s_main = _dot_nt(q, k_s[0:n0, :])
    s_t = [None] + [_dot_nt(q[t * T:, :], k_s[r0 + t * T:r0 + (t + 1) * T, :])
                    for t in range(1, BQ // T)]
    return s_main, s_t


def _b_softmax(scores, r0, tri):
    s_main, s_t = scores
    nt = BQ // T
    n0 = r0 + T
    p_main = []
    p_t = [[] for _ in range(nt)]
    ls = []
    for u in range(nt):
        rows = slice(u * T, (u + 1) * T)
        pieces = []
        if u == 0:
            if r0 > 0:
                pieces.append(s_main[rows, :r0])
            pieces.append(jnp.where(tri, s_main[rows, r0:], NEG))
        else:
            pieces.append(s_main[rows, :])
            for t in range(1, u + 1):
                blk = s_t[t][(u - t) * T:(u - t + 1) * T, :]
                pieces.append(jnp.where(tri, blk, NEG) if t == u else blk)
        s = jnp.concatenate(pieces, axis=1) if len(pieces) > 1 else pieces[0]
        m = jnp.max(s, axis=1, keepdims=True)
        p = jnp.exp2(s - m)
        ls.append(jnp.sum(p, axis=1, keepdims=True))
        p = p.astype(BF)
        p_main.append(p[:, :n0])
        for t in range(1, u + 1):
            p_t[t].append(p[:, n0 + (t - 1) * T:n0 + t * T])
    return p_main, p_t, ls


def _b_pv(probs, v_s, r0):
    p_main, p_t, ls = probs
    nt = BQ // T
    n0 = r0 + T
    pm = jnp.concatenate(p_main, axis=0)
    o = None
    for c0 in range(0, n0, KC):
        c1 = min(c0 + KC, n0)
        oc = _dot(pm[:, c0:c1], v_s[c0:c1, :])
        o = oc if o is None else o + oc
    os_ = [o[u * T:(u + 1) * T] for u in range(nt)]
    for t in range(1, nt):
        ot = _dot(jnp.concatenate(p_t[t], axis=0), v_s[r0 + t * T:r0 + (t + 1) * T, :])
        for u in range(t, nt):
            os_[u] = os_[u] + ot[(u - t) * T:(u - t + 1) * T]
    return jnp.concatenate([os_[u] * (1.0 / ls[u]) for u in range(nt)], axis=0)


def _kernel(xa_hbm, mem0_hbm, wq_hbm, wk_hbm, wv_hbm, wo_hbm,
            xb_hbm, c_hbm, bwq_hbm, bwk_hbm, bwv_hbm, bwo_hbm,
            out_hbm,
            c_s, hm_s, bwo_s, stage_k, stage_v, out_s,
            sems, w_sems, stage_sems, out_sems):

    def stage_copies(chunk, slot):
        rows = pl.ds(chunk * WCH, WCH)
        return (pltpu.make_async_copy(bwk_hbm.at[rows], stage_k.at[slot], stage_sems.at[0, slot]),
                pltpu.make_async_copy(bwv_hbm.at[rows], stage_v.at[slot], stage_sems.at[1, slot]))

    cp_c = pltpu.make_async_copy(c_hbm, c_s, sems.at[3])
    cp_bwo = pltpu.make_async_copy(bwo_hbm, bwo_s, sems.at[4])

    def phase_a(xat_s, xbt_s, mem0_s, wq_raw, wk_raw, wv_raw, bwq_raw, wo_s,
                wq_t, wk_t, wv_t, bwq_s, wck_s, wcv_s, xad_s, xb_s):
        def row_chunk(k, hbm, raw, t):
            rows = pl.ds(t * RCH, RCH)
            return pltpu.make_async_copy(hbm.at[rows], raw.at[rows], w_sems.at[k, t])

        def wo_chunk(j):
            heads = pl.ds(2 * j, 2)
            return pltpu.make_async_copy(wo_hbm.at[heads], wo_s.at[heads], w_sems.at[4, j])

        cp_xa = pltpu.make_async_copy(xa_hbm, xat_s, sems.at[0])
        cp_m0 = pltpu.make_async_copy(mem0_hbm, mem0_s, sems.at[1])
        cp_xb = pltpu.make_async_copy(xb_hbm, xbt_s, sems.at[2])
        for t in range(DM // RCH):
            row_chunk(0, wv_hbm, wv_raw, t).start()
        for j in range(H // 2):
            wo_chunk(j).start()
        for t in range(DM // RCH):
            row_chunk(1, wq_hbm, wq_raw, t).start()
        for t in range(DM // RCH):
            row_chunk(2, wk_hbm, wk_raw, t).start()
        cp_xa.start()
        cp_m0.start()
        for t in range(DM // RCH):
            row_chunk(3, bwq_hbm, bwq_raw, t).start()
        cp_xb.start()
        for s0 in range(NSLOT - 1):
            for cp in stage_copies(s0, s0):
                cp.start()
        for cp in (cp_c, cp_bwo):
            cp.start()

        def relayout(k, hbm, raw, store):
            def body(t, carry):
                row_chunk(k, hbm, raw, t).wait()
                rows = pl.ds(pl.multiple_of(t * RCH, RCH), RCH)
                store(rows, jnp.swapaxes(raw[rows], 0, 1))
                return carry
            lax.fori_loop(0, DM // RCH, body, 0)

        def store_to(dst):
            def store(rows, val):
                dst[:, rows, :] = val
            return store

        def pack_pair(e, o):
            w = jnp.concatenate(
                [e[:, 0:384], o[:, 0:384], e[:, 384:448], o[:, 384:448]], axis=1).astype(BF)
            return pltpu.bitcast(w, jnp.uint32)

        def transpose_x(src, dst):
            def body(t, carry):
                rows = pl.ds(pl.multiple_of(t * 256, 256), 256)
                x = src[:, rows]
                dst[rows, :] = jnp.concatenate([x, x[384:448, :]], axis=0).T
                return carry
            lax.fori_loop(0, S // 256, body, 0)

        relayout(0, wv_hbm, wv_raw, store_to(wv_t))

        def cv_body(j, carry):
            wo_chunk(j).wait()
            e = _dot_nt(wv_t[2 * j], wo_s[2 * j])
            o = _dot_nt(wv_t[2 * j + 1], wo_s[2 * j + 1])
            wcv_s[j] = pack_pair(e, o)
            return carry
        lax.fori_loop(0, H // 2, cv_body, 0, unroll=UCD)

        relayout(1, wq_hbm, wq_raw, store_to(wq_t))
        relayout(2, wk_hbm, wk_raw, store_to(wk_t))

        def ck_body(j, carry):
            e = _dot_nt(wk_t[2 * j], wq_t[2 * j]) * SCALE
            o = _dot_nt(wk_t[2 * j + 1], wq_t[2 * j + 1]) * SCALE
            wck_s[j] = pack_pair(e, o)
            return carry
        lax.fori_loop(0, H // 2, ck_body, 0, unroll=UCD)

        cp_xa.wait()
        cp_m0.wait()
        transpose_x(xat_s, xad_s)
        relayout(3, bwq_hbm, bwq_raw, store_to(bwq_s))
        cp_xb.wait()
        transpose_x(xbt_s, xb_s)

        m0 = mem0_s[...].astype(F32)
        mem_init = jnp.concatenate([m0, m0[:, 384:448]], axis=1)

        def pair_body(i, mem):
            slot = lax.rem(i, NSLOT)
            for cp in stage_copies(i, slot):
                cp.wait()

            @pl.when(i + NSLOT - 1 < _TRIPS['pairs'])
            def _():
                nxt = i + NSLOT - 1
                for cp in stage_copies(nxt, lax.rem(nxt, NSLOT)):
                    cp.start()

            def relayout_piece(n):
                part, src = n % 2, (stage_k, stage_v)[n // 2]
                wrows = pl.ds(pl.multiple_of(S + (n // 2) * DC + i * WCH + part * 16, 16), 16)
                hm_s[:, wrows, :] = jnp.swapaxes(src[slot, part * 16:(part + 1) * 16], 0, 1)

            per_head = S // (4 * FR)
            hq = i // per_head + (H - NPAIR // per_head)
            qbase = lax.rem(i, per_head) * (4 * FR)

            def q_fill(n):
                def run():
                    rows = pl.ds(pl.multiple_of(qbase + n * FR, FR), FR)
                    relayout_piece(n)
                    hm_s[hq, rows, :] = (_dot(xb_s[rows, 0:DM], bwq_s[hq]) * SCALE).astype(BF)
                return run

            lane = lax.broadcasted_iota(jnp.int32, (G, T), 1)
            r = lax.broadcasted_iota(jnp.int32, (G, 3 * T), 0)
            col = lax.broadcasted_iota(jnp.int32, (G, 3 * T), 1)
            kk = col - G * ((col * 1366) >> 16)
            valid_e = (kk < 32) | (kk >= 40)
            keep_e = valid_e & ((r >= 32) | (kk >= 40) | (kk <= r))
            fill_e = jnp.where(valid_e, NEG, -jnp.inf)
            valid_o = kk < 40
            kpos = jnp.where(kk < 24, kk + 8, kk - 32)
            qpos = jnp.where(r < 24, r + 8, r - 32)
            q_any = ((r >= 24) & (r < 32)) | (r >= 40)
            keep_o = valid_o & (q_any | ((kk >= 24) & (kk < 32)) | (kpos <= qpos))
            fill_o = jnp.where(valid_o, NEG, -jnp.inf)

            base = pl.multiple_of(i * 64, 64)
            xs = xad_s[pl.ds(base, 64), :]
            xs32 = xs[32:64, :].astype(F32)

            l1 = jnp.concatenate(
                [xs[0:32, :], jnp.concatenate([xs32[0:8, :], mem], axis=0).astype(BF)], axis=0)
            l1p = l1[:, 0:DM]
            k1 = [_dot(l1p, pltpu.bitcast(wck_s[j], BF)).astype(BF) for j in range(H // 2)]
            o1, v1 = _rec_attention(
                l1, k1, lambda j: _dot(l1p, pltpu.bitcast(wcv_s[j], BF)).astype(BF), q_fill(0),
                keep_e, fill_e, lane)
            q_fill(1)()

            l2 = jnp.concatenate([xs32[8:32, :], o1[40:48, :]], axis=0).astype(BF)
            l2p = l2[:, 0:DM]
            k2 = [jnp.concatenate([_dot(l2p, pltpu.bitcast(wck_s[j], BF)).astype(BF), k1[j][32:48, :]], axis=0)
                  for j in range(H // 2)]
            o2, _ = _rec_attention(
                jnp.concatenate([l2, l1[32:48, :]], axis=0), k2,
                lambda j: jnp.concatenate(
                    [_dot(l2p, pltpu.bitcast(wcv_s[j], BF)).astype(BF), v1[j][32:48, :]], axis=0),
                q_fill(2), keep_o, fill_o, lane)
            q_fill(3)()

            res = jnp.concatenate([o1[0:32, :], o2[32:40, :], o2[0:24, :]], axis=0)
            out_s[pl.ds(base, 64), 0:512] = res.astype(BF)
            return o2[24:32, :]

        lax.fori_loop(0, _TRIPS['pairs'], pair_body, mem_init, unroll=UCH)

    pl.run_scoped(
        phase_a,
        pltpu.VMEM((DM, S), BF), pltpu.VMEM((DM, S), BF), pltpu.VMEM((MEM, DM), BF),
        pltpu.VMEM((DM, H, DH), BF), pltpu.VMEM((DM, H, DH), BF), pltpu.VMEM((DM, H, DH), BF),
        pltpu.VMEM((DM, H, DH), BF),
        pltpu.VMEM((H, DM, DH), BF),
        pltpu.VMEM((H, DM, DH), BF), pltpu.VMEM((H, DM, DH), BF), pltpu.VMEM((H, DM, DH), BF),
        pltpu.VMEM((H, DM, DH), BF),
        pltpu.VMEM((H // 2, DM // 2, PAIR), jnp.uint32),
        pltpu.VMEM((H // 2, DM // 2, PAIR), jnp.uint32),
        pltpu.VMEM((S, 512), BF), pltpu.VMEM((S, 512), BF),
    )

    def phase_b(k_s, v_s, o_s):
        cp_c.wait()
        cp_bwo.wait()

        def head(h, carry):
            k_s[...] = _dot(c_s[...], hm_s[h, S:S + DC, :]).astype(BF)
            v_s[...] = _dot(c_s[...], hm_s[h, S + DC:S + 2 * DC, :]).astype(BF)
            row = lax.broadcasted_iota(jnp.int32, (T, T), 0)
            col = lax.broadcasted_iota(jnp.int32, (T, T), 1)
            tri = row >= col

            def qk(r0):
                q = hm_s[h, r0:r0 + BQ, :]
                return _b_qk(q, k_s, r0)

            starts = list(reversed(range(0, S, BQ)))
            scores = qk(starts[0])
            for n, r0 in enumerate(starts):
                nxt = qk(starts[n + 1]) if n + 1 < len(starts) else None
                probs = _b_softmax(scores, r0, tri)
                o_s[h, r0:r0 + BQ, :] = _b_pv(probs, v_s, r0).astype(BF)
                scores = nxt
            return carry
        lax.fori_loop(0, _TRIPS['heads'], head, 0)

        def out_copy(t):
            rows = pl.ds(pl.multiple_of(t * BO, BO), BO)
            return pltpu.make_async_copy(out_s.at[rows], out_hbm.at[rows], out_sems.at[t])

        def oproj(t, carry):
            rows = pl.ds(pl.multiple_of(t * BO, BO), BO)
            ctx = jnp.concatenate([o_s[h, rows, :] for h in range(H)], axis=1)
            wo = jnp.concatenate([bwo_s[h] for h in range(H)], axis=1)
            if OPT == 0:
                out_s[rows, DM:2 * DM] = _dot_nt(ctx, wo).astype(BF)
            else:
                bt = _dot_nt(wo, ctx)
                if OPT == 1:
                    bt = jnp.concatenate([jnp.zeros((64, BO), F32), bt], axis=0)
                    b = bt.T.astype(BF)
                else:
                    bt = jnp.concatenate([jnp.zeros((64, BO), BF), bt.astype(BF)], axis=0)
                    b = bt.T
                lo = lax.broadcasted_iota(jnp.int32, (BO, T), 1) < 64
                out_s[rows, 384:512] = jnp.where(lo, out_s[rows, 384:512], b[:, 0:T])
                out_s[rows, 512:896] = b[:, T:]
            out_copy(t).start()
            return carry
        lax.fori_loop(0, S // BO, oproj, 0, unroll=UOP)
        for t in range(S // BO):
            out_copy(t).wait()

    pl.run_scoped(
        phase_b,
        pltpu.VMEM((S, DH), BF), pltpu.VMEM((S, DH), BF),
        pltpu.VMEM((H, S, DH), BF),
    )


@functools.partial(jax.jit, static_argnames=("A_seg_len",))
def pallas_concat_heads__memory_aug_recurrent_mem_tr__compressed_kv_cla__prompt_kernel(
    A_x: jax.Array,
    A_mem0: jax.Array,
    A_Wq: jax.Array,
    A_Wk: jax.Array,
    A_Wv: jax.Array,
    A_Wo: jax.Array,
    A_seg_len,
    B_x: jax.Array,
    B_c_kv: jax.Array,
    B_w_q: jax.Array,
    B_w_uk: jax.Array,
    B_w_uv: jax.Array,
    B_w_o: jax.Array,
):
    assert int(A_seg_len) == SEG
    assert A_x.shape == (1, S, DM) and A_mem0.shape == (1, MEM, DM)
    assert A_Wq.shape == (DM, H, DH) and A_Wo.shape == (H, DH, DM)
    assert B_x.shape == (1, S, DM) and B_c_kv.shape == (1, S, DC)
    assert B_w_uk.shape == (DC, H, DH) and B_w_o.shape == (H, DH, DM)

    any_spec = pl.BlockSpec(memory_space=pl.ANY)
    out = pl.pallas_call(
        _kernel,
        out_shape=jax.ShapeDtypeStruct((S, 2 * DM), BF),
        in_specs=[any_spec] * 12,
        out_specs=any_spec,
        scratch_shapes=[
            pltpu.VMEM((S, DC), BF),
            pltpu.VMEM((H, S + 2 * DC, DH), BF),
            pltpu.VMEM((H, DM, DH), BF),
            pltpu.VMEM((NSLOT, WCH, H, DH), BF),
            pltpu.VMEM((NSLOT, WCH, H, DH), BF),
            pltpu.VMEM((S, 2 * DM), BF),
            pltpu.SemaphoreType.DMA((5,)),
            pltpu.SemaphoreType.DMA((5, 8)),
            pltpu.SemaphoreType.DMA((2, NSLOT)),
            pltpu.SemaphoreType.DMA((S // BO,)),
        ],
        compiler_params=pltpu.CompilerParams(vmem_limit_bytes=120 * 1024 * 1024),
    )(jnp.swapaxes(A_x, 1, 2).reshape(DM, S), A_mem0.reshape(MEM, DM), A_Wq, A_Wk, A_Wv,
      jnp.swapaxes(A_Wo, 1, 2),
      jnp.swapaxes(B_x, 1, 2).reshape(DM, S), B_c_kv.reshape(S, DC), B_w_q, B_w_uk, B_w_uv,
      jnp.swapaxes(B_w_o, 1, 2))
    return out.reshape(1, S, 2 * DM)
```

```python
import functools
import os

import jax
import jax.numpy as jnp
from jax import lax
import jax.experimental.pallas as pl
import jax.experimental.pallas.tpu as pltpu

BF = jnp.bfloat16
F32 = jnp.float32

S = 2048
DM = 448
H = 16
DH = 256
MEM = 8
SEG = 32
DC = 1024
LOG2E = 1.4426950408889634
SCALE = DH ** -0.5 * LOG2E
NEG = -1000000000.0 * LOG2E
T = 128
L = MEM + SEG
G = 48
PAIR = 2 * DM
BQ = 512
KC = 256
BO = 256
NPAIR = S // (2 * SEG)
WCH = DC // NPAIR
NSLOT = 3
FR = int(os.environ.get('FR', '256'))
UCD = int(os.environ.get('UCD', '1'))
UCH = int(os.environ.get('UCH', '1'))
UOP = int(os.environ.get('UOP', '1'))
RCH = 64
OPT = int(os.environ.get('OPT', '1'))
BO = int(os.environ.get('BO', '512'))
TIE_ROW = int(os.environ.get('TIE', '480'))
_TRIPS = dict(pairs=NPAIR, heads=H)


def _dot(a, b):
    return jnp.dot(a, b, preferred_element_type=F32)


def _dot_nt(a, b):
    return lax.dot_general(a, b, (((1,), (1,)), ((), ())), preferred_element_type=F32)


def _seg_reduce_bcast(x, lane, fill, combine, reduce_fn):
    nt = H * L // T
    tiles = [x[:, t * T:(t + 1) * T] for t in range(nt)]
    outs = [None] * nt
    for g in range(H):
        parts = []
        for t in range(nt):
            lo = max(L * g - T * t, 0)
            hi = min(L * g + L - T * t, T)
            if lo < hi:
                parts.append((t, (lane >= lo) & (lane < hi)))
        acc = None
        for t, msk in parts:
            sel = jnp.where(msk, tiles[t], fill)
            acc = sel if acc is None else combine(acc, sel)
        red = reduce_fn(acc, axis=1, keepdims=True)
        for t, msk in parts:
            if outs[t] is None:
                outs[t] = jnp.broadcast_to(red, tiles[t].shape)
            else:
                outs[t] = jnp.where(msk, red, outs[t])
    return jnp.concatenate(outs, axis=1)


def _seg_softmax(s, keep, lane):
    s = jnp.where(keep, s, NEG)
    m = _seg_reduce_bcast(s, lane, -jnp.inf, jnp.maximum, jnp.max)
    p = jnp.exp2(s - m)
    l = _seg_reduce_bcast(p, lane, 0.0, jnp.add, jnp.sum)
    return (p * (1.0 / l)).astype(BF)


def _stack(slabs):
    lo = lax.broadcasted_iota(jnp.int32, (L, T), 1) < 64
    blocks = []
    for r in slabs:
        tail = r[:, 768:896]
        blocks.append(jnp.concatenate([r[:, 0:384], jnp.where(lo, tail, 0.0)], axis=1))
        blocks.append(jnp.concatenate([r[:, 384:768], jnp.where(lo, 0.0, tail)], axis=1))
    return jnp.concatenate(blocks, axis=0).astype(BF)


def _rec_attention(qrows, kslabs, vslab_fn, filler, keep, lane):
    vslabs = [vslab_fn(0)]
    s = _dot_nt(qrows, _stack(kslabs))
    vslabs += [vslab_fn(j) for j in range(1, H // 2)]
    filler()
    p = _seg_softmax(s, keep, lane)
    o = _dot(p, _stack(vslabs))
    t = o[:, 384:512]
    return jnp.concatenate([o[:, 0:384], t + pltpu.roll(t, 64, 1)], axis=1)


def _b_qk(q, k_s, r0):
    n0 = r0 + T
    s_main = _dot_nt(q, k_s[0:n0, :])
    s_t = [None] + [_dot_nt(q[t * T:, :], k_s[r0 + t * T:r0 + (t + 1) * T, :])
                    for t in range(1, BQ // T)]
    return s_main, s_t


def _b_softmax(scores, r0, tri):
    s_main, s_t = scores
    nt = BQ // T
    n0 = r0 + T
    p_main = []
    p_t = [[] for _ in range(nt)]
    ls = []
    for u in range(nt):
        rows = slice(u * T, (u + 1) * T)
        pieces = []
        if u == 0:
            if r0 > 0:
                pieces.append(s_main[rows, :r0])
            pieces.append(jnp.where(tri, s_main[rows, r0:], NEG))
        else:
            pieces.append(s_main[rows, :])
            for t in range(1, u + 1):
                blk = s_t[t][(u - t) * T:(u - t + 1) * T, :]
                pieces.append(jnp.where(tri, blk, NEG) if t == u else blk)
        s = jnp.concatenate(pieces, axis=1) if len(pieces) > 1 else pieces[0]
        m = jnp.max(s, axis=1, keepdims=True)
        p = jnp.exp2(s - m)
        ls.append(jnp.sum(p, axis=1, keepdims=True))
        p = p.astype(BF)
        p_main.append(p[:, :n0])
        for t in range(1, u + 1):
            p_t[t].append(p[:, n0 + (t - 1) * T:n0 + t * T])
    return p_main, p_t, ls


def _b_pv(probs, v_s, r0):
    p_main, p_t, ls = probs
    nt = BQ // T
    n0 = r0 + T
    pm = jnp.concatenate(p_main, axis=0)
    o = None
    for c0 in range(0, n0, KC):
        c1 = min(c0 + KC, n0)
        oc = _dot(pm[:, c0:c1], v_s[c0:c1, :])
        o = oc if o is None else o + oc
    os_ = [o[u * T:(u + 1) * T] for u in range(nt)]
    for t in range(1, nt):
        ot = _dot(jnp.concatenate(p_t[t], axis=0), v_s[r0 + t * T:r0 + (t + 1) * T, :])
        for u in range(t, nt):
            os_[u] = os_[u] + ot[(u - t) * T:(u - t + 1) * T]
    return jnp.concatenate([os_[u] * (1.0 / ls[u]) for u in range(nt)], axis=0)


def _kernel(xa_hbm, mem0_hbm, wq_hbm, wk_hbm, wv_hbm, wo_hbm,
            xb_hbm, c_hbm, bwq_hbm, bwk_hbm, bwv_hbm, bwo_hbm,
            out_hbm,
            c_s, hm_s, bwo_s, stage_k, stage_v, out_s,
            sems, w_sems, stage_sems, out_sems):

    def stage_copies(chunk, slot):
        rows = pl.ds(chunk * WCH, WCH)
        return (pltpu.make_async_copy(bwk_hbm.at[rows], stage_k.at[slot], stage_sems.at[0, slot]),
                pltpu.make_async_copy(bwv_hbm.at[rows], stage_v.at[slot], stage_sems.at[1, slot]))

    cp_c = pltpu.make_async_copy(c_hbm, c_s, sems.at[3])
    cp_bwo = pltpu.make_async_copy(bwo_hbm, bwo_s, sems.at[4])

    def phase_a(xat_s, xbt_s, mem0_s, wq_raw, wk_raw, wv_raw, bwq_raw, wo_s,
                wq_t, wk_t, wv_t, bwq_s, wck_s, wcv_s, xad_s, xb_s):
        def row_chunk(k, hbm, raw, t):
            rows = pl.ds(t * RCH, RCH)
            return pltpu.make_async_copy(hbm.at[rows], raw.at[rows], w_sems.at[k, t])

        def wo_chunk(j):
            heads = pl.ds(2 * j, 2)
            return pltpu.make_async_copy(wo_hbm.at[heads], wo_s.at[heads], w_sems.at[4, j])

        cp_xa = pltpu.make_async_copy(xa_hbm, xat_s, sems.at[0])
        cp_m0 = pltpu.make_async_copy(mem0_hbm, mem0_s, sems.at[1])
        cp_xb = pltpu.make_async_copy(xb_hbm, xbt_s, sems.at[2])
        for t in range(DM // RCH):
            row_chunk(0, wv_hbm, wv_raw, t).start()
        for j in range(H // 2):
            wo_chunk(j).start()
        for t in range(DM // RCH):
            row_chunk(1, wq_hbm, wq_raw, t).start()
        for t in range(DM // RCH):
            row_chunk(2, wk_hbm, wk_raw, t).start()
        cp_xa.start()
        cp_m0.start()
        for t in range(DM // RCH):
            row_chunk(3, bwq_hbm, bwq_raw, t).start()
        cp_xb.start()
        for s0 in range(NSLOT - 1):
            for cp in stage_copies(s0, s0):
                cp.start()
        for cp in (cp_c, cp_bwo):
            cp.start()

        def relayout(k, hbm, raw, store):
            def body(t, carry):
                row_chunk(k, hbm, raw, t).wait()
                rows = pl.ds(pl.multiple_of(t * RCH, RCH), RCH)
                store(rows, jnp.swapaxes(raw[rows], 0, 1))
                return carry
            lax.fori_loop(0, DM // RCH, body, 0)

        def store_to(dst):
            def store(rows, val):
                dst[:, rows, :] = val
            return store

        def pack_pair(e, o):
            w = jnp.concatenate(
                [e[:, 0:384], o[:, 0:384], e[:, 384:448], o[:, 384:448]], axis=1).astype(BF)
            return pltpu.bitcast(w, jnp.uint32)

        def transpose_x(src, dst):
            def body(t, carry):
                rows = pl.ds(pl.multiple_of(t * 256, 256), 256)
                x = src[:, rows]
                dst[rows, :] = jnp.concatenate([x, x[384:448, :]], axis=0).T
                return carry
            lax.fori_loop(0, S // 256, body, 0)

        relayout(0, wv_hbm, wv_raw, store_to(wv_t))

        def cv_body(j, carry):
            wo_chunk(j).wait()
            e = _dot_nt(wv_t[2 * j], wo_s[2 * j])
            o = _dot_nt(wv_t[2 * j + 1], wo_s[2 * j + 1])
            wcv_s[j] = pack_pair(e, o)
            return carry
        lax.fori_loop(0, H // 2, cv_body, 0, unroll=UCD)

        relayout(1, wq_hbm, wq_raw, store_to(wq_t))
        relayout(2, wk_hbm, wk_raw, store_to(wk_t))

        def ck_body(j, carry):
            e = _dot_nt(wk_t[2 * j], wq_t[2 * j]) * SCALE
            o = _dot_nt(wk_t[2 * j + 1], wq_t[2 * j + 1]) * SCALE
            wck_s[j] = pack_pair(e, o)
            return carry
        lax.fori_loop(0, H // 2, ck_body, 0, unroll=UCD)

        cp_xa.wait()
        cp_m0.wait()
        transpose_x(xat_s, xad_s)
        relayout(3, bwq_hbm, bwq_raw, store_to(bwq_s))
        cp_xb.wait()
        transpose_x(xbt_s, xb_s)

        m0 = mem0_s[...].astype(F32)
        mem_init = jnp.concatenate([m0, m0[:, 384:448]], axis=1)

        def pair_body(i, mem):
            slot = lax.rem(i, NSLOT)
            for cp in stage_copies(i, slot):
                cp.wait()

            @pl.when(i + NSLOT - 1 < _TRIPS['pairs'])
            def _():
                nxt = i + NSLOT - 1
                for cp in stage_copies(nxt, lax.rem(nxt, NSLOT)):
                    cp.start()

            def relayout_piece(n):
                part, src = n % 2, (stage_k, stage_v)[n // 2]
                wrows = pl.ds(pl.multiple_of(S + (n // 2) * DC + i * WCH + part * 16, 16), 16)
                hm_s[:, wrows, :] = jnp.swapaxes(src[slot, part * 16:(part + 1) * 16], 0, 1)

            per_head = S // (4 * FR)
            hq = i // per_head + (H - NPAIR // per_head)
            qbase = lax.rem(i, per_head) * (4 * FR)

            def q_fill(n):
                def run():
                    rows = pl.ds(pl.multiple_of(qbase + n * FR, FR), FR)
                    relayout_piece(n)
                    hm_s[hq, rows, :] = (_dot(xb_s[rows, 0:DM], bwq_s[hq]) * SCALE).astype(BF)
                return run

            lane = lax.broadcasted_iota(jnp.int32, (G, T), 1)
            r = lax.broadcasted_iota(jnp.int32, (G, H * L), 0)
            col = lax.broadcasted_iota(jnp.int32, (G, H * L), 1)
            kk = col - L * ((col * 1639) >> 16)
            keep_e = (r >= 32) | (kk >= 32) | (kk <= r)
            kpos = jnp.where(kk < 24, kk + 8, kk - 32)
            qpos = jnp.where(r < 24, r + 8, r - 32)
            q_any = ((r >= 24) & (r < 32)) | (r >= 40)
            keep_o = q_any | ((kk >= 24) & (kk < 32)) | (kpos <= qpos)

            base = pl.multiple_of(i * 64, 64)
            xs = xad_s[pl.ds(base, 64), :]
            xs32 = xs[32:64, :].astype(F32)

            def proj(lhs, w_s, j):
                return _dot(lhs, pltpu.bitcast(w_s[j], BF))

            def own(x):
                return jnp.concatenate([x[0:32, :], x[40:48, :]], axis=0)

            l1 = jnp.concatenate(
                [xs[0:32, :], jnp.concatenate([xs32[0:8, :], mem], axis=0).astype(BF)], axis=0)
            l1p = l1[:, 0:DM]
            k1 = [proj(l1p, wck_s, j) for j in range(H // 2)]
            v1 = []

            def v1_fn(j):
                v1.append(proj(l1p, wcv_s, j))
                return own(v1[j])

            o1 = _rec_attention(l1, [own(k) for k in k1], v1_fn, q_fill(0), keep_e, lane)
            q_fill(1)()

            l2 = jnp.concatenate([xs32[8:32, :], o1[40:48, :]], axis=0).astype(BF)
            l2p = l2[:, 0:DM]
            k2 = [jnp.concatenate([proj(l2p, wck_s, j), k1[j][32:40, :]], axis=0)
                  for j in range(H // 2)]
            o2 = _rec_attention(
                jnp.concatenate([l2, l1[32:48, :]], axis=0), k2,
                lambda j: jnp.concatenate([proj(l2p, wcv_s, j), v1[j][32:40, :]], axis=0),
                q_fill(2), keep_o, lane)
            q_fill(3)()

            res = jnp.concatenate([o1[0:32, :], o2[32:40, :], o2[0:24, :]], axis=0)
            out_s[pl.ds(base, 64), 0:512] = res.astype(BF)
            return o2[24:32, :]

        lax.fori_loop(0, _TRIPS['pairs'], pair_body, mem_init, unroll=UCH)

    pl.run_scoped(
        phase_a,
        pltpu.VMEM((DM, S), BF), pltpu.VMEM((DM, S), BF), pltpu.VMEM((MEM, DM), BF),
        pltpu.VMEM((DM, H, DH), BF), pltpu.VMEM((DM, H, DH), BF), pltpu.VMEM((DM, H, DH), BF),
        pltpu.VMEM((DM, H, DH), BF),
        pltpu.VMEM((H, DM, DH), BF),
        pltpu.VMEM((H, DM, DH), BF), pltpu.VMEM((H, DM, DH), BF), pltpu.VMEM((H, DM, DH), BF),
        pltpu.VMEM((H, DM, DH), BF),
        pltpu.VMEM((H // 2, DM // 2, PAIR), jnp.uint32),
        pltpu.VMEM((H // 2, DM // 2, PAIR), jnp.uint32),
        pltpu.VMEM((S, 512), BF), pltpu.VMEM((S, 512), BF),
    )

    def phase_b(k_s, v_s, o_s):
        cp_c.wait()
        cp_bwo.wait()

        def head(h, carry):
            k_s[...] = _dot(c_s[...], hm_s[h, S:S + DC, :]).astype(BF)
            v_s[...] = _dot(c_s[...], hm_s[h, S + DC:S + 2 * DC, :]).astype(BF)
            row = lax.broadcasted_iota(jnp.int32, (T, T), 0)
            col = lax.broadcasted_iota(jnp.int32, (T, T), 1)
            tri = row >= col

            def qk(r0):
                q = hm_s[h, r0:r0 + BQ, :]
                return _b_qk(q, k_s, r0)

            starts = list(reversed(range(0, S, BQ)))
            scores = qk(starts[0])
            for n, r0 in enumerate(starts):
                nxt = qk(starts[n + 1]) if n + 1 < len(starts) else None
                probs = _b_softmax(scores, r0, tri)
                o_s[h, r0:r0 + BQ, :] = _b_pv(probs, v_s, r0).astype(BF)
                scores = nxt
            return carry
        lax.fori_loop(0, _TRIPS['heads'], head, 0)

        def out_copy(t):
            rows = pl.ds(pl.multiple_of(t * BO, BO), BO)
            return pltpu.make_async_copy(out_s.at[rows], out_hbm.at[rows], out_sems.at[t])

        def oproj(t, carry):
            rows = pl.ds(pl.multiple_of(t * BO, BO), BO)
            ctx = jnp.concatenate([o_s[h, rows, :] for h in range(H)], axis=1)
            wo = jnp.concatenate([bwo_s[h] for h in range(H)], axis=1)
            if OPT == 0:
                out_s[rows, DM:2 * DM] = _dot_nt(ctx, wo).astype(BF)
            else:
                bt = _dot_nt(wo, ctx)
                if OPT == 1:
                    bt = jnp.concatenate([jnp.zeros((64, BO), F32), bt], axis=0)
                    b = bt.T.astype(BF)
                else:
                    bt = jnp.concatenate([jnp.zeros((64, BO), BF), bt.astype(BF)], axis=0)
                    b = bt.T
                lo = lax.broadcasted_iota(jnp.int32, (BO, T), 1) < 64
                out_s[rows, 384:512] = jnp.where(lo, out_s[rows, 384:512], b[:, 0:T])
                out_s[rows, 512:896] = b[:, T:]
            out_copy(t).start()
            return carry
        lax.fori_loop(0, S // BO, oproj, 0, unroll=UOP)
        for t in range(S // BO):
            out_copy(t).wait()

    pl.run_scoped(
        phase_b,
        pltpu.VMEM((S, DH), BF), pltpu.VMEM((S, DH), BF),
        pltpu.VMEM((H, S, DH), BF),
    )


@functools.partial(jax.jit, static_argnames=("A_seg_len",))
def pallas_concat_heads__memory_aug_recurrent_mem_tr__compressed_kv_cla__prompt_kernel(
    A_x: jax.Array,
    A_mem0: jax.Array,
    A_Wq: jax.Array,
    A_Wk: jax.Array,
    A_Wv: jax.Array,
    A_Wo: jax.Array,
    A_seg_len,
    B_x: jax.Array,
    B_c_kv: jax.Array,
    B_w_q: jax.Array,
    B_w_uk: jax.Array,
    B_w_uv: jax.Array,
    B_w_o: jax.Array,
):
    assert int(A_seg_len) == SEG
    assert A_x.shape == (1, S, DM) and A_mem0.shape == (1, MEM, DM)
    assert A_Wq.shape == (DM, H, DH) and A_Wo.shape == (H, DH, DM)
    assert B_x.shape == (1, S, DM) and B_c_kv.shape == (1, S, DC)
    assert B_w_uk.shape == (DC, H, DH) and B_w_o.shape == (H, DH, DM)

    any_spec = pl.BlockSpec(memory_space=pl.ANY)
    out = pl.pallas_call(
        _kernel,
        out_shape=jax.ShapeDtypeStruct((S, 2 * DM), BF),
        in_specs=[any_spec] * 12,
        out_specs=any_spec,
        scratch_shapes=[
            pltpu.VMEM((S, DC), BF),
            pltpu.VMEM((H, S + 2 * DC, DH), BF),
            pltpu.VMEM((H, DM, DH), BF),
            pltpu.VMEM((NSLOT, WCH, H, DH), BF),
            pltpu.VMEM((NSLOT, WCH, H, DH), BF),
            pltpu.VMEM((S, 2 * DM), BF),
            pltpu.SemaphoreType.DMA((5,)),
            pltpu.SemaphoreType.DMA((5, 8)),
            pltpu.SemaphoreType.DMA((2, NSLOT)),
            pltpu.SemaphoreType.DMA((S // BO,)),
        ],
        compiler_params=pltpu.CompilerParams(vmem_limit_bytes=120 * 1024 * 1024),
    )(jnp.swapaxes(A_x, 1, 2).reshape(DM, S), A_mem0.reshape(MEM, DM), A_Wq, A_Wk, A_Wv,
      jnp.swapaxes(A_Wo, 1, 2),
      jnp.swapaxes(B_x, 1, 2).reshape(DM, S), B_c_kv.reshape(S, DC), B_w_q, B_w_uk, B_w_uv,
      jnp.swapaxes(B_w_o, 1, 2))
    return out.reshape(1, S, 2 * DM)
```

```python
import functools
import os

import jax
import jax.numpy as jnp
from jax import lax
import jax.experimental.pallas as pl
import jax.experimental.pallas.tpu as pltpu

BF = jnp.bfloat16
F32 = jnp.float32

S = 2048
DM = 448
H = 16
DH = 256
MEM = 8
SEG = 32
DC = 1024
LOG2E = 1.4426950408889634
SCALE = DH ** -0.5 * LOG2E
NEG = -1000000000.0 * LOG2E
T = 128
L = MEM + SEG
G = 48
PAIR = 2 * DM
BQ = 512
KC = 256
BO = 256
NPAIR = S // (2 * SEG)
WCH = DC // NPAIR
NSLOT = 3
FILL = [int(v) for v in os.environ.get('FILL', '192,96,224,192,96,224').split(',')]
PIECES = [[int(c) for c in v] for v in os.environ.get('PIECES', '0,,1,2,,3').split(',')]
NV0 = int(os.environ.get('NV0', '0'))
DSCHED = os.environ.get('DS', '000000077')
FR = int(os.environ.get('FR', '256'))
UCD = int(os.environ.get('UCD', '2'))
UCH = int(os.environ.get('UCH', '1'))
UOP = int(os.environ.get('UOP', '2'))
RCH = 64
OPT = int(os.environ.get('OPT', '1'))
BO = int(os.environ.get('BO', '256'))
TIE_ROW = int(os.environ.get('TIE', '480'))
_TRIPS = dict(pairs=NPAIR, heads=H, oproj=S // BO)


def _dot(a, b):
    return jnp.dot(a, b, preferred_element_type=F32)


def _dot_nt(a, b):
    return lax.dot_general(a, b, (((1,), (1,)), ((), ())), preferred_element_type=F32)


def _seg_reduce_bcast(x, lane, fill, combine, reduce_fn):
    nt = H * L // T
    tiles = [x[:, t * T:(t + 1) * T] for t in range(nt)]
    outs = [None] * nt
    for g in range(H):
        parts = []
        for t in range(nt):
            lo = max(L * g - T * t, 0)
            hi = min(L * g + L - T * t, T)
            if lo < hi:
                parts.append((t, (lane >= lo) & (lane < hi)))
        acc = None
        for t, msk in parts:
            sel = jnp.where(msk, tiles[t], fill)
            acc = sel if acc is None else combine(acc, sel)
        red = reduce_fn(acc, axis=1, keepdims=True)
        for t, msk in parts:
            if outs[t] is None:
                outs[t] = jnp.broadcast_to(red, tiles[t].shape)
            else:
                outs[t] = jnp.where(msk, red, outs[t])
    return jnp.concatenate(outs, axis=1)


def _seg_softmax(s, keep, lane):
    s = jnp.where(keep, s, NEG)
    m = _seg_reduce_bcast(s, lane, -jnp.inf, jnp.maximum, jnp.max)
    p = jnp.exp2(s - m)
    l = _seg_reduce_bcast(p, lane, 0.0, jnp.add, jnp.sum)
    return (p * (1.0 / l)).astype(BF)


def _stack(slabs):
    lo = lax.broadcasted_iota(jnp.int32, (L, T), 1) < 64
    blocks = []
    for r in slabs:
        tail = r[:, 768:896]
        blocks.append(jnp.concatenate([r[:, 0:384], jnp.where(lo, tail, 0.0)], axis=1))
        blocks.append(jnp.concatenate([r[:, 384:768], jnp.where(lo, 0.0, tail)], axis=1))
    return jnp.concatenate(blocks, axis=0).astype(BF)


def _rec_attention(qrows, kslabs, vslab_fn, filler0, filler, keep, lane):
    vslabs = [vslab_fn(j) for j in range(NV0)]
    filler0()
    s = _dot_nt(qrows, _stack(kslabs))
    vslabs += [vslab_fn(j) for j in range(NV0, H // 2)]
    filler()
    p = _seg_softmax(s, keep, lane)
    o = _dot(p, _stack(vslabs))
    t = o[:, 384:512]
    return jnp.concatenate([o[:, 0:384], t + pltpu.roll(t, 64, 1)], axis=1)


def _b_qk(q, k_s, r0):
    n0 = r0 + T
    s_main = _dot_nt(q, k_s[0:n0, :])
    s_t = [None] + [_dot_nt(q[t * T:, :], k_s[r0 + t * T:r0 + (t + 1) * T, :])
                    for t in range(1, BQ // T)]
    return s_main, s_t


def _b_softmax(scores, r0, tri):
    s_main, s_t = scores
    nt = BQ // T
    n0 = r0 + T
    p_main = []
    p_t = [[] for _ in range(nt)]
    ls = []
    for u in range(nt):
        rows = slice(u * T, (u + 1) * T)
        pieces = []
        if u == 0:
            if r0 > 0:
                pieces.append(s_main[rows, :r0])
            pieces.append(jnp.where(tri, s_main[rows, r0:], NEG))
        else:
            pieces.append(s_main[rows, :])
            for t in range(1, u + 1):
                blk = s_t[t][(u - t) * T:(u - t + 1) * T, :]
                pieces.append(jnp.where(tri, blk, NEG) if t == u else blk)
        s = jnp.concatenate(pieces, axis=1) if len(pieces) > 1 else pieces[0]
        m = jnp.max(s, axis=1, keepdims=True)
        p = jnp.exp2(s - m)
        ls.append(jnp.sum(p, axis=1, keepdims=True))
        p = p.astype(BF)
        p_main.append(p[:, :n0])
        for t in range(1, u + 1):
            p_t[t].append(p[:, n0 + (t - 1) * T:n0 + t * T])
    return p_main, p_t, ls


def _b_pv(probs, v_s, r0):
    p_main, p_t, ls = probs
    nt = BQ // T
    n0 = r0 + T
    pm = jnp.concatenate(p_main, axis=0)
    o = None
    for c0 in range(0, n0, KC):
        c1 = min(c0 + KC, n0)
        oc = _dot(pm[:, c0:c1], v_s[c0:c1, :])
        o = oc if o is None else o + oc
    os_ = [o[u * T:(u + 1) * T] for u in range(nt)]
    for t in range(1, nt):
        ot = _dot(jnp.concatenate(p_t[t], axis=0), v_s[r0 + t * T:r0 + (t + 1) * T, :])
        for u in range(t, nt):
            os_[u] = os_[u] + ot[(u - t) * T:(u - t + 1) * T]
    return jnp.concatenate([os_[u] * (1.0 / ls[u]) for u in range(nt)], axis=0)


def _kernel(xa_hbm, mem0_hbm, wq_hbm, wk_hbm, wv_hbm, wo_hbm,
            xb_hbm, c_hbm, bwq_hbm, bwk_hbm, bwv_hbm, bwo_hbm,
            out_hbm,
            c_s, hm_s, bwo_s, stage_k, stage_v, out_s,
            sems, w_sems, stage_sems, out_sems):

    def stage_copies(chunk, slot):
        rows = pl.ds(chunk * WCH, WCH)
        return (pltpu.make_async_copy(bwk_hbm.at[rows], stage_k.at[slot], stage_sems.at[0, slot]),
                pltpu.make_async_copy(bwv_hbm.at[rows], stage_v.at[slot], stage_sems.at[1, slot]))

    cp_c = pltpu.make_async_copy(c_hbm, c_s, sems.at[3])
    cp_bwo = pltpu.make_async_copy(bwo_hbm, bwo_s, sems.at[4])

    def phase_a(xat_s, xbt_s, mem0_s, wq_raw, wk_raw, wv_raw, bwq_raw, wo_s,
                wq_t, wk_t, wv_t, bwq_s, wck_s, wcv_s, xad_s, xb_s):
        def row_chunk(k, hbm, raw, t):
            rows = pl.ds(t * RCH, RCH)
            return pltpu.make_async_copy(hbm.at[rows], raw.at[rows], w_sems.at[k, t])

        def wo_chunk(j):
            heads = pl.ds(2 * j, 2)
            return pltpu.make_async_copy(wo_hbm.at[heads], wo_s.at[heads], w_sems.at[4, j])

        cp_xa = pltpu.make_async_copy(xa_hbm, xat_s, sems.at[0])
        cp_m0 = pltpu.make_async_copy(mem0_hbm, mem0_s, sems.at[1])
        cp_xb = pltpu.make_async_copy(xb_hbm, xbt_s, sems.at[2])
        groups = [
            [row_chunk(0, wv_hbm, wv_raw, t) for t in range(DM // RCH)],
            [wo_chunk(j) for j in range(H // 2)],
            [row_chunk(1, wq_hbm, wq_raw, t) for t in range(DM // RCH)],
            [row_chunk(2, wk_hbm, wk_raw, t) for t in range(DM // RCH)],
            [cp_xa, cp_m0],
            [row_chunk(3, bwq_hbm, bwq_raw, t) for t in range(DM // RCH)],
            [cp_xb],
            [cp for s0 in range(NSLOT - 1) for cp in stage_copies(s0, s0)],
            [cp_c, cp_bwo],
        ]

        def start_groups(point):
            for g, when in zip(groups, DSCHED):
                if int(when) == point:
                    for cp in g:
                        cp.start()

        start_groups(0)

        def relayout(k, hbm, raw, store):
            def body(t, carry):
                row_chunk(k, hbm, raw, t).wait()
                rows = pl.ds(pl.multiple_of(t * RCH, RCH), RCH)
                store(rows, jnp.swapaxes(raw[rows], 0, 1))
                return carry
            lax.fori_loop(0, DM // RCH, body, 0)

        def store_to(dst):
            def store(rows, val):
                dst[:, rows, :] = val
            return store

        def pack_pair(e, o):
            w = jnp.concatenate(
                [e[:, 0:384], o[:, 0:384], e[:, 384:448], o[:, 384:448]], axis=1).astype(BF)
            return pltpu.bitcast(w, jnp.uint32)

        def transpose_x(src, dst):
            def body(t, carry):
                rows = pl.ds(pl.multiple_of(t * 256, 256), 256)
                x = src[:, rows]
                dst[rows, :] = jnp.concatenate([x, x[384:448, :]], axis=0).T
                return carry
            lax.fori_loop(0, S // 256, body, 0)

        relayout(0, wv_hbm, wv_raw, store_to(wv_t))
        start_groups(1)

        def cv_body(j, carry):
            wo_chunk(j).wait()
            e = _dot_nt(wv_t[2 * j], wo_s[2 * j])
            o = _dot_nt(wv_t[2 * j + 1], wo_s[2 * j + 1])
            wcv_s[j] = pack_pair(e, o)
            return carry
        lax.fori_loop(0, H // 2, cv_body, 0, unroll=UCD)

        start_groups(2)
        relayout(1, wq_hbm, wq_raw, store_to(wq_t))
        start_groups(3)
        relayout(2, wk_hbm, wk_raw, store_to(wk_t))
        start_groups(4)

        def ck_body(j, carry):
            e = _dot_nt(wk_t[2 * j], wq_t[2 * j]) * SCALE
            o = _dot_nt(wk_t[2 * j + 1], wq_t[2 * j + 1]) * SCALE
            wck_s[j] = pack_pair(e, o)
            return carry
        lax.fori_loop(0, H // 2, ck_body, 0, unroll=UCD)

        start_groups(5)
        cp_xa.wait()
        cp_m0.wait()
        transpose_x(xat_s, xad_s)
        start_groups(6)
        relayout(3, bwq_hbm, bwq_raw, store_to(bwq_s))
        cp_xb.wait()
        start_groups(7)
        transpose_x(xbt_s, xb_s)

        m0 = mem0_s[...].astype(F32)
        mem_init = jnp.concatenate([m0, m0[:, 384:448]], axis=1)

        def pair_body(i, mem):
            slot = lax.rem(i, NSLOT)
            for cp in stage_copies(i, slot):
                cp.wait()

            @pl.when(i + NSLOT - 1 < _TRIPS['pairs'])
            def _():
                nxt = i + NSLOT - 1
                for cp in stage_copies(nxt, lax.rem(nxt, NSLOT)):
                    cp.start()

            def relayout_piece(n):
                part, src = n % 2, (stage_k, stage_v)[n // 2]
                wrows = pl.ds(pl.multiple_of(S + (n // 2) * DC + i * WCH + part * 16, 16), 16)
                hm_s[:, wrows, :] = jnp.swapaxes(src[slot, part * 16:(part + 1) * 16], 0, 1)

            hq = i // 2
            qbase = lax.rem(i, 2) * (S // 2)

            def q_fill(n):
                def run():
                    if FILL[n] == 0:
                        return
                    rows = pl.ds(pl.multiple_of(qbase + sum(FILL[:n]), 16), FILL[n])
                    for piece in PIECES[n]:
                        relayout_piece(piece)
                    hm_s[hq, rows, :] = (_dot(xb_s[rows, 0:DM], bwq_s[hq]) * SCALE).astype(BF)
                return run

            lane = lax.broadcasted_iota(jnp.int32, (G, T), 1)
            r = lax.broadcasted_iota(jnp.int32, (G, H * L), 0)
            col = lax.broadcasted_iota(jnp.int32, (G, H * L), 1)
            kk = col - L * ((col * 1639) >> 16)
            keep_e = (r >= 32) | (kk >= 32) | (kk <= r)
            kpos = jnp.where(kk < 24, kk + 8, kk - 32)
            qpos = jnp.where(r < 24, r + 8, r - 32)
            q_any = ((r >= 24) & (r < 32)) | (r >= 40)
            keep_o = q_any | ((kk >= 24) & (kk < 32)) | (kpos <= qpos)

            base = pl.multiple_of(i * 64, 64)
            xs = xad_s[pl.ds(base, 64), :]
            xs32 = xs[32:64, :].astype(F32)

            def proj(lhs, w_s, j):
                return _dot(lhs, pltpu.bitcast(w_s[j], BF))

            def own(x):
                return jnp.concatenate([x[0:32, :], x[40:48, :]], axis=0)

            l1 = jnp.concatenate(
                [xs[0:32, :], jnp.concatenate([xs32[0:8, :], mem], axis=0).astype(BF)], axis=0)
            l1p = l1[:, 0:DM]
            k1 = [proj(l1p, wck_s, j) for j in range(H // 2)]
            v1 = []

            def v1_fn(j):
                v1.append(proj(l1p, wcv_s, j))
                return own(v1[j])

            o1 = _rec_attention(l1, [own(k) for k in k1], v1_fn, q_fill(0), q_fill(1), keep_e, lane)
            q_fill(2)()

            l2 = jnp.concatenate([xs32[8:32, :], o1[40:48, :]], axis=0).astype(BF)
            l2p = l2[:, 0:DM]
            k2 = [jnp.concatenate([proj(l2p, wck_s, j), k1[j][32:40, :]], axis=0)
                  for j in range(H // 2)]
            o2 = _rec_attention(
                jnp.concatenate([l2, l1[32:48, :]], axis=0), k2,
                lambda j: jnp.concatenate([proj(l2p, wcv_s, j), v1[j][32:40, :]], axis=0),
                q_fill(3), q_fill(4), keep_o, lane)
            q_fill(5)()

            res = jnp.concatenate([o1[0:32, :], o2[32:40, :], o2[0:24, :]], axis=0)
            out_s[pl.ds(base, 64), 0:512] = res.astype(BF)
            return o2[24:32, :]

        lax.fori_loop(0, _TRIPS['pairs'], pair_body, mem_init, unroll=UCH)

    pl.run_scoped(
        phase_a,
        pltpu.VMEM((DM, S), BF), pltpu.VMEM((DM, S), BF), pltpu.VMEM((MEM, DM), BF),
        pltpu.VMEM((DM, H, DH), BF), pltpu.VMEM((DM, H, DH), BF), pltpu.VMEM((DM, H, DH), BF),
        pltpu.VMEM((DM, H, DH), BF),
        pltpu.VMEM((H, DM, DH), BF),
        pltpu.VMEM((H, DM, DH), BF), pltpu.VMEM((H, DM, DH), BF), pltpu.VMEM((H, DM, DH), BF),
        pltpu.VMEM((H, DM, DH), BF),
        pltpu.VMEM((H // 2, DM // 2, PAIR), jnp.uint32),
        pltpu.VMEM((H // 2, DM // 2, PAIR), jnp.uint32),
        pltpu.VMEM((S, 512), BF), pltpu.VMEM((S, 512), BF),
    )

    def phase_b(k_s, v_s, o_s):
        cp_c.wait()
        cp_bwo.wait()

        def head(h, carry):
            k_s[...] = _dot(c_s[...], hm_s[h, S:S + DC, :]).astype(BF)
            v_s[...] = _dot(c_s[...], hm_s[h, S + DC:S + 2 * DC, :]).astype(BF)
            row = lax.broadcasted_iota(jnp.int32, (T, T), 0)
            col = lax.broadcasted_iota(jnp.int32, (T, T), 1)
            tri = row >= col

            def qk(r0):
                q = hm_s[h, r0:r0 + BQ, :]
                return _b_qk(q, k_s, r0)

            starts = list(reversed(range(0, S, BQ)))
            scores = qk(starts[0])
            for n, r0 in enumerate(starts):
                nxt = qk(starts[n + 1]) if n + 1 < len(starts) else None
                probs = _b_softmax(scores, r0, tri)
                o_s[h, r0:r0 + BQ, :] = _b_pv(probs, v_s, r0).astype(BF)
                scores = nxt
            return carry
        lax.fori_loop(0, _TRIPS['heads'], head, 0)

        def out_copy(t):
            rows = pl.ds(pl.multiple_of(t * BO, BO), BO)
            return pltpu.make_async_copy(out_s.at[rows], out_hbm.at[rows], out_sems.at[t])

        def oproj(t, carry):
            rows = pl.ds(pl.multiple_of(t * BO, BO), BO)
            ctx = jnp.concatenate([o_s[h, rows, :] for h in range(H)], axis=1)
            wo = jnp.concatenate([bwo_s[h] for h in range(H)], axis=1)
            if OPT == 0:
                out_s[rows, DM:2 * DM] = _dot_nt(ctx, wo).astype(BF)
            else:
                bt = _dot_nt(wo, ctx)
                if OPT == 1:
                    bt = jnp.concatenate([jnp.zeros((64, BO), F32), bt], axis=0)
                    b = bt.T.astype(BF)
                else:
                    bt = jnp.concatenate([jnp.zeros((64, BO), BF), bt.astype(BF)], axis=0)
                    b = bt.T
                lo = lax.broadcasted_iota(jnp.int32, (BO, T), 1) < 64
                out_s[rows, 384:512] = jnp.where(lo, out_s[rows, 384:512], b[:, 0:T])
                out_s[rows, 512:896] = b[:, T:]
            out_copy(t).start()
            return carry
        lax.fori_loop(0, _TRIPS['oproj'], oproj, 0, unroll=UOP)
        for t in range(_TRIPS['oproj']):
            out_copy(t).wait()

    pl.run_scoped(
        phase_b,
        pltpu.VMEM((S, DH), BF), pltpu.VMEM((S, DH), BF),
        pltpu.VMEM((H, S, DH), BF),
    )


@functools.partial(jax.jit, static_argnames=("A_seg_len",))
def pallas_concat_heads__memory_aug_recurrent_mem_tr__compressed_kv_cla__prompt_kernel(
    A_x: jax.Array,
    A_mem0: jax.Array,
    A_Wq: jax.Array,
    A_Wk: jax.Array,
    A_Wv: jax.Array,
    A_Wo: jax.Array,
    A_seg_len,
    B_x: jax.Array,
    B_c_kv: jax.Array,
    B_w_q: jax.Array,
    B_w_uk: jax.Array,
    B_w_uv: jax.Array,
    B_w_o: jax.Array,
):
    assert int(A_seg_len) == SEG
    assert A_x.shape == (1, S, DM) and A_mem0.shape == (1, MEM, DM)
    assert A_Wq.shape == (DM, H, DH) and A_Wo.shape == (H, DH, DM)
    assert B_x.shape == (1, S, DM) and B_c_kv.shape == (1, S, DC)
    assert B_w_uk.shape == (DC, H, DH) and B_w_o.shape == (H, DH, DM)

    any_spec = pl.BlockSpec(memory_space=pl.ANY)
    out = pl.pallas_call(
        _kernel,
        out_shape=jax.ShapeDtypeStruct((S, 2 * DM), BF),
        in_specs=[any_spec] * 12,
        out_specs=any_spec,
        scratch_shapes=[
            pltpu.VMEM((S, DC), BF),
            pltpu.VMEM((H, S + 2 * DC, DH), BF),
            pltpu.VMEM((H, DM, DH), BF),
            pltpu.VMEM((NSLOT, WCH, H, DH), BF),
            pltpu.VMEM((NSLOT, WCH, H, DH), BF),
            pltpu.VMEM((S, 2 * DM), BF),
            pltpu.SemaphoreType.DMA((5,)),
            pltpu.SemaphoreType.DMA((5, 8)),
            pltpu.SemaphoreType.DMA((2, NSLOT)),
            pltpu.SemaphoreType.DMA((S // BO,)),
        ],
        compiler_params=pltpu.CompilerParams(vmem_limit_bytes=120 * 1024 * 1024),
    )(jnp.swapaxes(A_x, 1, 2).reshape(DM, S), A_mem0.reshape(MEM, DM), A_Wq, A_Wk, A_Wv,
      jnp.swapaxes(A_Wo, 1, 2),
      jnp.swapaxes(B_x, 1, 2).reshape(DM, S), B_c_kv.reshape(S, DC), B_w_q, B_w_uk, B_w_uv,
      jnp.swapaxes(B_w_o, 1, 2))
    return out.reshape(1, S, 2 * DM)
```

```python
import functools
import os

import jax
import jax.numpy as jnp
from jax import lax
import jax.experimental.pallas as pl
import jax.experimental.pallas.tpu as pltpu

BF = jnp.bfloat16
F32 = jnp.float32

S = 2048
DM = 448
H = 16
DH = 256
MEM = 8
SEG = 32
DC = 1024
LOG2E = 1.4426950408889634
SCALE = DH ** -0.5 * LOG2E
NEG = -1000000000.0 * LOG2E
T = 128
L = MEM + SEG
G = 48
PAIR = 2 * DM
BQ = int(os.environ.get('BQ', '512'))
KC = int(os.environ.get('KC', '256'))
BO = 256
NPAIR = S // (2 * SEG)
WCH = DC // NPAIR
NSLOT = 3
OTIE = int(os.environ.get('OTIE', '2'))
LTIE = int(os.environ.get('LTIE', '0'))
FILL = [int(v) for v in os.environ.get('FILL', '192,96,224,192,96,224').split(',')]
PIECES = [[int(c) for c in v] for v in os.environ.get('PIECES', '0,,1,2,,3').split(',')]
NV0 = int(os.environ.get('NV0', '0'))
DSCHED = os.environ.get('DS', '000000077')
FR = int(os.environ.get('FR', '256'))
UCD = int(os.environ.get('UCD', '2'))
UCH = int(os.environ.get('UCH', '1'))
UOP = int(os.environ.get('UOP', '2'))
RCH = 64
OPT = int(os.environ.get('OPT', '1'))
BO = int(os.environ.get('BO', '256'))
TIE_ROW = int(os.environ.get('TIE', '480'))
_TRIPS = dict(pairs=NPAIR, heads=H, oproj=S // BO)


def _dot(a, b):
    return jnp.dot(a, b, preferred_element_type=F32)


def _dot_nt(a, b):
    return lax.dot_general(a, b, (((1,), (1,)), ((), ())), preferred_element_type=F32)


def _seg_reduce_bcast(x, lane, fill, combine, reduce_fn):
    nt = H * L // T
    tiles = [x[:, t * T:(t + 1) * T] for t in range(nt)]
    outs = [None] * nt
    for g in range(H):
        parts = []
        for t in range(nt):
            lo = max(L * g - T * t, 0)
            hi = min(L * g + L - T * t, T)
            if lo < hi:
                parts.append((t, (lane >= lo) & (lane < hi)))
        acc = None
        for t, msk in parts:
            sel = jnp.where(msk, tiles[t], fill)
            acc = sel if acc is None else combine(acc, sel)
        red = reduce_fn(acc, axis=1, keepdims=True)
        for t, msk in parts:
            if outs[t] is None:
                outs[t] = jnp.broadcast_to(red, tiles[t].shape)
            else:
                outs[t] = jnp.where(msk, red, outs[t])
    return jnp.concatenate(outs, axis=1)


def _seg_softmax(s, keep, lane):
    s = jnp.where(keep, s, NEG)
    m = _seg_reduce_bcast(s, lane, -jnp.inf, jnp.maximum, jnp.max)
    p = jnp.exp2(s - m)
    l = _seg_reduce_bcast(p, lane, 0.0, jnp.add, jnp.sum)
    return (p * (1.0 / l)).astype(BF)


def _stack(slabs):
    lo = lax.broadcasted_iota(jnp.int32, (L, T), 1) < 64
    blocks = []
    for r in slabs:
        tail = r[:, 768:896]
        blocks.append(jnp.concatenate([r[:, 0:384], jnp.where(lo, tail, 0.0)], axis=1))
        blocks.append(jnp.concatenate([r[:, 384:768], jnp.where(lo, 0.0, tail)], axis=1))
    return jnp.concatenate(blocks, axis=0).astype(BF)


def _rec_attention(qrows, kslabs, vslab_fn, filler0, filler, keep, lane):
    vslabs = [vslab_fn(j) for j in range(NV0)]
    filler0()
    s = _dot_nt(qrows, _stack(kslabs))
    vslabs += [vslab_fn(j) for j in range(NV0, H // 2)]
    filler()
    p = _seg_softmax(s, keep, lane)
    o = _dot(p, _stack(vslabs))
    t = o[:, 384:512]
    return jnp.concatenate([o[:, 0:384], t + pltpu.roll(t, 64, 1)], axis=1)


def _b_qk(q, k_s, r0, tri):
    nt = BQ // T

    def mask_top(blk):
        top = jnp.where(tri, blk[0:T, :], NEG)
        return jnp.concatenate([top, blk[T:, :]], axis=0) if blk.shape[0] > T else top

    s_main = _dot_nt(q, k_s[0:r0 + T, :])
    chunks = [(0, c0, s_main[:, c0:min(c0 + KC, r0)]) for c0 in range(0, r0, KC)]
    chunks.append((0, r0, mask_top(s_main[:, r0:r0 + T])))
    for t in range(1, nt):
        chunks.append((t * T, r0 + t * T, mask_top(
            _dot_nt(q[t * T:, :], k_s[r0 + t * T:r0 + (t + 1) * T, :]))))
    ms = []
    for u in range(nt):
        row = [c[u * T - f:(u + 1) * T - f, :] for f, _, c in chunks if f <= u * T]
        row = jnp.concatenate(row, axis=1) if len(row) > 1 else row[0]
        ms.append(jnp.max(row, axis=1, keepdims=True))
    return chunks, jnp.concatenate(ms, axis=0)


def _b_pv(scores, v_s, never):
    chunks, m = scores
    nt = BQ // T
    o = [None] * nt
    l = None
    ocs = []
    mb = jnp.broadcast_to(m, (BQ, T))
    for f, k0, c in chunks:
        mc = mb if (l is None or not LTIE) else jnp.where(never, l, mb)
        mc = mc[f:, :]
        if OTIE and len(ocs) >= OTIE:
            pf, prev = ocs[-OTIE]
            mc = jnp.where(never, prev[f - pf:, 0:T], mc)
        ps = [jnp.exp2(c[:, j * T:(j + 1) * T] - mc) for j in range(c.shape[1] // T)]
        p = jnp.concatenate(ps, axis=1) if len(ps) > 1 else ps[0]
        oc = _dot(p.astype(BF), v_s[k0:k0 + c.shape[1], :])
        ocs.append((f, oc))
        lc = ps[0]
        for x in ps[1:]:
            lc = lc + x
        if l is None:
            l = lc
        elif f == 0:
            l = l + lc
        else:
            l = jnp.concatenate([l[0:f, :], l[f:, :] + lc], axis=0)
        for u in range(f // T, nt):
            rows = slice(u * T - f, (u + 1) * T - f)
            o[u] = oc[rows] if o[u] is None else o[u] + oc[rows]
    return jnp.concatenate(o, axis=0) * (1.0 / jnp.sum(l, axis=1, keepdims=True))


def _kernel(xa_hbm, mem0_hbm, wq_hbm, wk_hbm, wv_hbm, wo_hbm,
            xb_hbm, c_hbm, bwq_hbm, bwk_hbm, bwv_hbm, bwo_hbm,
            out_hbm,
            c_s, hm_s, bwo_s, stage_k, stage_v, out_s,
            sems, w_sems, stage_sems, out_sems):

    def stage_copies(chunk, slot):
        rows = pl.ds(chunk * WCH, WCH)
        return (pltpu.make_async_copy(bwk_hbm.at[rows], stage_k.at[slot], stage_sems.at[0, slot]),
                pltpu.make_async_copy(bwv_hbm.at[rows], stage_v.at[slot], stage_sems.at[1, slot]))

    cp_c = pltpu.make_async_copy(c_hbm, c_s, sems.at[3])
    cp_bwo = pltpu.make_async_copy(bwo_hbm, bwo_s, sems.at[4])

    def phase_a(xat_s, xbt_s, mem0_s, wq_raw, wk_raw, wv_raw, bwq_raw, wo_s,
                wq_t, wk_t, wv_t, bwq_s, wck_s, wcv_s, xad_s, xb_s):
        def row_chunk(k, hbm, raw, t):
            rows = pl.ds(t * RCH, RCH)
            return pltpu.make_async_copy(hbm.at[rows], raw.at[rows], w_sems.at[k, t])

        def wo_chunk(j):
            heads = pl.ds(2 * j, 2)
            return pltpu.make_async_copy(wo_hbm.at[heads], wo_s.at[heads], w_sems.at[4, j])

        cp_xa = pltpu.make_async_copy(xa_hbm, xat_s, sems.at[0])
        cp_m0 = pltpu.make_async_copy(mem0_hbm, mem0_s, sems.at[1])
        cp_xb = pltpu.make_async_copy(xb_hbm, xbt_s, sems.at[2])
        groups = [
            [row_chunk(0, wv_hbm, wv_raw, t) for t in range(DM // RCH)],
            [wo_chunk(j) for j in range(H // 2)],
            [row_chunk(1, wq_hbm, wq_raw, t) for t in range(DM // RCH)],
            [row_chunk(2, wk_hbm, wk_raw, t) for t in range(DM // RCH)],
            [cp_xa, cp_m0],
            [row_chunk(3, bwq_hbm, bwq_raw, t) for t in range(DM // RCH)],
            [cp_xb],
            [cp for s0 in range(NSLOT - 1) for cp in stage_copies(s0, s0)],
            [cp_c, cp_bwo],
        ]

        def start_groups(point):
            for g, when in zip(groups, DSCHED):
                if int(when) == point:
                    for cp in g:
                        cp.start()

        start_groups(0)

        def relayout(k, hbm, raw, store):
            def body(t, carry):
                row_chunk(k, hbm, raw, t).wait()
                rows = pl.ds(pl.multiple_of(t * RCH, RCH), RCH)
                store(rows, jnp.swapaxes(raw[rows], 0, 1))
                return carry
            lax.fori_loop(0, DM // RCH, body, 0)

        def store_to(dst):
            def store(rows, val):
                dst[:, rows, :] = val
            return store

        def pack_pair(e, o):
            w = jnp.concatenate(
                [e[:, 0:384], o[:, 0:384], e[:, 384:448], o[:, 384:448]], axis=1).astype(BF)
            return pltpu.bitcast(w, jnp.uint32)

        def transpose_x(src, dst):
            def body(t, carry):
                rows = pl.ds(pl.multiple_of(t * 256, 256), 256)
                x = src[:, rows]
                dst[rows, :] = jnp.concatenate([x, x[384:448, :]], axis=0).T
                return carry
            lax.fori_loop(0, S // 256, body, 0)

        relayout(0, wv_hbm, wv_raw, store_to(wv_t))
        start_groups(1)

        def cv_body(j, carry):
            wo_chunk(j).wait()
            e = _dot_nt(wv_t[2 * j], wo_s[2 * j])
            o = _dot_nt(wv_t[2 * j + 1], wo_s[2 * j + 1])
            wcv_s[j] = pack_pair(e, o)
            return carry
        lax.fori_loop(0, H // 2, cv_body, 0, unroll=UCD)

        start_groups(2)
        relayout(1, wq_hbm, wq_raw, store_to(wq_t))
        start_groups(3)
        relayout(2, wk_hbm, wk_raw, store_to(wk_t))
        start_groups(4)

        def ck_body(j, carry):
            e = _dot_nt(wk_t[2 * j], wq_t[2 * j]) * SCALE
            o = _dot_nt(wk_t[2 * j + 1], wq_t[2 * j + 1]) * SCALE
            wck_s[j] = pack_pair(e, o)
            return carry
        lax.fori_loop(0, H // 2, ck_body, 0, unroll=UCD)

        start_groups(5)
        cp_xa.wait()
        cp_m0.wait()
        transpose_x(xat_s, xad_s)
        start_groups(6)
        relayout(3, bwq_hbm, bwq_raw, store_to(bwq_s))
        cp_xb.wait()
        start_groups(7)
        transpose_x(xbt_s, xb_s)

        m0 = mem0_s[...].astype(F32)
        mem_init = jnp.concatenate([m0, m0[:, 384:448]], axis=1)

        def pair_body(i, mem):
            slot = lax.rem(i, NSLOT)
            for cp in stage_copies(i, slot):
                cp.wait()

            @pl.when(i + NSLOT - 1 < _TRIPS['pairs'])
            def _():
                nxt = i + NSLOT - 1
                for cp in stage_copies(nxt, lax.rem(nxt, NSLOT)):
                    cp.start()

            def relayout_piece(n):
                part, src = n % 2, (stage_k, stage_v)[n // 2]
                wrows = pl.ds(pl.multiple_of(S + (n // 2) * DC + i * WCH + part * 16, 16), 16)
                hm_s[:, wrows, :] = jnp.swapaxes(src[slot, part * 16:(part + 1) * 16], 0, 1)

            hq = i // 2
            qbase = lax.rem(i, 2) * (S // 2)

            def q_fill(n):
                def run():
                    if FILL[n] == 0:
                        return
                    rows = pl.ds(pl.multiple_of(qbase + sum(FILL[:n]), 16), FILL[n])
                    for piece in PIECES[n]:
                        relayout_piece(piece)
                    hm_s[hq, rows, :] = (_dot(xb_s[rows, 0:DM], bwq_s[hq]) * SCALE).astype(BF)
                return run

            lane = lax.broadcasted_iota(jnp.int32, (G, T), 1)
            r = lax.broadcasted_iota(jnp.int32, (G, H * L), 0)
            col = lax.broadcasted_iota(jnp.int32, (G, H * L), 1)
            kk = col - L * ((col * 1639) >> 16)
            keep_e = (r >= 32) | (kk >= 32) | (kk <= r)
            kpos = jnp.where(kk < 24, kk + 8, kk - 32)
            qpos = jnp.where(r < 24, r + 8, r - 32)
            q_any = ((r >= 24) & (r < 32)) | (r >= 40)
            keep_o = q_any | ((kk >= 24) & (kk < 32)) | (kpos <= qpos)

            base = pl.multiple_of(i * 64, 64)
            xs = xad_s[pl.ds(base, 64), :]
            xs32 = xs[32:64, :].astype(F32)

            def proj(lhs, w_s, j):
                return _dot(lhs, pltpu.bitcast(w_s[j], BF))

            def own(x):
                return jnp.concatenate([x[0:32, :], x[40:48, :]], axis=0)

            l1 = jnp.concatenate(
                [xs[0:32, :], jnp.concatenate([xs32[0:8, :], mem], axis=0).astype(BF)], axis=0)
            l1p = l1[:, 0:DM]
            k1 = [proj(l1p, wck_s, j) for j in range(H // 2)]
            v1 = []

            def v1_fn(j):
                v1.append(proj(l1p, wcv_s, j))
                return own(v1[j])

            o1 = _rec_attention(l1, [own(k) for k in k1], v1_fn, q_fill(0), q_fill(1), keep_e, lane)
            q_fill(2)()

            l2 = jnp.concatenate([xs32[8:32, :], o1[40:48, :]], axis=0).astype(BF)
            l2p = l2[:, 0:DM]
            k2 = [jnp.concatenate([proj(l2p, wck_s, j), k1[j][32:40, :]], axis=0)
                  for j in range(H // 2)]
            o2 = _rec_attention(
                jnp.concatenate([l2, l1[32:48, :]], axis=0), k2,
                lambda j: jnp.concatenate([proj(l2p, wcv_s, j), v1[j][32:40, :]], axis=0),
                q_fill(3), q_fill(4), keep_o, lane)
            q_fill(5)()

            res = jnp.concatenate([o1[0:32, :], o2[32:40, :], o2[0:24, :]], axis=0)
            out_s[pl.ds(base, 64), 0:512] = res.astype(BF)
            return o2[24:32, :]

        lax.fori_loop(0, _TRIPS['pairs'], pair_body, mem_init, unroll=UCH)

    pl.run_scoped(
        phase_a,
        pltpu.VMEM((DM, S), BF), pltpu.VMEM((DM, S), BF), pltpu.VMEM((MEM, DM), BF),
        pltpu.VMEM((DM, H, DH), BF), pltpu.VMEM((DM, H, DH), BF), pltpu.VMEM((DM, H, DH), BF),
        pltpu.VMEM((DM, H, DH), BF),
        pltpu.VMEM((H, DM, DH), BF),
        pltpu.VMEM((H, DM, DH), BF), pltpu.VMEM((H, DM, DH), BF), pltpu.VMEM((H, DM, DH), BF),
        pltpu.VMEM((H, DM, DH), BF),
        pltpu.VMEM((H // 2, DM // 2, PAIR), jnp.uint32),
        pltpu.VMEM((H // 2, DM // 2, PAIR), jnp.uint32),
        pltpu.VMEM((S, 512), BF), pltpu.VMEM((S, 512), BF),
    )

    def phase_b(k_s, v_s, o_s):
        cp_c.wait()
        cp_bwo.wait()

        def head(h, carry):
            k_s[...] = _dot(c_s[...], hm_s[h, S:S + DC, :]).astype(BF)
            v_s[...] = _dot(c_s[...], hm_s[h, S + DC:S + 2 * DC, :]).astype(BF)
            row = lax.broadcasted_iota(jnp.int32, (T, T), 0)
            col = lax.broadcasted_iota(jnp.int32, (T, T), 1)
            tri = row >= col

            def qk(r0):
                q = hm_s[h, r0:r0 + BQ, :]
                return _b_qk(q, k_s, r0, tri)

            starts = list(reversed(range(0, S, BQ)))
            scores = qk(starts[0])
            for n, r0 in enumerate(starts):
                nxt = qk(starts[n + 1]) if n + 1 < len(starts) else None
                o_s[h, r0:r0 + BQ, :] = _b_pv(scores, v_s, h < 0).astype(BF)
                scores = nxt
            return carry
        lax.fori_loop(0, _TRIPS['heads'], head, 0)

        def out_copy(t):
            rows = pl.ds(pl.multiple_of(t * BO, BO), BO)
            return pltpu.make_async_copy(out_s.at[rows], out_hbm.at[rows], out_sems.at[t])

        def oproj(t, carry):
            rows = pl.ds(pl.multiple_of(t * BO, BO), BO)
            ctx = jnp.concatenate([o_s[h, rows, :] for h in range(H)], axis=1)
            wo = jnp.concatenate([bwo_s[h] for h in range(H)], axis=1)
            if OPT == 0:
                out_s[rows, DM:2 * DM] = _dot_nt(ctx, wo).astype(BF)
            else:
                bt = _dot_nt(wo, ctx)
                if OPT == 1:
                    bt = jnp.concatenate([jnp.zeros((64, BO), F32), bt], axis=0)
                    b = bt.T.astype(BF)
                else:
                    bt = jnp.concatenate([jnp.zeros((64, BO), BF), bt.astype(BF)], axis=0)
                    b = bt.T
                lo = lax.broadcasted_iota(jnp.int32, (BO, T), 1) < 64
                out_s[rows, 384:512] = jnp.where(lo, out_s[rows, 384:512], b[:, 0:T])
                out_s[rows, 512:896] = b[:, T:]
            out_copy(t).start()
            return carry
        lax.fori_loop(0, _TRIPS['oproj'], oproj, 0, unroll=UOP)
        for t in range(_TRIPS['oproj']):
            out_copy(t).wait()

    pl.run_scoped(
        phase_b,
        pltpu.VMEM((S, DH), BF), pltpu.VMEM((S, DH), BF),
        pltpu.VMEM((H, S, DH), BF),
    )


@functools.partial(jax.jit, static_argnames=("A_seg_len",))
def pallas_concat_heads__memory_aug_recurrent_mem_tr__compressed_kv_cla__prompt_kernel(
    A_x: jax.Array,
    A_mem0: jax.Array,
    A_Wq: jax.Array,
    A_Wk: jax.Array,
    A_Wv: jax.Array,
    A_Wo: jax.Array,
    A_seg_len,
    B_x: jax.Array,
    B_c_kv: jax.Array,
    B_w_q: jax.Array,
    B_w_uk: jax.Array,
    B_w_uv: jax.Array,
    B_w_o: jax.Array,
):
    assert int(A_seg_len) == SEG
    assert A_x.shape == (1, S, DM) and A_mem0.shape == (1, MEM, DM)
    assert A_Wq.shape == (DM, H, DH) and A_Wo.shape == (H, DH, DM)
    assert B_x.shape == (1, S, DM) and B_c_kv.shape == (1, S, DC)
    assert B_w_uk.shape == (DC, H, DH) and B_w_o.shape == (H, DH, DM)

    any_spec = pl.BlockSpec(memory_space=pl.ANY)
    out = pl.pallas_call(
        _kernel,
        out_shape=jax.ShapeDtypeStruct((S, 2 * DM), BF),
        in_specs=[any_spec] * 12,
        out_specs=any_spec,
        scratch_shapes=[
            pltpu.VMEM((S, DC), BF),
            pltpu.VMEM((H, S + 2 * DC, DH), BF),
            pltpu.VMEM((H, DM, DH), BF),
            pltpu.VMEM((NSLOT, WCH, H, DH), BF),
            pltpu.VMEM((NSLOT, WCH, H, DH), BF),
            pltpu.VMEM((S, 2 * DM), BF),
            pltpu.SemaphoreType.DMA((5,)),
            pltpu.SemaphoreType.DMA((5, 8)),
            pltpu.SemaphoreType.DMA((2, NSLOT)),
            pltpu.SemaphoreType.DMA((S // BO,)),
        ],
        compiler_params=pltpu.CompilerParams(vmem_limit_bytes=120 * 1024 * 1024),
    )(jnp.swapaxes(A_x, 1, 2).reshape(DM, S), A_mem0.reshape(MEM, DM), A_Wq, A_Wk, A_Wv,
      jnp.swapaxes(A_Wo, 1, 2),
      jnp.swapaxes(B_x, 1, 2).reshape(DM, S), B_c_kv.reshape(S, DC), B_w_q, B_w_uk, B_w_uv,
      jnp.swapaxes(B_w_o, 1, 2))
    return out.reshape(1, S, 2 * DM)
```

```python
import jax
import jax.numpy as jnp
from jax import lax
import jax.experimental.pallas as pl
import jax.experimental.pallas.tpu as pltpu

BF = jnp.bfloat16
F32 = jnp.float32

S = 2048
DM = 448
H = 16
DH = 256
MEM = 8
SEG = 32
DC = 1024
LOG2E = 1.4426950408889634
SCALE = DH ** -0.5 * LOG2E
NEG = -1000000000.0 * LOG2E
T = 128
L = MEM + SEG
G = 48
PAIR = 2 * DM
BQ = 512
KC = 256
BO = 256
NPAIR = S // (2 * SEG)
WCH = DC // NPAIR
NSLOT = 3
RCH = 64
LAG = 2
FILL = (192, 96, 224, 192, 96, 224)
PIECES = ((0,), (), (1,), (2,), (), (3,))


def _dot(a, b):
    return jnp.dot(a, b, preferred_element_type=F32)


def _dot_nt(a, b):
    return lax.dot_general(a, b, (((1,), (1,)), ((), ())), preferred_element_type=F32)


def _seg_reduce_bcast(x, lane, fill, combine, reduce_fn):
    nt = H * L // T
    tiles = [x[:, t * T:(t + 1) * T] for t in range(nt)]
    outs = [None] * nt
    for g in range(H):
        parts = []
        for t in range(nt):
            lo = max(L * g - T * t, 0)
            hi = min(L * g + L - T * t, T)
            if lo < hi:
                parts.append((t, (lane >= lo) & (lane < hi)))
        acc = None
        for t, msk in parts:
            sel = jnp.where(msk, tiles[t], fill)
            acc = sel if acc is None else combine(acc, sel)
        red = reduce_fn(acc, axis=1, keepdims=True)
        for t, msk in parts:
            if outs[t] is None:
                outs[t] = jnp.broadcast_to(red, tiles[t].shape)
            else:
                outs[t] = jnp.where(msk, red, outs[t])
    return jnp.concatenate(outs, axis=1)


def _seg_softmax(s, keep, lane):
    s = jnp.where(keep, s, NEG)
    m = _seg_reduce_bcast(s, lane, -jnp.inf, jnp.maximum, jnp.max)
    p = jnp.exp2(s - m)
    l = _seg_reduce_bcast(p, lane, 0.0, jnp.add, jnp.sum)
    return (p * (1.0 / l)).astype(BF)


def _stack(slabs):
    lo = lax.broadcasted_iota(jnp.int32, (L, T), 1) < 64
    blocks = []
    for r in slabs:
        tail = r[:, 768:896]
        blocks.append(jnp.concatenate([r[:, 0:384], jnp.where(lo, tail, 0.0)], axis=1))
        blocks.append(jnp.concatenate([r[:, 384:768], jnp.where(lo, 0.0, tail)], axis=1))
    return jnp.concatenate(blocks, axis=0).astype(BF)


def _rec_attention(qrows, kslabs, vslab_fn, filler0, filler, keep, lane):
    filler0()
    s = _dot_nt(qrows, _stack(kslabs))
    vslabs = [vslab_fn(j) for j in range(H // 2)]
    filler()
    p = _seg_softmax(s, keep, lane)
    o = _dot(p, _stack(vslabs))
    t = o[:, 384:512]
    return jnp.concatenate([o[:, 0:384], t + pltpu.roll(t, 64, 1)], axis=1)


def _b_qk(q, k_s, r0, tri):
    nt = BQ // T

    def mask_top(blk):
        top = jnp.where(tri, blk[0:T, :], NEG)
        return jnp.concatenate([top, blk[T:, :]], axis=0) if blk.shape[0] > T else top

    s_main = _dot_nt(q, k_s[0:r0 + T, :])
    chunks = [(0, c0, s_main[:, c0:min(c0 + KC, r0)]) for c0 in range(0, r0, KC)]
    chunks.append((0, r0, mask_top(s_main[:, r0:r0 + T])))
    for t in range(1, nt):
        chunks.append((t * T, r0 + t * T, mask_top(
            _dot_nt(q[t * T:, :], k_s[r0 + t * T:r0 + (t + 1) * T, :]))))
    ms = []
    for u in range(nt):
        row = [c[u * T - f:(u + 1) * T - f, :] for f, _, c in chunks if f <= u * T]
        row = jnp.concatenate(row, axis=1) if len(row) > 1 else row[0]
        ms.append(jnp.max(row, axis=1, keepdims=True))
    return chunks, jnp.concatenate(ms, axis=0)


def _b_pv(scores, v_s, never):
    chunks, m = scores
    nt = BQ // T
    o = [None] * nt
    l = None
    ocs = []
    mb = jnp.broadcast_to(m, (BQ, T))
    for f, k0, c in chunks:
        mc = mb[f:, :]
        if len(ocs) >= LAG:
            pf, prev = ocs[-LAG]
            mc = jnp.where(never, prev[f - pf:, 0:T], mc)
        ps = [jnp.exp2(c[:, j * T:(j + 1) * T] - mc) for j in range(c.shape[1] // T)]
        p = jnp.concatenate(ps, axis=1) if len(ps) > 1 else ps[0]
        oc = _dot(p.astype(BF), v_s[k0:k0 + c.shape[1], :])
        ocs.append((f, oc))
        lc = ps[0]
        for x in ps[1:]:
            lc = lc + x
        if l is None:
            l = lc
        elif f == 0:
            l = l + lc
        else:
            l = jnp.concatenate([l[0:f, :], l[f:, :] + lc], axis=0)
        for u in range(f // T, nt):
            rows = slice(u * T - f, (u + 1) * T - f)
            o[u] = oc[rows] if o[u] is None else o[u] + oc[rows]
    return jnp.concatenate(o, axis=0) * (1.0 / jnp.sum(l, axis=1, keepdims=True))


def _kernel(xa_hbm, mem0_hbm, wq_hbm, wk_hbm, wv_hbm, wo_hbm,
            xb_hbm, c_hbm, bwq_hbm, bwk_hbm, bwv_hbm, bwo_hbm,
            out_hbm,
            c_s, hm_s, bwo_s, stage_k, stage_v, out_s,
            sems, w_sems, stage_sems, out_sems):

    def stage_copies(chunk, slot):
        rows = pl.ds(chunk * WCH, WCH)
        return (pltpu.make_async_copy(bwk_hbm.at[rows], stage_k.at[slot], stage_sems.at[0, slot]),
                pltpu.make_async_copy(bwv_hbm.at[rows], stage_v.at[slot], stage_sems.at[1, slot]))

    cp_c = pltpu.make_async_copy(c_hbm, c_s, sems.at[3])
    cp_bwo = pltpu.make_async_copy(bwo_hbm, bwo_s, sems.at[4])

    def phase_a(xat_s, xbt_s, mem0_s, wq_raw, wk_raw, wv_raw, bwq_raw, wo_s,
                wq_t, wv_t, bwq_s, wck_s, wcv_s, xad_s, xb_s):
        def row_chunk(k, hbm, raw, t):
            rows = pl.ds(t * RCH, RCH)
            return pltpu.make_async_copy(hbm.at[rows], raw.at[rows], w_sems.at[k, t])

        def wo_chunk(j):
            heads = pl.ds(2 * j, 2)
            return pltpu.make_async_copy(wo_hbm.at[heads], wo_s.at[heads], w_sems.at[4, j])

        cp_xa = pltpu.make_async_copy(xa_hbm, xat_s, sems.at[0])
        cp_m0 = pltpu.make_async_copy(mem0_hbm, mem0_s, sems.at[1])
        cp_xb = pltpu.make_async_copy(xb_hbm, xbt_s, sems.at[2])
        early = [row_chunk(0, wv_hbm, wv_raw, t) for t in range(DM // RCH)]
        early += [wo_chunk(j) for j in range(H // 2)]
        early += [row_chunk(1, wq_hbm, wq_raw, t) for t in range(DM // RCH)]
        early += [row_chunk(2, wk_hbm, wk_raw, t) for t in range(DM // RCH)]
        early += [cp_xa, cp_m0]
        early += [row_chunk(3, bwq_hbm, bwq_raw, t) for t in range(DM // RCH)]
        early += [cp_xb]
        for cp in early:
            cp.start()

        def relayout(k, hbm, raw, dst):
            def body(t, carry):
                row_chunk(k, hbm, raw, t).wait()
                rows = pl.ds(pl.multiple_of(t * RCH, RCH), RCH)
                dst[:, rows, :] = jnp.swapaxes(raw[rows], 0, 1)
                return carry
            lax.fori_loop(0, DM // RCH, body, 0)

        def pack_pair(e, o):
            w = jnp.concatenate(
                [e[:, 0:384], o[:, 0:384], e[:, 384:448], o[:, 384:448]], axis=1).astype(BF)
            return pltpu.bitcast(w, jnp.uint32)

        def transpose_x(src, dst):
            def body(t, carry):
                rows = pl.ds(pl.multiple_of(t * 256, 256), 256)
                x = src[:, rows]
                dst[rows, :] = jnp.concatenate([x, x[384:448, :]], axis=0).T
                return carry
            lax.fori_loop(0, S // 256, body, 0)

        relayout(0, wv_hbm, wv_raw, wv_t)

        def cv_body(j, carry):
            wo_chunk(j).wait()
            e = _dot_nt(wv_t[2 * j], wo_s[2 * j])
            o = _dot_nt(wv_t[2 * j + 1], wo_s[2 * j + 1])
            wcv_s[j] = pack_pair(e, o)
            return carry
        lax.fori_loop(0, H // 2, cv_body, 0, unroll=2)

        relayout(1, wq_hbm, wq_raw, wq_t)

        def ck_body(t, carry):
            row_chunk(2, wk_hbm, wk_raw, t).wait()
            wk = jnp.swapaxes(wk_raw[pl.ds(pl.multiple_of(t * RCH, RCH), RCH)], 0, 1)
            rows = pl.ds(pl.multiple_of(t * (RCH // 2), RCH // 2), RCH // 2)
            for j in range(H // 2):
                e = _dot_nt(wk[2 * j], wq_t[2 * j]) * SCALE
                o = _dot_nt(wk[2 * j + 1], wq_t[2 * j + 1]) * SCALE
                wck_s[j, rows, :] = pack_pair(e, o)
            return carry
        lax.fori_loop(0, DM // RCH, ck_body, 0)

        cp_xa.wait()
        cp_m0.wait()
        transpose_x(xat_s, xad_s)
        relayout(3, bwq_hbm, bwq_raw, bwq_s)
        cp_xb.wait()
        for s0 in range(NSLOT - 1):
            for cp in stage_copies(s0, s0):
                cp.start()
        cp_c.start()
        cp_bwo.start()
        transpose_x(xbt_s, xb_s)

        m0 = mem0_s[...].astype(F32)
        mem_init = jnp.concatenate([m0, m0[:, 384:448]], axis=1)

        def pair_body(i, mem):
            slot = lax.rem(i, NSLOT)
            for cp in stage_copies(i, slot):
                cp.wait()

            @pl.when(i + NSLOT - 1 < NPAIR)
            def _():
                nxt = i + NSLOT - 1
                for cp in stage_copies(nxt, lax.rem(nxt, NSLOT)):
                    cp.start()

            def relayout_piece(n):
                part, src = n % 2, (stage_k, stage_v)[n // 2]
                wrows = pl.ds(pl.multiple_of(S + (n // 2) * DC + i * WCH + part * 16, 16), 16)
                hm_s[:, wrows, :] = jnp.swapaxes(src[slot, part * 16:(part + 1) * 16], 0, 1)

            hq = i // 2
            qbase = lax.rem(i, 2) * (S // 2)

            def q_fill(n):
                def run():
                    rows = pl.ds(pl.multiple_of(qbase + sum(FILL[:n]), 16), FILL[n])
                    for piece in PIECES[n]:
                        relayout_piece(piece)
                    hm_s[hq, rows, :] = (_dot(xb_s[rows, 0:DM], bwq_s[hq]) * SCALE).astype(BF)
                return run

            lane = lax.broadcasted_iota(jnp.int32, (G, T), 1)
            r = lax.broadcasted_iota(jnp.int32, (G, H * L), 0)
            col = lax.broadcasted_iota(jnp.int32, (G, H * L), 1)
            kk = col - L * ((col * 1639) >> 16)
            keep_e = (r >= 32) | (kk >= 32) | (kk <= r)
            kpos = jnp.where(kk < 24, kk + 8, kk - 32)
            qpos = jnp.where(r < 24, r + 8, r - 32)
            q_any = ((r >= 24) & (r < 32)) | (r >= 40)
            keep_o = q_any | ((kk >= 24) & (kk < 32)) | (kpos <= qpos)

            base = pl.multiple_of(i * 64, 64)
            xs = xad_s[pl.ds(base, 64), :]
            xs32 = xs[32:64, :].astype(F32)

            def proj(lhs, w_s, j):
                return _dot(lhs, pltpu.bitcast(w_s[j], BF))

            def own(x):
                return jnp.concatenate([x[0:32, :], x[40:48, :]], axis=0)

            l1 = jnp.concatenate(
                [xs[0:32, :], jnp.concatenate([xs32[0:8, :], mem], axis=0).astype(BF)], axis=0)
            l1p = l1[:, 0:DM]
            k1 = [proj(l1p, wck_s, j) for j in range(H // 2)]
            v1 = []

            def v1_fn(j):
                v1.append(proj(l1p, wcv_s, j))
                return own(v1[j])

            o1 = _rec_attention(l1, [own(k) for k in k1], v1_fn, q_fill(0), q_fill(1), keep_e, lane)
            q_fill(2)()

            l2 = jnp.concatenate([xs32[8:32, :], o1[40:48, :]], axis=0).astype(BF)
            l2p = l2[:, 0:DM]
            k2 = [jnp.concatenate([proj(l2p, wck_s, j), k1[j][32:40, :]], axis=0)
                  for j in range(H // 2)]
            o2 = _rec_attention(
                jnp.concatenate([l2, l1[32:48, :]], axis=0), k2,
                lambda j: jnp.concatenate([proj(l2p, wcv_s, j), v1[j][32:40, :]], axis=0),
                q_fill(3), q_fill(4), keep_o, lane)
            q_fill(5)()

            res = jnp.concatenate([o1[0:32, :], o2[32:40, :], o2[0:24, :]], axis=0)
            out_s[pl.ds(base, 64), 0:512] = res.astype(BF)
            return o2[24:32, :]

        lax.fori_loop(0, NPAIR, pair_body, mem_init)

    pl.run_scoped(
        phase_a,
        pltpu.VMEM((DM, S), BF), pltpu.VMEM((DM, S), BF), pltpu.VMEM((MEM, DM), BF),
        pltpu.VMEM((DM, H, DH), BF), pltpu.VMEM((DM, H, DH), BF), pltpu.VMEM((DM, H, DH), BF),
        pltpu.VMEM((DM, H, DH), BF),
        pltpu.VMEM((H, DM, DH), BF),
        pltpu.VMEM((H, DM, DH), BF), pltpu.VMEM((H, DM, DH), BF),
        pltpu.VMEM((H, DM, DH), BF),
        pltpu.VMEM((H // 2, DM // 2, PAIR), jnp.uint32),
        pltpu.VMEM((H // 2, DM // 2, PAIR), jnp.uint32),
        pltpu.VMEM((S, 512), BF), pltpu.VMEM((S, 512), BF),
    )

    def phase_b(k_s, v_s, o_s):
        cp_c.wait()
        cp_bwo.wait()

        def head(h, carry):
            k_s[...] = _dot(c_s[...], hm_s[h, S:S + DC, :]).astype(BF)
            v_s[...] = _dot(c_s[...], hm_s[h, S + DC:S + 2 * DC, :]).astype(BF)
            row = lax.broadcasted_iota(jnp.int32, (T, T), 0)
            col = lax.broadcasted_iota(jnp.int32, (T, T), 1)
            tri = row >= col

            def qk(r0):
                q = hm_s[h, r0:r0 + BQ, :]
                return _b_qk(q, k_s, r0, tri)

            starts = list(reversed(range(0, S, BQ)))
            scores = qk(starts[0])
            for n, r0 in enumerate(starts):
                nxt = qk(starts[n + 1]) if n + 1 < len(starts) else None
                o_s[h, r0:r0 + BQ, :] = _b_pv(scores, v_s, h < 0).astype(BF)
                scores = nxt
            return carry
        lax.fori_loop(0, H, head, 0)

        def out_copy(t):
            rows = pl.ds(pl.multiple_of(t * BO, BO), BO)
            return pltpu.make_async_copy(out_s.at[rows], out_hbm.at[rows], out_sems.at[t])

        def oproj(t, carry):
            rows = pl.ds(pl.multiple_of(t * BO, BO), BO)
            ctx = jnp.concatenate([o_s[h, rows, :] for h in range(H)], axis=1)
            wo = jnp.concatenate([bwo_s[h] for h in range(H)], axis=1)
            bt = _dot_nt(wo, ctx)
            b = jnp.concatenate([jnp.zeros((64, BO), F32), bt], axis=0).T.astype(BF)
            lo = lax.broadcasted_iota(jnp.int32, (BO, T), 1) < 64
            out_s[rows, 384:512] = jnp.where(lo, out_s[rows, 384:512], b[:, 0:T])
            out_s[rows, 512:896] = b[:, T:]
            out_copy(t).start()
            return carry
        lax.fori_loop(0, S // BO, oproj, 0, unroll=2)
        for t in range(S // BO):
            out_copy(t).wait()

    pl.run_scoped(
        phase_b,
        pltpu.VMEM((S, DH), BF), pltpu.VMEM((S, DH), BF),
        pltpu.VMEM((H, S, DH), BF),
    )


@jax.jit
def pallas_concat_heads__memory_aug_recurrent_mem_tr__compressed_kv_cla__prompt_kernel(
    A_x: jax.Array,
    A_mem0: jax.Array,
    A_Wq: jax.Array,
    A_Wk: jax.Array,
    A_Wv: jax.Array,
    A_Wo: jax.Array,
    A_seg_len: jax.Array,
    B_x: jax.Array,
    B_c_kv: jax.Array,
    B_w_q: jax.Array,
    B_w_uk: jax.Array,
    B_w_uv: jax.Array,
    B_w_o: jax.Array,
):
    del A_seg_len
    assert A_x.shape == (1, S, DM) and A_mem0.shape == (1, MEM, DM)
    assert A_Wq.shape == (DM, H, DH) and A_Wo.shape == (H, DH, DM)
    assert B_x.shape == (1, S, DM) and B_c_kv.shape == (1, S, DC)
    assert B_w_uk.shape == (DC, H, DH) and B_w_o.shape == (H, DH, DM)

    any_spec = pl.BlockSpec(memory_space=pl.ANY)
    out = pl.pallas_call(
        _kernel,
        out_shape=jax.ShapeDtypeStruct((S, 2 * DM), BF),
        in_specs=[any_spec] * 12,
        out_specs=any_spec,
        scratch_shapes=[
            pltpu.VMEM((S, DC), BF),
            pltpu.VMEM((H, S + 2 * DC, DH), BF),
            pltpu.VMEM((H, DM, DH), BF),
            pltpu.VMEM((NSLOT, WCH, H, DH), BF),
            pltpu.VMEM((NSLOT, WCH, H, DH), BF),
            pltpu.VMEM((S, 2 * DM), BF),
            pltpu.SemaphoreType.DMA((5,)),
            pltpu.SemaphoreType.DMA((5, 8)),
            pltpu.SemaphoreType.DMA((2, NSLOT)),
            pltpu.SemaphoreType.DMA((S // BO,)),
        ],
        compiler_params=pltpu.CompilerParams(vmem_limit_bytes=120 * 1024 * 1024),
    )(jnp.swapaxes(A_x, 1, 2).reshape(DM, S), A_mem0.reshape(MEM, DM), A_Wq, A_Wk, A_Wv,
      jnp.swapaxes(A_Wo, 1, 2),
      jnp.swapaxes(B_x, 1, 2).reshape(DM, S), B_c_kv.reshape(S, DC), B_w_q, B_w_uk, B_w_uv,
      jnp.swapaxes(B_w_o, 1, 2))
    return out.reshape(1, S, 2 * DM)
```

```python
import jax
import jax.numpy as jnp
from jax import lax
import jax.experimental.pallas as pl
import jax.experimental.pallas.tpu as pltpu

BF = jnp.bfloat16
F32 = jnp.float32

S = 2048
DM = 448
H = 16
DH = 256
MEM = 8
SEG = 32
DC = 1024
LOG2E = 1.4426950408889634
SCALE = DH ** -0.5 * LOG2E
NEG = -1000000000.0 * LOG2E
T = 128
L = MEM + SEG
G = 48
PAIR = 2 * DM
BQ = 512
KC = 256
BO = 128
UOP = 4
NPAIR = S // (2 * SEG)
WCH = DC // NPAIR
NSLOT = 3
RCH = 64
LAG = 2
FILL = (144, 64, 192, 144, 64, 192)
HALF = (0, 1, 1, 0, 1, 1)
PIECES = ((0,), (), (1,), (2,), (), (3,))
R0 = S - 4 * (FILL[0] + FILL[3])
assert (FILL[1] + FILL[2] + FILL[4] + FILL[5]) * 4 == S
NCH = DM // RCH
HD = DM // 2
XO = (H // 2) * HD
XP = 512
NX0 = -(-R0 // XP)
CPLAN = ((0, 0, 3), 's', 't', (1, 0, 1), 's', (1, 1, 3))
DPLAN = ((0, 0, 2), 's', (0, 2, 3), 's', 't', (1, 0, 1), 's', (1, 1, 3))


def _dot(a, b):
    return jnp.dot(a, b, preferred_element_type=F32)


def _dot_nt(a, b):
    return lax.dot_general(a, b, (((1,), (1,)), ((), ())), preferred_element_type=F32)


def _seg_reduce_bcast(x, lane, fill, combine, reduce_fn):
    nt = H * L // T
    tiles = [x[:, t * T:(t + 1) * T] for t in range(nt)]
    outs = [None] * nt
    for g in range(H):
        parts = []
        for t in range(nt):
            lo = max(L * g - T * t, 0)
            hi = min(L * g + L - T * t, T)
            if lo < hi:
                parts.append((t, (lane >= lo) & (lane < hi)))
        acc = None
        for t, msk in parts:
            sel = jnp.where(msk, tiles[t], fill)
            acc = sel if acc is None else combine(acc, sel)
        red = reduce_fn(acc, axis=1, keepdims=True)
        for t, msk in parts:
            if outs[t] is None:
                outs[t] = jnp.broadcast_to(red, tiles[t].shape)
            else:
                outs[t] = jnp.where(msk, red, outs[t])
    return jnp.concatenate(outs, axis=1)


def _seg_softmax(s, keep, lane):
    s = jnp.where(keep, s, NEG)
    m = _seg_reduce_bcast(s, lane, -jnp.inf, jnp.maximum, jnp.max)
    p = jnp.exp2(s - m)
    l = _seg_reduce_bcast(p, lane, 0.0, jnp.add, jnp.sum)
    return (p * (1.0 / l)).astype(BF)


def _stack(slabs):
    lo = lax.broadcasted_iota(jnp.int32, (L, T), 1) < 64
    blocks = []
    for r in slabs:
        tail = r[:, 768:896]
        blocks.append(jnp.concatenate([r[:, 0:384], jnp.where(lo, tail, 0.0)], axis=1))
        blocks.append(jnp.concatenate([r[:, 384:768], jnp.where(lo, 0.0, tail)], axis=1))
    return jnp.concatenate(blocks, axis=0).astype(BF)


def _rec_attention(qrows, kslabs, vslab_fn, filler0, filler, keep, lane):
    filler0()
    s = _dot_nt(qrows, _stack(kslabs))
    vslabs = [vslab_fn(j) for j in range(H // 2)]
    filler()
    p = _seg_softmax(s, keep, lane)
    o = _dot(p, _stack(vslabs))
    t = o[:, 384:512]
    return jnp.concatenate([o[:, 0:384], t + pltpu.roll(t, 64, 1)], axis=1)


def _b_qk(q, k_s, r0, tri):
    nt = BQ // T

    def mask_top(blk):
        top = jnp.where(tri, blk[0:T, :], NEG)
        return jnp.concatenate([top, blk[T:, :]], axis=0) if blk.shape[0] > T else top

    s_main = _dot_nt(q, k_s[0:r0 + T, :])
    chunks = [(0, c0, s_main[:, c0:min(c0 + KC, r0)]) for c0 in range(0, r0, KC)]
    chunks.append((0, r0, mask_top(s_main[:, r0:r0 + T])))
    for t in range(1, nt):
        chunks.append((t * T, r0 + t * T, mask_top(
            _dot_nt(q[t * T:, :], k_s[r0 + t * T:r0 + (t + 1) * T, :]))))
    ms = []
    for u in range(nt):
        row = [c[u * T - f:(u + 1) * T - f, :] for f, _, c in chunks if f <= u * T]
        row = jnp.concatenate(row, axis=1) if len(row) > 1 else row[0]
        ms.append(jnp.max(row, axis=1, keepdims=True))
    return chunks, jnp.concatenate(ms, axis=0)


def _b_pv(scores, v_s, never):
    chunks, m = scores
    nt = BQ // T
    o = [None] * nt
    l = None
    ocs = []
    mb = jnp.broadcast_to(m, (BQ, T))
    for f, k0, c in chunks:
        mc = mb[f:, :]
        if len(ocs) >= LAG:
            pf, prev = ocs[-LAG]
            mc = jnp.where(never, prev[f - pf:, 0:T], mc)
        ps = [jnp.exp2(c[:, j * T:(j + 1) * T] - mc) for j in range(c.shape[1] // T)]
        p = jnp.concatenate(ps, axis=1) if len(ps) > 1 else ps[0]
        oc = _dot(p.astype(BF), v_s[k0:k0 + c.shape[1], :])
        ocs.append((f, oc))
        lc = ps[0]
        for x in ps[1:]:
            lc = lc + x
        if l is None:
            l = lc
        elif f == 0:
            l = l + lc
        else:
            l = jnp.concatenate([l[0:f, :], l[f:, :] + lc], axis=0)
        for u in range(f // T, nt):
            rows = slice(u * T - f, (u + 1) * T - f)
            o[u] = oc[rows] if o[u] is None else o[u] + oc[rows]
    return jnp.concatenate(o, axis=0) * (1.0 / jnp.sum(l, axis=1, keepdims=True))


def _kernel(xa_hbm, mem0_hbm, wq_hbm, wk_hbm, wv_hbm, wo_hbm,
            xb_hbm, c_hbm, bwq_hbm, bwk_hbm, bwv_hbm, bwo_hbm,
            out_hbm,
            c_s, hm_s, bwo_s, stage_k, stage_v, out_s,
            sems, w_sems, stage_sems, out_sems):

    def stage_copies(chunk, slot):
        rows = pl.ds(chunk * WCH, WCH)
        return (pltpu.make_async_copy(bwk_hbm.at[rows], stage_k.at[slot], stage_sems.at[0, slot]),
                pltpu.make_async_copy(bwv_hbm.at[rows], stage_v.at[slot], stage_sems.at[1, slot]))

    cp_c = pltpu.make_async_copy(c_hbm, c_s, sems.at[2])
    cp_bwo = pltpu.make_async_copy(bwo_hbm, bwo_s, sems.at[3])

    def phase_a(xt_s, mem0_s, raw, wo_s, bwq_s, wx_s, wy_s):
        srcs = (bwq_hbm, wq_hbm, wk_hbm, wv_hbm)

        def row_chunk(k, t):
            return pltpu.make_async_copy(
                srcs[k].at[pl.ds(t * RCH, RCH)], raw.at[pl.ds((k * NCH + t) * RCH, RCH)],
                w_sems.at[k, t])

        def bwq_chunk(c, t):
            rows, lanes = pl.ds(t * RCH, RCH), pl.ds(c * T, T)
            return pltpu.make_async_copy(
                bwq_hbm.at[rows, :, lanes], raw.at[rows, :, lanes], w_sems.at[6 * c, t])

        def wo_chunk(j):
            heads = pl.ds(2 * j, 2)
            return pltpu.make_async_copy(wo_hbm.at[heads], wo_s.at[heads], w_sems.at[4, j])

        def x_piece(k, src_k=None):
            sk = k if src_k is None else src_k
            src = (xb_hbm, xa_hbm)[sk // 4].at[:, pl.ds((sk % 4) * XP, XP)]
            return pltpu.make_async_copy(
                src, xt_s.at[:, pl.ds(pl.multiple_of(k * XP, XP), XP)], w_sems.at[5, k])

        cp_m0 = pltpu.make_async_copy(mem0_hbm, mem0_s, sems.at[1])
        early = [x_piece(k) for k in range(NX0)]
        early += [bwq_chunk(0, t) for t in range(NCH)]
        for t in range(NCH):
            early += [row_chunk(1, t), row_chunk(2, t)]
        early += [row_chunk(3, t) for t in range(NCH)]
        for j in range(H // 2):
            early += [wo_chunk(j)] + ([x_piece(j)] if j >= NX0 else [])
            early += [bwq_chunk(1, j - 1)] if j > 0 else []
        early += [cp_m0]
        for cp in early:
            cp.start()

        def u32(w):
            return pltpu.bitcast(w.astype(BF), jnp.uint32)

        def fold_pair(dst, p, lhs, rhs, scale, plan, sides):
            def put(lanes, val):
                val = val if scale is None else val * scale
                dst[pl.ds(pl.multiple_of(p * HD, 8), HD), lanes] = u32(val)

            zero = jnp.zeros((64, DH), BF)
            tails = jnp.concatenate(
                [jnp.concatenate([rhs[0][384:448, :], zero], axis=1),
                 jnp.concatenate([zero, rhs[1][384:448, :]], axis=1)], axis=0)
            sides = iter(sides)
            for step in plan:
                if step == 't':
                    put(slice(768, 896), _dot_nt(jnp.concatenate(lhs, axis=1), tails))
                elif step == 's':
                    next(sides)()
                else:
                    n, c0, c1 = step
                    put(slice(384 * n + c0 * T, 384 * n + c1 * T),
                        _dot_nt(lhs[n], rhs[n][c0 * T:c1 * T, :]))

        def transpose_x(n):
            cols = pl.ds(pl.multiple_of(n * 256, 256), 256)
            x = xt_s[:, cols]
            rows = pl.ds(pl.multiple_of(XO + n * 128, 128), 128)
            wy_s[rows, 0:512] = u32(jnp.concatenate([x, x[384:448, :]], axis=0).T)

        def x_rows(start, n, width):
            rows = pl.ds(pl.multiple_of(XO + start // 2, 8), n // 2)
            return pltpu.bitcast(wy_s[rows, 0:width], BF)

        raw[4 * DM:4 * DM + RCH] = jnp.zeros((RCH, H, DH), BF)

        def x0_body(n, carry):
            @pl.when(lax.rem(n, 2) == 0)
            def _():
                x_piece(n // 2, 0).wait()
            transpose_x(n)
            return carry
        lax.fori_loop(0, 2 * NX0, x0_body, 0)

        def pair_up(w):
            return [jnp.concatenate([w[2 * m], w[2 * m + 1]], axis=1) for m in range(H // 2)]

        def bwq_body(t, carry):
            bwq_chunk(0, t).wait()
            rows = pl.ds(pl.multiple_of(t * RCH, RCH), RCH)
            for m, w in enumerate(pair_up(jnp.swapaxes(raw[rows, :, 0:T], 0, 1))):
                bwq_s[m, rows, :] = w
            return carry
        lax.fori_loop(0, NCH, bwq_body, 0)

        def chunk_rows(k, p, n, size, lanes=slice(None)):
            g = jnp.where(p > 0, k * NCH + p - 1, 4 * NCH)
            return raw[pl.ds(pl.multiple_of(g * RCH + n * size, size), size), :, lanes]

        def q_proj(m, half, start, n):
            w = bwq_s[m] if half == 0 else pltpu.bitcast(wy_s[wv_slot(m, 2, 0, HD)], BF)
            q = (_dot(x_rows(start, n, DM), w) * SCALE).astype(BF)
            rows = pl.ds(pl.multiple_of(start, 16), n)
            for odd in range(2):
                hm_s[2 * m + odd, rows, half * T:(half + 1) * T] = q[:, odd * T:(odd + 1) * T]

        def wv_slot(pair, odd, start, n):
            return (pl.ds(pl.multiple_of(XO + pair * HD + start, 8), n),
                    slice(odd * DH, (odd + 1) * DH))

        def pair_loop(unroll, waits, work):
            def body(i, carry):
                later = []
                for u in range(unroll):
                    p = i * unroll + u
                    for first, cp in waits(p, jnp.maximum(p - 1, 0)):
                        assert first <= unroll
                        if u >= first:
                            cp.wait()
                        else:
                            later.append(cp)

                @pl.when(i > 0)
                def _():
                    for cp in later:
                        cp.wait()

                for u in range(unroll):
                    p = i * unroll + u
                    work(p, jnp.maximum(p - 1, 0))
                return carry
            lax.fori_loop(0, H // 2 // unroll, body, 0)

        def q0_work(p, prev):
            def relayout(k):
                dst = pl.ds(pl.multiple_of(S + k * DM + prev * RCH, RCH), RCH)
                hm_s[:, dst, :] = jnp.swapaxes(chunk_rows(1 + k, p, 0, RCH), 0, 1)

            q_proj(p, 0, 0, R0 // 2)
            relayout(0)
            q_proj(p, 0, R0 // 2, R0 // 4)
            relayout(1)
            q_proj(p, 0, 3 * R0 // 4, R0 // 4)
        pair_loop(1, lambda p, prev: [(1, row_chunk(1, prev)), (1, row_chunk(2, prev))], q0_work)

        def ck_work(p, prev):
            def relayout(n):
                w = jnp.swapaxes(chunk_rows(3, p, n, RCH // 2), 0, 1)
                for h in range(H):
                    start = prev * (RCH // 2) + n * (RCH // 4)
                    wx_s[wv_slot(h // 2, h % 2, start, RCH // 4)] = u32(w[h])

            fold_pair(wx_s, p, [hm_s[2 * p + n, S + DM:S + 2 * DM, :] for n in range(2)],
                      [hm_s[2 * p + n, S:S + DM, :] for n in range(2)], SCALE,
                      CPLAN, [lambda: relayout(0), lambda: relayout(1)])
        pair_loop(2, lambda p, prev: [(1, row_chunk(3, prev))], ck_work)

        for s0 in range(NSLOT - 1):
            for cp in stage_copies(s0, s0):
                cp.start()

        def cv_work(p, prev):
            def relayout_bwq():
                w = jnp.swapaxes(chunk_rows(0, p, 0, RCH, slice(T, 2 * T)), 0, 1)
                for m, wm in enumerate(pair_up(w)):
                    wy_s[wv_slot(m, 2, prev * (RCH // 2), RCH // 2)] = u32(wm)

            sides = [relayout_bwq, lambda: transpose_x(2 * p), lambda: transpose_x(2 * p + 1)]
            fold_pair(wy_s, p, [pltpu.bitcast(wx_s[wv_slot(p, n, 0, HD)], BF) for n in range(2)],
                      [wo_s[2 * p + n] for n in range(2)], None,
                      DPLAN, sides)
        pair_loop(2, lambda p, prev: [(0, wo_chunk(p)), (NX0, x_piece(p, 0)),
                                       (1, bwq_chunk(1, prev))], cv_work)

        cp_c.start()
        cp_bwo.start()
        cp_m0.wait()

        m0 = mem0_s[...].astype(F32)
        mem_init = jnp.concatenate([m0, m0[:, 384:448]], axis=1)

        def pair_body(i, mem):
            slot = lax.rem(i, NSLOT)
            for cp in stage_copies(i, slot):
                cp.wait()

            @pl.when(i + NSLOT - 1 < NPAIR)
            def _():
                nxt = i + NSLOT - 1
                for cp in stage_copies(nxt, lax.rem(nxt, NSLOT)):
                    cp.start()

            def relayout_piece(n):
                part, src = n % 2, (stage_k, stage_v)[n // 2]
                wrows = pl.ds(pl.multiple_of(S + (n // 2) * DC + i * WCH + part * 16, 16), 16)
                hm_s[:, wrows, :] = jnp.swapaxes(src[slot, part * 16:(part + 1) * 16], 0, 1)

            def q_fill(n):
                def run():
                    same = [f for f, c in zip(FILL, HALF) if c == HALF[n]]
                    done = sum(f for f, c in zip(FILL[:n], HALF) if c == HALF[n])
                    start = (R0 if HALF[n] == 0 else 0) + lax.rem(i, 4) * sum(same) + done
                    for piece in PIECES[n]:
                        relayout_piece(piece)
                    q_proj(i // 4, HALF[n], start, FILL[n])
                return run

            lane = lax.broadcasted_iota(jnp.int32, (G, T), 1)
            r = lax.broadcasted_iota(jnp.int32, (G, H * L), 0)
            col = lax.broadcasted_iota(jnp.int32, (G, H * L), 1)
            kk = col - L * ((col * 1639) >> 16)
            keep_e = (r >= 32) | (kk >= 32) | (kk <= r)
            kpos = jnp.where(kk < 24, kk + 8, kk - 32)
            qpos = jnp.where(r < 24, r + 8, r - 32)
            q_any = ((r >= 24) & (r < 32)) | (r >= 40)
            keep_o = q_any | ((kk >= 24) & (kk < 32)) | (kpos <= qpos)

            base = pl.multiple_of(i * 64, 64)
            xs = x_rows(S + base, 64, 512)
            xs32 = xs[32:64, :].astype(F32)

            def proj(lhs, w_s, j):
                return _dot(lhs, pltpu.bitcast(w_s[j * HD:(j + 1) * HD, :], BF))

            def own(x):
                return jnp.concatenate([x[0:32, :], x[40:48, :]], axis=0)

            l1 = jnp.concatenate(
                [xs[0:32, :], jnp.concatenate([xs32[0:8, :], mem], axis=0).astype(BF)], axis=0)
            l1p = l1[:, 0:DM]
            k1 = [proj(l1p, wx_s, j) for j in range(H // 2)]
            v1 = []

            def v1_fn(j):
                v1.append(proj(l1p, wy_s, j))
                return own(v1[j])

            o1 = _rec_attention(l1, [own(k) for k in k1], v1_fn, q_fill(0), q_fill(1), keep_e, lane)
            q_fill(2)()

            l2 = jnp.concatenate([xs32[8:32, :], o1[40:48, :]], axis=0).astype(BF)
            l2p = l2[:, 0:DM]
            k2 = [jnp.concatenate([proj(l2p, wx_s, j), k1[j][32:40, :]], axis=0)
                  for j in range(H // 2)]
            o2 = _rec_attention(
                jnp.concatenate([l2, l1[32:48, :]], axis=0), k2,
                lambda j: jnp.concatenate([proj(l2p, wy_s, j), v1[j][32:40, :]], axis=0),
                q_fill(3), q_fill(4), keep_o, lane)
            q_fill(5)()

            res = jnp.concatenate([o1[0:32, :], o2[32:40, :], o2[0:24, :]], axis=0)
            out_s[pl.ds(base, 64), 0:512] = res.astype(BF)
            return o2[24:32, :]

        lax.fori_loop(0, NPAIR, pair_body, mem_init)

    pl.run_scoped(
        phase_a,
        pltpu.VMEM((DM, 2 * S), BF), pltpu.VMEM((MEM, DM), BF),
        pltpu.VMEM((4 * DM + RCH, H, DH), BF),
        pltpu.VMEM((H, DM, DH), BF), pltpu.VMEM((H // 2, DM, DH), BF),
        pltpu.VMEM((2 * XO, PAIR), jnp.uint32),
        pltpu.VMEM((XO + S, PAIR), jnp.uint32),
    )

    def phase_b(k_s, v_s, o_s, bt_s):
        cp_a = pltpu.make_async_copy(out_s.at[:, 0:384], out_hbm.at[:, 0:384], sems.at[0])
        cp_a.start()
        cp_c.wait()
        cp_bwo.wait()

        def head(h, carry):
            k_s[...] = _dot(c_s[...], hm_s[h, S:S + DC, :]).astype(BF)
            v_s[...] = _dot(c_s[...], hm_s[h, S + DC:S + 2 * DC, :]).astype(BF)
            row = lax.broadcasted_iota(jnp.int32, (T, T), 0)
            col = lax.broadcasted_iota(jnp.int32, (T, T), 1)
            tri = row >= col

            def qk(r0):
                q = hm_s[h, r0:r0 + BQ, :]
                return _b_qk(q, k_s, r0, tri)

            starts = list(reversed(range(0, S, BQ)))
            scores = qk(starts[0])
            for n, r0 in enumerate(starts):
                nxt = qk(starts[n + 1]) if n + 1 < len(starts) else None
                o_s[h, r0:r0 + BQ, :] = _b_pv(scores, v_s, h < 0).astype(BF)
                scores = nxt
            return carry
        lax.fori_loop(0, H, head, 0)

        def out_copy(t):
            rows = pl.ds(pl.multiple_of(t * BO, BO), BO)
            return pltpu.make_async_copy(
                out_s.at[rows, 384:2 * DM], out_hbm.at[rows, 384:2 * DM], out_sems.at[t])

        def project(t, after, never):
            rows = pl.ds(pl.multiple_of(t * BO, BO), BO)
            ctx = [o_s[h, rows, :] for h in range(H)]
            for n in range(2):
                ctx[8 + n] = jnp.where(never, after[:, n * DH:(n + 1) * DH], ctx[8 + n])
            wo = jnp.concatenate([bwo_s[h] for h in range(H)], axis=1)
            return _dot_nt(wo, jnp.concatenate(ctx, axis=1))

        def emit(t, bt):
            rows = pl.ds(pl.multiple_of(t * BO, BO), BO)
            b = jnp.concatenate([jnp.zeros((64, BO), F32), bt], axis=0).T.astype(BF)
            lo = lax.broadcasted_iota(jnp.int32, (BO, T), 1) < 64
            out_s[rows, 384:512] = jnp.where(lo, out_s[rows, 384:512], b[:, 0:T])
            out_s[rows, 512:896] = b[:, T:]
            return b

        bt_s[...] = jnp.zeros((DM, BO), F32)

        def oproj(i, carry):
            prev = jnp.maximum(UOP * i - 1, 0)
            b = emit(prev, bt_s[...])

            @pl.when(i > 0)
            def _():
                out_copy(prev).start()

            for u in range(UOP - 1):
                b = emit(UOP * i + u, project(UOP * i + u, b, i < 0))
                out_copy(UOP * i + u).start()
            bt_s[...] = project(UOP * i + UOP - 1, b, i < 0)
            return carry
        lax.fori_loop(0, S // BO // UOP, oproj, 0)
        emit(S // BO - 1, bt_s[...])
        out_copy(S // BO - 1).start()
        cp_a.wait()
        for t in range(S // BO):
            out_copy(t).wait()

    pl.run_scoped(
        phase_b,
        pltpu.VMEM((S, DH), BF), pltpu.VMEM((S, DH), BF),
        pltpu.VMEM((H, S, DH), BF), pltpu.VMEM((DM, BO), F32),
    )


@jax.jit
def pallas_concat_heads__memory_aug_recurrent_mem_tr__compressed_kv_cla__prompt_kernel(
    A_x: jax.Array,
    A_mem0: jax.Array,
    A_Wq: jax.Array,
    A_Wk: jax.Array,
    A_Wv: jax.Array,
    A_Wo: jax.Array,
    A_seg_len: jax.Array,
    B_x: jax.Array,
    B_c_kv: jax.Array,
    B_w_q: jax.Array,
    B_w_uk: jax.Array,
    B_w_uv: jax.Array,
    B_w_o: jax.Array,
):
    del A_seg_len
    assert A_x.shape == (1, S, DM) and A_mem0.shape == (1, MEM, DM)
    assert A_Wq.shape == (DM, H, DH) and A_Wo.shape == (H, DH, DM)
    assert B_x.shape == (1, S, DM) and B_c_kv.shape == (1, S, DC)
    assert B_w_uk.shape == (DC, H, DH) and B_w_o.shape == (H, DH, DM)

    any_spec = pl.BlockSpec(memory_space=pl.ANY)
    out = pl.pallas_call(
        _kernel,
        out_shape=jax.ShapeDtypeStruct((S, 2 * DM), BF),
        in_specs=[any_spec] * 12,
        out_specs=any_spec,
        scratch_shapes=[
            pltpu.VMEM((S, DC), BF),
            pltpu.VMEM((H, S + 2 * DC, DH), BF),
            pltpu.VMEM((H, DM, DH), BF),
            pltpu.VMEM((NSLOT, WCH, H, DH), BF),
            pltpu.VMEM((NSLOT, WCH, H, DH), BF),
            pltpu.VMEM((S, 2 * DM), BF),
            pltpu.SemaphoreType.DMA((4,)),
            pltpu.SemaphoreType.DMA((7, 8)),
            pltpu.SemaphoreType.DMA((2, NSLOT)),
            pltpu.SemaphoreType.DMA((S // BO,)),
        ],
        compiler_params=pltpu.CompilerParams(vmem_limit_bytes=120 * 1024 * 1024),
    )(jnp.swapaxes(A_x, 1, 2).reshape(DM, S), A_mem0.reshape(MEM, DM), A_Wq, A_Wk, A_Wv,
      jnp.swapaxes(A_Wo, 1, 2),
      jnp.swapaxes(B_x, 1, 2).reshape(DM, S), B_c_kv.reshape(S, DC), B_w_q, B_w_uk, B_w_uv,
      jnp.swapaxes(B_w_o, 1, 2))
    return out.reshape(1, S, 2 * DM)
```

```python
import jax
import jax.numpy as jnp
from jax import lax
import jax.experimental.pallas as pl
import jax.experimental.pallas.tpu as pltpu

BF = jnp.bfloat16
F32 = jnp.float32

S = 2048
DM = 448
H = 16
DH = 256
MEM = 8
SEG = 32
DC = 1024
LOG2E = 1.4426950408889634
SCALE = DH ** -0.5 * LOG2E
NEG = -1000000000.0 * LOG2E
T = 128
L = MEM + SEG
G = 48
PAIR = 2 * DM
BQ = 512
KC = 256
BO = 128
UOP = 2
UCH = 2
NPAIR = S // (2 * SEG)
WCH = DC // NPAIR
NSLOT = 2 * UCH
RCH = 64
LAG = 2
FILL = (144, 96, 176, 144, 96, 176, 144, 96, 176, 144, 96, 112)
HALF = (0, 1, 1, 0, 1, 1) * UCH
PIECES = ((0,), (), (1,), (2,), (), (3,))
R0 = S - 2 * sum(f for f, c in zip(FILL, HALF) if c == 0)
assert sum(f for f, c in zip(FILL, HALF) if c == 1) * 2 == S and UCH == 2
NCH = DM // RCH
HD = DM // 2
XO = (H // 2) * HD
XP = 512
NX0 = -(-R0 // XP)
CPLAN = ((0, 0, 3), 's', 't', (1, 0, 1), 's', (1, 1, 3))
DPLAN = ((0, 0, 2), 's', (0, 2, 3), 's', 't', (1, 0, 1), 's', (1, 1, 3))


def _dot(a, b):
    return jnp.dot(a, b, preferred_element_type=F32)


def _dot_nt(a, b):
    return lax.dot_general(a, b, (((1,), (1,)), ((), ())), preferred_element_type=F32)


def _seg_reduce_bcast(x, lane, fill, combine, reduce_fn):
    nt = H * L // T
    tiles = [x[:, t * T:(t + 1) * T] for t in range(nt)]
    outs = [None] * nt
    for g in range(H):
        parts = []
        for t in range(nt):
            lo = max(L * g - T * t, 0)
            hi = min(L * g + L - T * t, T)
            if lo < hi:
                parts.append((t, (lane >= lo) & (lane < hi)))
        acc = None
        for t, msk in parts:
            sel = jnp.where(msk, tiles[t], fill)
            acc = sel if acc is None else combine(acc, sel)
        red = reduce_fn(acc, axis=1, keepdims=True)
        for t, msk in parts:
            if outs[t] is None:
                outs[t] = jnp.broadcast_to(red, tiles[t].shape)
            else:
                outs[t] = jnp.where(msk, red, outs[t])
    return jnp.concatenate(outs, axis=1)


def _seg_softmax(s, keep, lane):
    s = jnp.where(keep, s, NEG)
    m = _seg_reduce_bcast(s, lane, -jnp.inf, jnp.maximum, jnp.max)
    p = jnp.exp2(s - m)
    l = _seg_reduce_bcast(p, lane, 0.0, jnp.add, jnp.sum)
    return (p * (1.0 / l)).astype(BF)


def _stack(slabs):
    lo = lax.broadcasted_iota(jnp.int32, (L, T), 1) < 64
    blocks = []
    for r in slabs:
        tail = r[:, 768:896]
        blocks.append(jnp.concatenate([r[:, 0:384], jnp.where(lo, tail, 0.0)], axis=1))
        blocks.append(jnp.concatenate([r[:, 384:768], jnp.where(lo, 0.0, tail)], axis=1))
    return jnp.concatenate(blocks, axis=0).astype(BF)


def _rec_attention(qrows, kslabs, vslab_fn, filler0, filler, keep, lane):
    filler0()
    s = _dot_nt(qrows, _stack(kslabs))
    vslabs = [vslab_fn(j) for j in range(H // 2)]
    filler()
    p = _seg_softmax(s, keep, lane)
    o = _dot(p, _stack(vslabs))
    t = o[:, 384:512]
    return jnp.concatenate([o[:, 0:384], t + pltpu.roll(t, 64, 1)], axis=1)


def _b_qk(q, k_s, r0, tri):
    nt = BQ // T

    def mask_top(blk):
        top = jnp.where(tri, blk[0:T, :], NEG)
        return jnp.concatenate([top, blk[T:, :]], axis=0) if blk.shape[0] > T else top

    s_main = _dot_nt(q, k_s[0:r0 + T, :])
    chunks = [(0, c0, s_main[:, c0:min(c0 + KC, r0)]) for c0 in range(0, r0, KC)]
    chunks.append((0, r0, mask_top(s_main[:, r0:r0 + T])))
    for t in range(1, nt):
        chunks.append((t * T, r0 + t * T, mask_top(
            _dot_nt(q[t * T:, :], k_s[r0 + t * T:r0 + (t + 1) * T, :]))))
    ms = []
    for u in range(nt):
        row = [c[u * T - f:(u + 1) * T - f, :] for f, _, c in chunks if f <= u * T]
        row = jnp.concatenate(row, axis=1) if len(row) > 1 else row[0]
        ms.append(jnp.max(row, axis=1, keepdims=True))
    return chunks, jnp.concatenate(ms, axis=0)


def _b_pv(scores, v_s, never):
    chunks, m = scores
    nt = BQ // T
    o = [None] * nt
    l = None
    ocs = []
    mb = jnp.broadcast_to(m, (BQ, T))
    for f, k0, c in chunks:
        mc = mb[f:, :]
        if len(ocs) >= LAG:
            pf, prev = ocs[-LAG]
            mc = jnp.where(never, prev[f - pf:, 0:T], mc)
        ps = [jnp.exp2(c[:, j * T:(j + 1) * T] - mc) for j in range(c.shape[1] // T)]
        p = jnp.concatenate(ps, axis=1) if len(ps) > 1 else ps[0]
        oc = _dot(p.astype(BF), v_s[k0:k0 + c.shape[1], :])
        ocs.append((f, oc))
        lc = ps[0]
        for x in ps[1:]:
            lc = lc + x
        if l is None:
            l = lc
        elif f == 0:
            l = l + lc
        else:
            l = jnp.concatenate([l[0:f, :], l[f:, :] + lc], axis=0)
        for u in range(f // T, nt):
            rows = slice(u * T - f, (u + 1) * T - f)
            o[u] = oc[rows] if o[u] is None else o[u] + oc[rows]
    return jnp.concatenate(o, axis=0) * (1.0 / jnp.sum(l, axis=1, keepdims=True))


def _kernel(xa_hbm, mem0_hbm, wq_hbm, wk_hbm, wv_hbm, wo_hbm,
            xb_hbm, c_hbm, bwq_hbm, bwk_hbm, bwv_hbm, bwo_hbm,
            out_hbm,
            c_s, hm_s, bwo_s, stage_k, stage_v, out_s,
            sems, w_sems, stage_sems, out_sems):

    def stage_copies(chunk, slot):
        rows = pl.ds(chunk * WCH, WCH)
        return (pltpu.make_async_copy(bwk_hbm.at[rows], stage_k.at[slot], stage_sems.at[0, slot]),
                pltpu.make_async_copy(bwv_hbm.at[rows], stage_v.at[slot], stage_sems.at[1, slot]))

    cp_c = pltpu.make_async_copy(c_hbm, c_s, sems.at[2])
    cp_bwo = pltpu.make_async_copy(bwo_hbm, bwo_s, sems.at[3])

    def phase_a(xt_s, mem0_s, raw, wo_s, bwq_s, wx_s, wy_s):
        srcs = (bwq_hbm, wq_hbm, wk_hbm, wv_hbm)

        def row_chunk(k, t):
            return pltpu.make_async_copy(
                srcs[k].at[pl.ds(t * RCH, RCH)], raw.at[pl.ds((k * NCH + t) * RCH, RCH)],
                w_sems.at[k, t])

        def bwq_chunk(c, t):
            rows, lanes = pl.ds(t * RCH, RCH), pl.ds(c * T, T)
            return pltpu.make_async_copy(
                bwq_hbm.at[rows, :, lanes], raw.at[rows, :, lanes], w_sems.at[6 * c, t])

        def wo_chunk(j):
            heads = pl.ds(2 * j, 2)
            return pltpu.make_async_copy(wo_hbm.at[heads], wo_s.at[heads], w_sems.at[4, j])

        def x_piece(k, src_k=None):
            sk = k if src_k is None else src_k
            src = (xb_hbm, xa_hbm)[sk // 4].at[:, pl.ds((sk % 4) * XP, XP)]
            return pltpu.make_async_copy(
                src, xt_s.at[:, pl.ds(pl.multiple_of(k * XP, XP), XP)], w_sems.at[5, k])

        cp_m0 = pltpu.make_async_copy(mem0_hbm, mem0_s, sems.at[1])
        early = [x_piece(k) for k in range(NX0)]
        early += [bwq_chunk(0, t) for t in range(NCH)]
        for t in range(NCH):
            early += [row_chunk(1, t), row_chunk(2, t)]
        early += [row_chunk(3, t) for t in range(NCH)]
        for j in range(H // 2):
            early += [wo_chunk(j)] + ([x_piece(j)] if j >= NX0 else [])
            early += [bwq_chunk(1, j - 1)] if j > 0 else []
        early += [cp_m0]
        for cp in early:
            cp.start()

        def u32(w):
            return pltpu.bitcast(w.astype(BF), jnp.uint32)

        def fold_pair(dst, p, lhs, rhs, scale, plan, sides):
            def put(lanes, val):
                val = val if scale is None else val * scale
                dst[pl.ds(pl.multiple_of(p * HD, 8), HD), lanes] = u32(val)

            zero = jnp.zeros((64, DH), BF)
            tails = jnp.concatenate(
                [jnp.concatenate([rhs[0][384:448, :], zero], axis=1),
                 jnp.concatenate([zero, rhs[1][384:448, :]], axis=1)], axis=0)
            sides = iter(sides)
            for step in plan:
                if step == 't':
                    put(slice(768, 896), _dot_nt(jnp.concatenate(lhs, axis=1), tails))
                elif step == 's':
                    next(sides)()
                else:
                    n, c0, c1 = step
                    put(slice(384 * n + c0 * T, 384 * n + c1 * T),
                        _dot_nt(lhs[n], rhs[n][c0 * T:c1 * T, :]))

        def transpose_x(n):
            cols = pl.ds(pl.multiple_of(n * 256, 256), 256)
            x = xt_s[:, cols]
            rows = pl.ds(pl.multiple_of(XO + n * 128, 128), 128)
            wy_s[rows, 0:512] = u32(jnp.concatenate([x, x[384:448, :]], axis=0).T)

        def x_rows(start, n, width):
            rows = pl.ds(pl.multiple_of(XO + start // 2, 8), n // 2)
            return pltpu.bitcast(wy_s[rows, 0:width], BF)

        def zero_body(n, carry):
            raw[pl.ds(4 * DM + n * 8, 8)] = jnp.zeros((8, H, DH), BF)
            return carry
        lax.fori_loop(0, RCH // 8, zero_body, 0)

        def x0_body(n, carry):
            @pl.when(lax.rem(n, 2) == 0)
            def _():
                x_piece(n // 2, 0).wait()
            transpose_x(n)
            return carry
        lax.fori_loop(0, 2 * NX0, x0_body, 0)

        def pair_up(w):
            return [jnp.concatenate([w[2 * m], w[2 * m + 1]], axis=1) for m in range(H // 2)]

        def bwq_body(t, carry):
            bwq_chunk(0, t).wait()
            rows = pl.ds(pl.multiple_of(t * RCH, RCH), RCH)
            for m, w in enumerate(pair_up(jnp.swapaxes(raw[rows, :, 0:T], 0, 1))):
                bwq_s[m, rows, :] = w
            return carry
        lax.fori_loop(0, NCH, bwq_body, 0)

        def chunk_rows(k, p, n, size, lanes=slice(None)):
            g = jnp.where(p > 0, k * NCH + p - 1, 4 * NCH)
            return raw[pl.ds(pl.multiple_of(g * RCH + n * size, size), size), :, lanes]

        def q_proj(m, half, start, n):
            w = bwq_s[m] if half == 0 else pltpu.bitcast(wy_s[wv_slot(m, 2, 0, HD)], BF)
            q = (_dot(x_rows(start, n, DM), w) * SCALE).astype(BF)
            rows = pl.ds(pl.multiple_of(start, 16), n)
            for odd in range(2):
                hm_s[2 * m + odd, rows, half * T:(half + 1) * T] = q[:, odd * T:(odd + 1) * T]

        def wv_slot(pair, odd, start, n):
            return (pl.ds(pl.multiple_of(XO + pair * HD + start, 8), n),
                    slice(odd * DH, (odd + 1) * DH))

        def pair_loop(unroll, waits, work):
            def body(i, carry):
                later = []
                for u in range(unroll):
                    p = i * unroll + u
                    for first, cp in waits(p, jnp.maximum(p - 1, 0)):
                        if u >= first:
                            cp.wait()
                        else:
                            assert first <= unroll
                            later.append(cp)

                @pl.when(i > 0)
                def _():
                    for cp in later:
                        cp.wait()

                for u in range(unroll):
                    p = i * unroll + u
                    work(p, jnp.maximum(p - 1, 0))
                return carry
            lax.fori_loop(0, H // 2 // unroll, body, 0)

        def q0_work(p, prev):
            def relayout(k):
                dst = pl.ds(pl.multiple_of(S + k * DM + prev * RCH, RCH), RCH)
                hm_s[:, dst, :] = jnp.swapaxes(chunk_rows(1 + k, p, 0, RCH), 0, 1)

            q_proj(p, 0, 0, R0 // 2)
            relayout(0)
            q_proj(p, 0, R0 // 2, R0 // 4)
            relayout(1)
            q_proj(p, 0, 3 * R0 // 4, R0 // 4)
        pair_loop(1, lambda p, prev: [(1, row_chunk(1, prev)), (1, row_chunk(2, prev))], q0_work)

        def ck_work(p, prev):
            def relayout(n):
                w = jnp.swapaxes(chunk_rows(3, p, n, RCH // 2), 0, 1)
                for h in range(H):
                    start = prev * (RCH // 2) + n * (RCH // 4)
                    wx_s[wv_slot(h // 2, h % 2, start, RCH // 4)] = u32(w[h])

            fold_pair(wx_s, p, [hm_s[2 * p + n, S + DM:S + 2 * DM, :] for n in range(2)],
                      [hm_s[2 * p + n, S:S + DM, :] for n in range(2)], SCALE,
                      CPLAN, [lambda: relayout(0), lambda: relayout(1)])
        pair_loop(1, lambda p, prev: [(1, row_chunk(3, prev))], ck_work)

        for s0 in range(UCH):
            for cp in stage_copies(s0, s0):
                cp.start()

        def cv_work(p, prev):
            def relayout_bwq():
                w = jnp.swapaxes(chunk_rows(0, p, 0, RCH, slice(T, 2 * T)), 0, 1)
                for m, wm in enumerate(pair_up(w)):
                    wy_s[wv_slot(m, 2, prev * (RCH // 2), RCH // 2)] = u32(wm)

            sides = [relayout_bwq, lambda: transpose_x(2 * p), lambda: transpose_x(2 * p + 1)]
            fold_pair(wy_s, p, [pltpu.bitcast(wx_s[wv_slot(p, n, 0, HD)], BF) for n in range(2)],
                      [wo_s[2 * p + n] for n in range(2)], None,
                      DPLAN, sides)
        pair_loop(2, lambda p, prev: [(0, wo_chunk(p)), (NX0, x_piece(p, 0)),
                                       (1, bwq_chunk(1, prev))], cv_work)

        cp_c.start()
        cp_bwo.start()
        cp_m0.wait()

        m0 = mem0_s[...].astype(F32)
        mem_init = jnp.concatenate([m0, m0[:, 384:448]], axis=1)

        def chain_body(b, mem):
            for u in range(UCH):
                i = b * UCH + u
                for cp in stage_copies(i, lax.rem(i, NSLOT)):
                    cp.wait()

            @pl.when(b + 1 < NPAIR // UCH)
            def _():
                for u in range(UCH):
                    nxt = (b + 1) * UCH + u
                    for cp in stage_copies(nxt, lax.rem(nxt, NSLOT)):
                        cp.start()

            for u in range(UCH):
                mem = pair_body(b, u, mem)
            return mem

        def pair_body(b, u, mem):
            i = b * UCH + u
            slot = lax.rem(i, NSLOT)

            def relayout_piece(n):
                part, src = n % 2, (stage_k, stage_v)[n // 2]
                wrows = pl.ds(pl.multiple_of(S + (n // 2) * DC + i * WCH + part * 16, 16), 16)
                hm_s[:, wrows, :] = jnp.swapaxes(src[slot, part * 16:(part + 1) * 16], 0, 1)

            def q_fill(k):
                def run():
                    n = 6 * u + k
                    same = [f for f, c in zip(FILL, HALF) if c == HALF[n]]
                    done = sum(f for f, c in zip(FILL[:n], HALF) if c == HALF[n])
                    start = (R0 if HALF[n] == 0 else 0) + lax.rem(b, 2) * sum(same) + done
                    for piece in PIECES[k]:
                        relayout_piece(piece)
                    q_proj(b // 2, HALF[n], start, FILL[n])
                return run

            lane = lax.broadcasted_iota(jnp.int32, (G, T), 1)
            r = lax.broadcasted_iota(jnp.int32, (G, H * L), 0)
            col = lax.broadcasted_iota(jnp.int32, (G, H * L), 1)
            kk = col - L * ((col * 1639) >> 16)
            keep_e = (r >= 32) | (kk >= 32) | (kk <= r)
            kpos = jnp.where(kk < 24, kk + 8, kk - 32)
            qpos = jnp.where(r < 24, r + 8, r - 32)
            q_any = ((r >= 24) & (r < 32)) | (r >= 40)
            keep_o = q_any | ((kk >= 24) & (kk < 32)) | (kpos <= qpos)

            base = pl.multiple_of(i * 64, 64)
            xs = x_rows(S + base, 64, 512)
            xs32 = xs[32:64, :].astype(F32)

            def proj(lhs, w_s, j):
                return _dot(lhs, pltpu.bitcast(w_s[j * HD:(j + 1) * HD, :], BF))

            def own(x):
                return jnp.concatenate([x[0:32, :], x[40:48, :]], axis=0)

            l1 = jnp.concatenate(
                [xs[0:32, :], jnp.concatenate([xs32[0:8, :], mem], axis=0).astype(BF)], axis=0)
            l1p = l1[:, 0:DM]
            k1 = [proj(l1p, wx_s, j) for j in range(H // 2)]
            v1 = []

            def v1_fn(j):
                v1.append(proj(l1p, wy_s, j))
                return own(v1[j])

            o1 = _rec_attention(l1, [own(k) for k in k1], v1_fn, q_fill(0), q_fill(1), keep_e, lane)
            q_fill(2)()

            l2 = jnp.concatenate([xs32[8:32, :], o1[40:48, :]], axis=0).astype(BF)
            l2p = l2[:, 0:DM]
            k2 = [jnp.concatenate([proj(l2p, wx_s, j), k1[j][32:40, :]], axis=0)
                  for j in range(H // 2)]
            o2 = _rec_attention(
                jnp.concatenate([l2, l1[32:48, :]], axis=0), k2,
                lambda j: jnp.concatenate([proj(l2p, wy_s, j), v1[j][32:40, :]], axis=0),
                q_fill(3), q_fill(4), keep_o, lane)
            q_fill(5)()

            res = jnp.concatenate([o1[0:32, :], o2[32:40, :], o2[0:24, :]], axis=0)
            out_s[pl.ds(base, 64), 0:512] = res.astype(BF)
            return o2[24:32, :]

        lax.fori_loop(0, NPAIR // UCH, chain_body, mem_init)

    pl.run_scoped(
        phase_a,
        pltpu.VMEM((DM, 2 * S), BF), pltpu.VMEM((MEM, DM), BF),
        pltpu.VMEM((4 * DM + RCH, H, DH), BF),
        pltpu.VMEM((H, DM, DH), BF), pltpu.VMEM((H // 2, DM, DH), BF),
        pltpu.VMEM((2 * XO, PAIR), jnp.uint32),
        pltpu.VMEM((XO + S, PAIR), jnp.uint32),
    )

    def phase_b(k_s, v_s, o_s, bt_s):
        cp_a = pltpu.make_async_copy(out_s.at[:, 0:384], out_hbm.at[:, 0:384], sems.at[0])
        cp_a.start()
        cp_c.wait()
        cp_bwo.wait()

        def head(h, carry):
            k_s[...] = _dot(c_s[...], hm_s[h, S:S + DC, :]).astype(BF)
            v_s[...] = _dot(c_s[...], hm_s[h, S + DC:S + 2 * DC, :]).astype(BF)
            row = lax.broadcasted_iota(jnp.int32, (T, T), 0)
            col = lax.broadcasted_iota(jnp.int32, (T, T), 1)
            tri = row >= col

            def qk(r0):
                q = hm_s[h, r0:r0 + BQ, :]
                return _b_qk(q, k_s, r0, tri)

            starts = list(reversed(range(0, S, BQ)))
            scores = qk(starts[0])
            for n, r0 in enumerate(starts):
                nxt = qk(starts[n + 1]) if n + 1 < len(starts) else None
                o_s[h, r0:r0 + BQ, :] = _b_pv(scores, v_s, h < 0).astype(BF)
                scores = nxt
            return carry
        lax.fori_loop(0, H, head, 0)

        def out_copy(t):
            rows = pl.ds(pl.multiple_of(t * BO, BO), BO)
            return pltpu.make_async_copy(
                out_s.at[rows, 384:2 * DM], out_hbm.at[rows, 384:2 * DM], out_sems.at[t])

        def project(t, after, never):
            rows = pl.ds(pl.multiple_of(t * BO, BO), BO)
            ctx = [o_s[h, rows, :] for h in range(H)]
            for n in range(2):
                ctx[8 + n] = jnp.where(never, after[:, n * DH:(n + 1) * DH], ctx[8 + n])
            wo = jnp.concatenate([bwo_s[h] for h in range(H)], axis=1)
            return _dot_nt(wo, jnp.concatenate(ctx, axis=1))

        def emit(t, bt):
            rows = pl.ds(pl.multiple_of(t * BO, BO), BO)
            b = jnp.concatenate([jnp.zeros((64, BO), F32), bt], axis=0).T.astype(BF)
            lo = lax.broadcasted_iota(jnp.int32, (BO, T), 1) < 64
            out_s[rows, 384:512] = jnp.where(lo, out_s[rows, 384:512], b[:, 0:T])
            out_s[rows, 512:896] = b[:, T:]
            return b

        bt_s[...] = jnp.zeros((DM, BO), F32)

        def oproj(i, carry):
            prev = jnp.maximum(UOP * i - 1, 0)
            b = emit(prev, bt_s[...])

            @pl.when(i > 0)
            def _():
                out_copy(prev).start()

            for u in range(UOP - 1):
                b = emit(UOP * i + u, project(UOP * i + u, b, i < 0))
                out_copy(UOP * i + u).start()
            bt_s[...] = project(UOP * i + UOP - 1, b, i < 0)
            return carry
        lax.fori_loop(0, S // BO // UOP, oproj, 0)
        emit(S // BO - 1, bt_s[...])
        out_copy(S // BO - 1).start()
        cp_a.wait()
        for t in range(S // BO):
            out_copy(t).wait()

    pl.run_scoped(
        phase_b,
        pltpu.VMEM((S, DH), BF), pltpu.VMEM((S, DH), BF),
        pltpu.VMEM((H, S, DH), BF), pltpu.VMEM((DM, BO), F32),
    )


@jax.jit
def pallas_concat_heads__memory_aug_recurrent_mem_tr__compressed_kv_cla__prompt_kernel(
    A_x: jax.Array,
    A_mem0: jax.Array,
    A_Wq: jax.Array,
    A_Wk: jax.Array,
    A_Wv: jax.Array,
    A_Wo: jax.Array,
    A_seg_len: jax.Array,
    B_x: jax.Array,
    B_c_kv: jax.Array,
    B_w_q: jax.Array,
    B_w_uk: jax.Array,
    B_w_uv: jax.Array,
    B_w_o: jax.Array,
):
    del A_seg_len
    assert A_x.shape == (1, S, DM) and A_mem0.shape == (1, MEM, DM)
    assert A_Wq.shape == (DM, H, DH) and A_Wo.shape == (H, DH, DM)
    assert B_x.shape == (1, S, DM) and B_c_kv.shape == (1, S, DC)
    assert B_w_uk.shape == (DC, H, DH) and B_w_o.shape == (H, DH, DM)

    any_spec = pl.BlockSpec(memory_space=pl.ANY)
    out = pl.pallas_call(
        _kernel,
        out_shape=jax.ShapeDtypeStruct((S, 2 * DM), BF),
        in_specs=[any_spec] * 12,
        out_specs=any_spec,
        scratch_shapes=[
            pltpu.VMEM((S, DC), BF),
            pltpu.VMEM((H, S + 2 * DC, DH), BF),
            pltpu.VMEM((H, DM, DH), BF),
            pltpu.VMEM((NSLOT, WCH, H, DH), BF),
            pltpu.VMEM((NSLOT, WCH, H, DH), BF),
            pltpu.VMEM((S, 2 * DM), BF),
            pltpu.SemaphoreType.DMA((4,)),
            pltpu.SemaphoreType.DMA((7, 8)),
            pltpu.SemaphoreType.DMA((2, NSLOT)),
            pltpu.SemaphoreType.DMA((S // BO,)),
        ],
        compiler_params=pltpu.CompilerParams(
            vmem_limit_bytes=120 * 1024 * 1024,
            disable_bounds_checks=True,
            disable_semaphore_checks=True),
    )(jnp.swapaxes(A_x, 1, 2).reshape(DM, S), A_mem0.reshape(MEM, DM), A_Wq, A_Wk, A_Wv,
      jnp.swapaxes(A_Wo, 1, 2),
      jnp.swapaxes(B_x, 1, 2).reshape(DM, S), B_c_kv.reshape(S, DC), B_w_q, B_w_uk, B_w_uv,
      jnp.swapaxes(B_w_o, 1, 2))
    return out.reshape(1, S, 2 * DM)
```

```python
import jax
import jax.numpy as jnp
from jax import lax
import jax.experimental.pallas as pl
import jax.experimental.pallas.tpu as pltpu

BF = jnp.bfloat16
F32 = jnp.float32

S = 2048
DM = 448
H = 16
DH = 256
MEM = 8
SEG = 32
DC = 1024
LOG2E = 1.4426950408889634
SCALE = DH ** -0.5 * LOG2E
NEG = -1000000000.0 * LOG2E
T = 128
L = MEM + SEG
G = 48
PAIR = 2 * DM
BQ = 512
KC = 256
BO = 128
UOP = 2
UCH = 2
NPAIR = S // (2 * SEG)
WCH = DC // NPAIR
NSLOT = 2 * UCH
RCH = 64
LAG = 2
FILL = (144, 96, 176, 144, 96, 176, 144, 96, 176, 144, 96, 112)
HALF = (0, 1, 1, 0, 1, 1) * UCH
PIECES = ((0,), (), (1,), (2,), (), (3,))
R0 = S - 2 * sum(f for f, c in zip(FILL, HALF) if c == 0)
assert sum(f for f, c in zip(FILL, HALF) if c == 1) * 2 == S and UCH == 2
NCH = DM // RCH
HD = DM // 2
XO = (H // 2) * HD
XP = 512
NX0 = -(-R0 // XP)
CPLAN = ((0, 0, 3), 's', 't', (1, 0, 1), 's', (1, 1, 3))
DPLAN = ((0, 0, 2), 's', (0, 2, 3), 's', 't', (1, 0, 1), 's', (1, 1, 3))


def _dot(a, b):
    return jnp.dot(a, b, preferred_element_type=F32)


def _dot_nt(a, b):
    return lax.dot_general(a, b, (((1,), (1,)), ((), ())), preferred_element_type=F32)


def _seg_reduce_bcast(x, lane, fill, combine, reduce_fn):
    nt = H * L // T
    tiles = [x[:, t * T:(t + 1) * T] for t in range(nt)]
    outs = [None] * nt
    for g in range(H):
        parts = []
        for t in range(nt):
            lo = max(L * g - T * t, 0)
            hi = min(L * g + L - T * t, T)
            if lo < hi:
                parts.append((t, (lane >= lo) & (lane < hi)))
        acc = None
        for t, msk in parts:
            sel = jnp.where(msk, tiles[t], fill)
            acc = sel if acc is None else combine(acc, sel)
        red = reduce_fn(acc, axis=1, keepdims=True)
        for t, msk in parts:
            if outs[t] is None:
                outs[t] = jnp.broadcast_to(red, tiles[t].shape)
            else:
                outs[t] = jnp.where(msk, red, outs[t])
    return jnp.concatenate(outs, axis=1)


def _seg_softmax(s, keep, lane):
    s = jnp.where(keep, s, NEG)
    m = _seg_reduce_bcast(s, lane, -jnp.inf, jnp.maximum, jnp.max)
    p = jnp.exp2(s - m)
    l = _seg_reduce_bcast(p, lane, 0.0, jnp.add, jnp.sum)
    return (p * (1.0 / l)).astype(BF)


def _stack(slabs):
    lo = lax.broadcasted_iota(jnp.int32, (L, T), 1) < 64
    blocks = []
    for r in slabs:
        tail = r[:, 768:896]
        blocks.append(jnp.concatenate([r[:, 0:384], jnp.where(lo, tail, 0.0)], axis=1))
        blocks.append(jnp.concatenate([r[:, 384:768], jnp.where(lo, 0.0, tail)], axis=1))
    return jnp.concatenate(blocks, axis=0).astype(BF)


def _rec_attention(qrows, kslabs, vslab_fn, filler0, filler, keep, lane):
    filler0()
    s = _dot_nt(qrows, _stack(kslabs))
    vslabs = [vslab_fn(j) for j in range(H // 2)]
    filler()
    p = _seg_softmax(s, keep, lane)
    o = _dot(p, _stack(vslabs))
    t = o[:, 384:512]
    return jnp.concatenate([o[:, 0:384], t + pltpu.roll(t, 64, 1)], axis=1)


def _b_qk(q, k_s, r0, tri):
    nt = BQ // T

    def mask_top(blk):
        top = jnp.where(tri, blk[0:T, :], NEG)
        return jnp.concatenate([top, blk[T:, :]], axis=0) if blk.shape[0] > T else top

    s_main = _dot_nt(q, k_s[0:r0 + T, :])
    chunks = [(0, c0, s_main[:, c0:min(c0 + KC, r0)]) for c0 in range(0, r0, KC)]
    chunks.append((0, r0, mask_top(s_main[:, r0:r0 + T])))
    for t in range(1, nt):
        chunks.append((t * T, r0 + t * T, mask_top(
            _dot_nt(q[t * T:, :], k_s[r0 + t * T:r0 + (t + 1) * T, :]))))
    ms = []
    for u in range(nt):
        row = [c[u * T - f:(u + 1) * T - f, :] for f, _, c in chunks if f <= u * T]
        row = jnp.concatenate(row, axis=1) if len(row) > 1 else row[0]
        ms.append(jnp.max(row, axis=1, keepdims=True))
    return chunks, jnp.concatenate(ms, axis=0)


def _b_pv(scores, v_s, never):
    chunks, m = scores
    nt = BQ // T
    o = [None] * nt
    l = None
    ocs = []
    mb = jnp.broadcast_to(m, (BQ, T))
    for f, k0, c in chunks:
        mc = mb[f:, :]
        if len(ocs) >= LAG:
            pf, prev = ocs[-LAG]
            mc = jnp.where(never, prev[f - pf:, 0:T], mc)
        ps = [jnp.exp2(c[:, j * T:(j + 1) * T] - mc) for j in range(c.shape[1] // T)]
        p = jnp.concatenate(ps, axis=1) if len(ps) > 1 else ps[0]
        oc = _dot(p.astype(BF), v_s[k0:k0 + c.shape[1], :])
        ocs.append((f, oc))
        lc = ps[0]
        for x in ps[1:]:
            lc = lc + x
        if l is None:
            l = lc
        elif f == 0:
            l = l + lc
        else:
            l = jnp.concatenate([l[0:f, :], l[f:, :] + lc], axis=0)
        for u in range(f // T, nt):
            rows = slice(u * T - f, (u + 1) * T - f)
            o[u] = oc[rows] if o[u] is None else o[u] + oc[rows]
    return jnp.concatenate(o, axis=0) * (1.0 / jnp.sum(l, axis=1, keepdims=True))


def _kernel(xa_hbm, mem0_hbm, wq_hbm, wk_hbm, wv_hbm, wo_hbm,
            xb_hbm, c_hbm, bwq_hbm, bwk_hbm, bwv_hbm, bwo_hbm,
            out_hbm,
            c_s, hm_s, bwo_s, stage_k, stage_v, out_s,
            sems, w_sems, stage_sems, out_sems):

    def stage_copies(chunk, slot):
        rows = pl.ds(chunk * WCH, WCH)
        return (pltpu.make_async_copy(bwk_hbm.at[rows], stage_k.at[slot], stage_sems.at[0, slot]),
                pltpu.make_async_copy(bwv_hbm.at[rows], stage_v.at[slot], stage_sems.at[1, slot]))

    cp_c = pltpu.make_async_copy(c_hbm, c_s, sems.at[2])
    cp_bwo = pltpu.make_async_copy(bwo_hbm, bwo_s, sems.at[3])

    def phase_a(xt_s, mem0_s, raw, wo_s, bwq_s, wx_s, wy_s):
        srcs = (bwq_hbm, wq_hbm, wk_hbm, wv_hbm)

        def row_chunk(k, t):
            return pltpu.make_async_copy(
                srcs[k].at[pl.ds(t * RCH, RCH)], raw.at[pl.ds((k * NCH + t) * RCH, RCH)],
                w_sems.at[k, t])

        def bwq_chunk(c, t):
            rows, lanes = pl.ds(t * RCH, RCH), pl.ds(c * T, T)
            return pltpu.make_async_copy(
                bwq_hbm.at[rows, :, lanes], raw.at[rows, :, lanes], w_sems.at[6 * c, t])

        def wo_chunk(j):
            heads = pl.ds(2 * j, 2)
            return pltpu.make_async_copy(wo_hbm.at[heads], wo_s.at[heads], w_sems.at[4, j])

        def x_piece(k, src_k=None):
            sk = k if src_k is None else src_k
            src = (xb_hbm, xa_hbm)[sk // 4].at[:, pl.ds((sk % 4) * XP, XP)]
            return pltpu.make_async_copy(
                src, xt_s.at[:, pl.ds(pl.multiple_of(k * XP, XP), XP)], w_sems.at[5, k])

        cp_m0 = pltpu.make_async_copy(mem0_hbm, mem0_s, sems.at[1])

        def start_each(copies):
            def body(t, carry):
                for cp in copies(t):
                    cp.start()
                return carry
            lax.fori_loop(0, NCH, body, 0)

        for k in range(NX0):
            x_piece(k).start()
        start_each(lambda t: [bwq_chunk(0, t)])
        start_each(lambda t: [row_chunk(1, t), row_chunk(2, t)])
        start_each(lambda t: [row_chunk(3, t)])
        for j in range(H // 2):
            wo_chunk(j).start()
            if j >= NX0:
                x_piece(j).start()
            if j > 0:
                bwq_chunk(1, j - 1).start()
        cp_m0.start()

        def u32(w):
            return pltpu.bitcast(w.astype(BF), jnp.uint32)

        def fold_pair(dst, p, lhs, rhs, scale, plan, sides):
            def put(lanes, val):
                val = val if scale is None else val * scale
                dst[pl.ds(pl.multiple_of(p * HD, 8), HD), lanes] = u32(val)

            zero = jnp.zeros((64, DH), BF)
            tails = jnp.concatenate(
                [jnp.concatenate([rhs[0][384:448, :], zero], axis=1),
                 jnp.concatenate([zero, rhs[1][384:448, :]], axis=1)], axis=0)
            sides = iter(sides)
            for step in plan:
                if step == 't':
                    put(slice(768, 896), _dot_nt(jnp.concatenate(lhs, axis=1), tails))
                elif step == 's':
                    next(sides)()
                else:
                    n, c0, c1 = step
                    put(slice(384 * n + c0 * T, 384 * n + c1 * T),
                        _dot_nt(lhs[n], rhs[n][c0 * T:c1 * T, :]))

        def transpose_x(n):
            cols = pl.ds(pl.multiple_of(n * 256, 256), 256)
            x = xt_s[:, cols]
            rows = pl.ds(pl.multiple_of(XO + n * 128, 128), 128)
            wy_s[rows, 0:512] = u32(jnp.concatenate([x, x[384:448, :]], axis=0).T)

        def x_rows(start, n, width):
            rows = pl.ds(pl.multiple_of(XO + start // 2, 8), n // 2)
            return pltpu.bitcast(wy_s[rows, 0:width], BF)

        def zero_body(n, carry):
            raw[pl.ds(4 * DM + n * 8, 8)] = jnp.zeros((8, H, DH), BF)
            return carry
        lax.fori_loop(0, RCH // 8, zero_body, 0)

        def x0_body(n, carry):
            @pl.when(lax.rem(n, 2) == 0)
            def _():
                x_piece(n // 2, 0).wait()
            transpose_x(n)
            return carry
        lax.fori_loop(0, 2 * NX0, x0_body, 0)

        def pair_up(w):
            return [jnp.concatenate([w[2 * m], w[2 * m + 1]], axis=1) for m in range(H // 2)]

        def bwq_body(t, carry):
            bwq_chunk(0, t).wait()
            rows = pl.ds(pl.multiple_of(t * RCH, RCH), RCH)
            for m, w in enumerate(pair_up(jnp.swapaxes(raw[rows, :, 0:T], 0, 1))):
                bwq_s[m, rows, :] = w
            return carry
        lax.fori_loop(0, NCH, bwq_body, 0)

        def chunk_rows(k, p, n, size, lanes=slice(None)):
            g = jnp.where(p > 0, k * NCH + p - 1, 4 * NCH)
            return raw[pl.ds(pl.multiple_of(g * RCH + n * size, size), size), :, lanes]

        def q_proj(m, half, start, n):
            w = bwq_s[m] if half == 0 else pltpu.bitcast(wy_s[wv_slot(m, 2, 0, HD)], BF)
            q = (_dot(x_rows(start, n, DM), w) * SCALE).astype(BF)
            rows = pl.ds(pl.multiple_of(start, 16), n)
            for odd in range(2):
                hm_s[2 * m + odd, rows, half * T:(half + 1) * T] = q[:, odd * T:(odd + 1) * T]

        def wv_slot(pair, odd, start, n):
            return (pl.ds(pl.multiple_of(XO + pair * HD + start, 8), n),
                    slice(odd * DH, (odd + 1) * DH))

        def pair_loop(unroll, waits, work):
            def body(i, carry):
                later = []
                for u in range(unroll):
                    p = i * unroll + u
                    for first, cp in waits(p, jnp.maximum(p - 1, 0)):
                        if u >= first:
                            cp.wait()
                        else:
                            assert first <= unroll
                            later.append(cp)

                @pl.when(i > 0)
                def _():
                    for cp in later:
                        cp.wait()

                for u in range(unroll):
                    p = i * unroll + u
                    work(p, jnp.maximum(p - 1, 0))
                return carry
            lax.fori_loop(0, H // 2 // unroll, body, 0)

        def q0_work(p, prev):
            def relayout(k):
                dst = pl.ds(pl.multiple_of(S + k * DM + prev * RCH, RCH), RCH)
                hm_s[:, dst, :] = jnp.swapaxes(chunk_rows(1 + k, p, 0, RCH), 0, 1)

            q_proj(p, 0, 0, R0 // 2)
            relayout(0)
            q_proj(p, 0, R0 // 2, R0 // 4)
            relayout(1)
            q_proj(p, 0, 3 * R0 // 4, R0 // 4)
        pair_loop(1, lambda p, prev: [(1, row_chunk(1, prev)), (1, row_chunk(2, prev))], q0_work)

        def ck_work(p, prev):
            def relayout(n):
                w = jnp.swapaxes(chunk_rows(3, p, n, RCH // 2), 0, 1)
                for h in range(H):
                    start = prev * (RCH // 2) + n * (RCH // 4)
                    wx_s[wv_slot(h // 2, h % 2, start, RCH // 4)] = u32(w[h])

            fold_pair(wx_s, p, [hm_s[2 * p + n, S + DM:S + 2 * DM, :] for n in range(2)],
                      [hm_s[2 * p + n, S:S + DM, :] for n in range(2)], SCALE,
                      CPLAN, [lambda: relayout(0), lambda: relayout(1)])
        pair_loop(1, lambda p, prev: [(1, row_chunk(3, prev))], ck_work)

        for s0 in range(UCH):
            for cp in stage_copies(s0, s0):
                cp.start()

        def cv_work(p, prev):
            def relayout_bwq():
                w = jnp.swapaxes(chunk_rows(0, p, 0, RCH, slice(T, 2 * T)), 0, 1)
                for m, wm in enumerate(pair_up(w)):
                    wy_s[wv_slot(m, 2, prev * (RCH // 2), RCH // 2)] = u32(wm)

            sides = [relayout_bwq, lambda: transpose_x(2 * p), lambda: transpose_x(2 * p + 1)]
            fold_pair(wy_s, p, [pltpu.bitcast(wx_s[wv_slot(p, n, 0, HD)], BF) for n in range(2)],
                      [wo_s[2 * p + n] for n in range(2)], None,
                      DPLAN, sides)
        pair_loop(2, lambda p, prev: [(0, wo_chunk(p)), (NX0, x_piece(p, 0)),
                                       (1, bwq_chunk(1, prev))], cv_work)

        cp_c.start()
        cp_bwo.start()
        cp_m0.wait()

        m0 = mem0_s[...].astype(F32)
        mem_init = jnp.concatenate([m0, m0[:, 384:448]], axis=1)

        def chain_body(b, mem):
            for u in range(UCH):
                i = b * UCH + u
                for cp in stage_copies(i, lax.rem(i, NSLOT)):
                    cp.wait()

            @pl.when(b + 1 < NPAIR // UCH)
            def _():
                for u in range(UCH):
                    nxt = (b + 1) * UCH + u
                    for cp in stage_copies(nxt, lax.rem(nxt, NSLOT)):
                        cp.start()

            for u in range(UCH):
                mem = pair_body(b, u, mem)
            return mem

        def pair_body(b, u, mem):
            i = b * UCH + u
            slot = lax.rem(i, NSLOT)

            def relayout_piece(n):
                part, src = n % 2, (stage_k, stage_v)[n // 2]
                wrows = pl.ds(pl.multiple_of(S + (n // 2) * DC + i * WCH + part * 16, 16), 16)
                hm_s[:, wrows, :] = jnp.swapaxes(src[slot, part * 16:(part + 1) * 16], 0, 1)

            def q_fill(k):
                def run():
                    n = 6 * u + k
                    same = [f for f, c in zip(FILL, HALF) if c == HALF[n]]
                    done = sum(f for f, c in zip(FILL[:n], HALF) if c == HALF[n])
                    start = (R0 if HALF[n] == 0 else 0) + lax.rem(b, 2) * sum(same) + done
                    for piece in PIECES[k]:
                        relayout_piece(piece)
                    q_proj(b // 2, HALF[n], start, FILL[n])
                return run

            lane = lax.broadcasted_iota(jnp.int32, (G, T), 1)
            r = lax.broadcasted_iota(jnp.int32, (G, H * L), 0)
            col = lax.broadcasted_iota(jnp.int32, (G, H * L), 1)
            kk = col - L * ((col * 1639) >> 16)
            keep_e = (r >= 32) | (kk >= 32) | (kk <= r)
            kpos = jnp.where(kk < 24, kk + 8, kk - 32)
            qpos = jnp.where(r < 24, r + 8, r - 32)
            q_any = ((r >= 24) & (r < 32)) | (r >= 40)
            keep_o = q_any | ((kk >= 24) & (kk < 32)) | (kpos <= qpos)

            base = pl.multiple_of(i * 64, 64)
            xs = x_rows(S + base, 64, 512)
            xs32 = xs[32:64, :].astype(F32)

            def proj(lhs, w_s, j):
                return _dot(lhs, pltpu.bitcast(w_s[j * HD:(j + 1) * HD, :], BF))

            def own(x):
                return jnp.concatenate([x[0:32, :], x[40:48, :]], axis=0)

            l1 = jnp.concatenate(
                [xs[0:32, :], jnp.concatenate([xs32[0:8, :], mem], axis=0).astype(BF)], axis=0)
            l1p = l1[:, 0:DM]
            k1 = [proj(l1p, wx_s, j) for j in range(H // 2)]
            v1 = []

            def v1_fn(j):
                v1.append(proj(l1p, wy_s, j))
                return own(v1[j])

            o1 = _rec_attention(l1, [own(k) for k in k1], v1_fn, q_fill(0), q_fill(1), keep_e, lane)
            q_fill(2)()

            l2 = jnp.concatenate([xs32[8:32, :], o1[40:48, :]], axis=0).astype(BF)
            l2p = l2[:, 0:DM]
            k2 = [jnp.concatenate([proj(l2p, wx_s, j), k1[j][32:40, :]], axis=0)
                  for j in range(H // 2)]
            o2 = _rec_attention(
                jnp.concatenate([l2, l1[32:48, :]], axis=0), k2,
                lambda j: jnp.concatenate([proj(l2p, wy_s, j), v1[j][32:40, :]], axis=0),
                q_fill(3), q_fill(4), keep_o, lane)
            q_fill(5)()

            res = jnp.concatenate([o1[0:32, :], o2[32:40, :], o2[0:24, :]], axis=0)
            out_s[pl.ds(base, 64), 0:512] = res.astype(BF)
            return o2[24:32, :]

        lax.fori_loop(0, NPAIR // UCH, chain_body, mem_init)

    pl.run_scoped(
        phase_a,
        pltpu.VMEM((DM, 2 * S), BF), pltpu.VMEM((MEM, DM), BF),
        pltpu.VMEM((4 * DM + RCH, H, DH), BF),
        pltpu.VMEM((H, DM, DH), BF), pltpu.VMEM((H // 2, DM, DH), BF),
        pltpu.VMEM((2 * XO, PAIR), jnp.uint32),
        pltpu.VMEM((XO + S, PAIR), jnp.uint32),
    )

    def phase_b(k_s, v_s, o_s, bt_s):
        cp_a = pltpu.make_async_copy(out_s.at[:, 0:384], out_hbm.at[:, 0:384], sems.at[0])
        cp_a.start()
        cp_c.wait()
        cp_bwo.wait()

        def head(h, carry):
            k_s[...] = _dot(c_s[...], hm_s[h, S:S + DC, :]).astype(BF)
            v_s[...] = _dot(c_s[...], hm_s[h, S + DC:S + 2 * DC, :]).astype(BF)
            row = lax.broadcasted_iota(jnp.int32, (T, T), 0)
            col = lax.broadcasted_iota(jnp.int32, (T, T), 1)
            tri = row >= col

            def qk(r0):
                q = hm_s[h, r0:r0 + BQ, :]
                return _b_qk(q, k_s, r0, tri)

            starts = list(reversed(range(0, S, BQ)))
            scores = qk(starts[0])
            for n, r0 in enumerate(starts):
                nxt = qk(starts[n + 1]) if n + 1 < len(starts) else None
                o_s[h, r0:r0 + BQ, :] = _b_pv(scores, v_s, h < 0).astype(BF)
                scores = nxt
            return carry
        lax.fori_loop(0, H, head, 0)

        def out_copy(t):
            rows = pl.ds(pl.multiple_of(t * BO, BO), BO)
            return pltpu.make_async_copy(
                out_s.at[rows, 384:2 * DM], out_hbm.at[rows, 384:2 * DM], out_sems.at[t])

        def project(t, after, never):
            rows = pl.ds(pl.multiple_of(t * BO, BO), BO)
            ctx = [o_s[h, rows, :] for h in range(H)]
            for n in range(2):
                ctx[8 + n] = jnp.where(never, after[:, n * DH:(n + 1) * DH], ctx[8 + n])
            wo = jnp.concatenate([bwo_s[h] for h in range(H)], axis=1)
            return _dot_nt(wo, jnp.concatenate(ctx, axis=1))

        def emit(t, bt):
            rows = pl.ds(pl.multiple_of(t * BO, BO), BO)
            b = jnp.concatenate([jnp.zeros((64, BO), F32), bt], axis=0).T.astype(BF)
            lo = lax.broadcasted_iota(jnp.int32, (BO, T), 1) < 64
            out_s[rows, 384:512] = jnp.where(lo, out_s[rows, 384:512], b[:, 0:T])
            out_s[rows, 512:896] = b[:, T:]
            return b

        bt_s[...] = jnp.zeros((DM, BO), F32)

        def oproj(i, carry):
            prev = jnp.maximum(UOP * i - 1, 0)
            b = emit(prev, bt_s[...])

            @pl.when(i > 0)
            def _():
                out_copy(prev).start()

            for u in range(UOP - 1):
                b = emit(UOP * i + u, project(UOP * i + u, b, i < 0))
                out_copy(UOP * i + u).start()
            bt_s[...] = project(UOP * i + UOP - 1, b, i < 0)
            return carry
        lax.fori_loop(0, S // BO // UOP, oproj, 0)
        emit(S // BO - 1, bt_s[...])
        out_copy(S // BO - 1).start()
        cp_a.wait()
        for t in range(S // BO):
            out_copy(t).wait()

    pl.run_scoped(
        phase_b,
        pltpu.VMEM((S, DH), BF), pltpu.VMEM((S, DH), BF),
        pltpu.VMEM((H, S, DH), BF), pltpu.VMEM((DM, BO), F32),
    )


@jax.jit
def pallas_concat_heads__memory_aug_recurrent_mem_tr__compressed_kv_cla__prompt_kernel(
    A_x: jax.Array,
    A_mem0: jax.Array,
    A_Wq: jax.Array,
    A_Wk: jax.Array,
    A_Wv: jax.Array,
    A_Wo: jax.Array,
    A_seg_len: jax.Array,
    B_x: jax.Array,
    B_c_kv: jax.Array,
    B_w_q: jax.Array,
    B_w_uk: jax.Array,
    B_w_uv: jax.Array,
    B_w_o: jax.Array,
):
    del A_seg_len
    assert A_x.shape == (1, S, DM) and A_mem0.shape == (1, MEM, DM)
    assert A_Wq.shape == (DM, H, DH) and A_Wo.shape == (H, DH, DM)
    assert B_x.shape == (1, S, DM) and B_c_kv.shape == (1, S, DC)
    assert B_w_uk.shape == (DC, H, DH) and B_w_o.shape == (H, DH, DM)

    any_spec = pl.BlockSpec(memory_space=pl.ANY)
    out = pl.pallas_call(
        _kernel,
        out_shape=jax.ShapeDtypeStruct((S, 2 * DM), BF),
        in_specs=[any_spec] * 12,
        out_specs=any_spec,
        scratch_shapes=[
            pltpu.VMEM((S, DC), BF),
            pltpu.VMEM((H, S + 2 * DC, DH), BF),
            pltpu.VMEM((H, DM, DH), BF),
            pltpu.VMEM((NSLOT, WCH, H, DH), BF),
            pltpu.VMEM((NSLOT, WCH, H, DH), BF),
            pltpu.VMEM((S, 2 * DM), BF),
            pltpu.SemaphoreType.DMA((4,)),
            pltpu.SemaphoreType.DMA((7, 8)),
            pltpu.SemaphoreType.DMA((2, NSLOT)),
            pltpu.SemaphoreType.DMA((S // BO,)),
        ],
        compiler_params=pltpu.CompilerParams(
            vmem_limit_bytes=120 * 1024 * 1024,
            disable_bounds_checks=True,
            disable_semaphore_checks=True),
    )(jnp.swapaxes(A_x, 1, 2).reshape(DM, S), A_mem0.reshape(MEM, DM), A_Wq, A_Wk, A_Wv,
      jnp.swapaxes(A_Wo, 1, 2),
      jnp.swapaxes(B_x, 1, 2).reshape(DM, S), B_c_kv.reshape(S, DC), B_w_q, B_w_uk, B_w_uv,
      jnp.swapaxes(B_w_o, 1, 2))
    return out.reshape(1, S, 2 * DM)
```

```python
import jax
import jax.numpy as jnp
from jax import lax
import jax.experimental.pallas as pl
import jax.experimental.pallas.tpu as pltpu

BF = jnp.bfloat16
F32 = jnp.float32

S = 2048
DM = 448
H = 16
DH = 256
MEM = 8
SEG = 32
DC = 1024
LOG2E = 1.4426950408889634
SCALE = DH ** -0.5 * LOG2E
NEG = -1000000000.0 * LOG2E
T = 128
L = MEM + SEG
G = 48
PAIR = 2 * DM
BQ = 512
KC = 256
BO = 128
UOP = 2
UCH = 2
NPAIR = S // (2 * SEG)
WCH = DC // NPAIR
NSLOT = 2 * UCH
RCH = 64
LAG = 2
FILL = (144, 96, 176, 144, 80, 176, 144, 96, 176, 144, 80, 112)
HALF = (0, 1, 1, 0, 1, 1, 0, 1, 1, 1, 1, 0)
PIECES = ((0,), (), (1,), (2,), (), (3,))
R0 = S - 2 * sum(f for f, c in zip(FILL, HALF) if c == 0)
assert sum(f for f, c in zip(FILL, HALF) if c == 1) * 2 == S and UCH == 2
NCH = DM // RCH
HD = DM // 2
XO = (H // 2) * HD
XP = 512
NX0 = -(-R0 // XP)
CPLAN = ((0, 0, 3), 's', 't', (1, 0, 1), 's', (1, 1, 3))
DPLAN = ((0, 0, 2), 's', (0, 2, 3), 's', 't', (1, 0, 1), 's', (1, 1, 3))


def _dot(a, b):
    return jnp.dot(a, b, preferred_element_type=F32)


def _dot_nt(a, b):
    return lax.dot_general(a, b, (((1,), (1,)), ((), ())), preferred_element_type=F32)


def _seg_reduce_bcast(x, lane, fill, combine, reduce_fn):
    nt = H * L // T
    tiles = [x[:, t * T:(t + 1) * T] for t in range(nt)]
    outs = [None] * nt
    for g in range(H):
        parts = []
        for t in range(nt):
            lo = max(L * g - T * t, 0)
            hi = min(L * g + L - T * t, T)
            if lo < hi:
                parts.append((t, (lane >= lo) & (lane < hi)))
        acc = None
        for t, msk in parts:
            sel = jnp.where(msk, tiles[t], fill)
            acc = sel if acc is None else combine(acc, sel)
        red = reduce_fn(acc, axis=1, keepdims=True)
        for t, msk in parts:
            if outs[t] is None:
                outs[t] = jnp.broadcast_to(red, tiles[t].shape)
            else:
                outs[t] = jnp.where(msk, red, outs[t])
    return jnp.concatenate(outs, axis=1)


def _seg_softmax(s, keep, lane):
    s = jnp.where(keep, s, NEG)
    m = _seg_reduce_bcast(s, lane, -jnp.inf, jnp.maximum, jnp.max)
    p = jnp.exp2(s - m)
    l = _seg_reduce_bcast(p, lane, 0.0, jnp.add, jnp.sum)
    return (p * (1.0 / l)).astype(BF)


def _stack(slabs):
    lo = lax.broadcasted_iota(jnp.int32, (L, T), 1) < 64
    blocks = []
    for r in slabs:
        tail = r[:, 768:896]
        blocks.append(jnp.concatenate([r[:, 0:384], jnp.where(lo, tail, 0.0)], axis=1))
        blocks.append(jnp.concatenate([r[:, 384:768], jnp.where(lo, 0.0, tail)], axis=1))
    return jnp.concatenate(blocks, axis=0).astype(BF)


def _rec_attention(qrows, kslabs, vslab_fn, filler0, filler, keep, lane):
    filler0()
    s = _dot_nt(qrows, _stack(kslabs))
    vslabs = [vslab_fn(j) for j in range(H // 2)]
    filler()
    p = _seg_softmax(s, keep, lane)
    o = _dot(p, _stack(vslabs))
    t = o[:, 384:512]
    return jnp.concatenate([o[:, 0:384], t + pltpu.roll(t, 64, 1)], axis=1)


def _b_qk(q, k_s, r0, tri):
    nt = BQ // T

    def mask_top(blk):
        top = jnp.where(tri, blk[0:T, :], NEG)
        return jnp.concatenate([top, blk[T:, :]], axis=0) if blk.shape[0] > T else top

    s_main = _dot_nt(q, k_s[0:r0 + T, :])
    chunks = [(0, c0, s_main[:, c0:min(c0 + KC, r0)]) for c0 in range(0, r0, KC)]
    chunks.append((0, r0, mask_top(s_main[:, r0:r0 + T])))
    for t in range(1, nt):
        chunks.append((t * T, r0 + t * T, mask_top(
            _dot_nt(q[t * T:, :], k_s[r0 + t * T:r0 + (t + 1) * T, :]))))
    ms = []
    for u in range(nt):
        row = [c[u * T - f:(u + 1) * T - f, :] for f, _, c in chunks if f <= u * T]
        row = jnp.concatenate(row, axis=1) if len(row) > 1 else row[0]
        ms.append(jnp.max(row, axis=1, keepdims=True))
    return chunks, jnp.concatenate(ms, axis=0)


def _b_pv(scores, v_s, never):
    chunks, m = scores
    nt = BQ // T
    o = [None] * nt
    l = None
    ocs = []
    mb = jnp.broadcast_to(m, (BQ, T))
    for f, k0, c in chunks:
        mc = mb[f:, :]
        if len(ocs) >= LAG:
            pf, prev = ocs[-LAG]
            mc = jnp.where(never, prev[f - pf:, 0:T], mc)
        ps = [jnp.exp2(c[:, j * T:(j + 1) * T] - mc) for j in range(c.shape[1] // T)]
        p = jnp.concatenate(ps, axis=1) if len(ps) > 1 else ps[0]
        oc = _dot(p.astype(BF), v_s[k0:k0 + c.shape[1], :])
        ocs.append((f, oc))
        lc = ps[0]
        for x in ps[1:]:
            lc = lc + x
        if l is None:
            l = lc
        elif f == 0:
            l = l + lc
        else:
            l = jnp.concatenate([l[0:f, :], l[f:, :] + lc], axis=0)
        for u in range(f // T, nt):
            rows = slice(u * T - f, (u + 1) * T - f)
            o[u] = oc[rows] if o[u] is None else o[u] + oc[rows]
    return jnp.concatenate(o, axis=0) * (1.0 / jnp.sum(l, axis=1, keepdims=True))


def _kernel(xa_hbm, mem0_hbm, wq_hbm, wk_hbm, wv_hbm, wo_hbm,
            xb_hbm, c_hbm, bwq_hbm, bwk_hbm, bwv_hbm, bwo_hbm,
            out_hbm,
            c_s, hm_s, bwo_s, stage_k, stage_v, out_s,
            sems, w_sems, stage_sems, out_sems):

    def stage_copies(chunk, slot):
        rows = pl.ds(chunk * WCH, WCH)
        return (pltpu.make_async_copy(bwk_hbm.at[rows], stage_k.at[slot], stage_sems.at[0, slot]),
                pltpu.make_async_copy(bwv_hbm.at[rows], stage_v.at[slot], stage_sems.at[1, slot]))

    cp_c = pltpu.make_async_copy(c_hbm, c_s, sems.at[2])
    cp_bwo = pltpu.make_async_copy(bwo_hbm, bwo_s, sems.at[3])

    def phase_a(xt_s, mem0_s, raw, wo_s, bwq_s, wx_s, wy_s):
        srcs = (bwq_hbm, wq_hbm, wk_hbm, wv_hbm)

        def row_chunk(k, t):
            return pltpu.make_async_copy(
                srcs[k].at[pl.ds(t * RCH, RCH)], raw.at[pl.ds((k * NCH + t) * RCH, RCH)],
                w_sems.at[k, t])

        def bwq_chunk(c, t):
            rows, lanes = pl.ds(t * RCH, RCH), pl.ds(c * T, T)
            return pltpu.make_async_copy(
                bwq_hbm.at[rows, :, lanes], raw.at[rows, :, lanes], w_sems.at[6 * c, t])

        def wo_chunk(j):
            heads = pl.ds(2 * j, 2)
            return pltpu.make_async_copy(wo_hbm.at[heads], wo_s.at[heads], w_sems.at[4, j])

        def x_piece(k, src_k=None):
            sk = k if src_k is None else src_k
            src = (xb_hbm, xa_hbm)[sk // 4].at[:, pl.ds((sk % 4) * XP, XP)]
            return pltpu.make_async_copy(
                src, xt_s.at[:, pl.ds(pl.multiple_of(k * XP, XP), XP)], w_sems.at[5, k])

        cp_m0 = pltpu.make_async_copy(mem0_hbm, mem0_s, sems.at[1])

        def start_each(copies):
            def body(t, carry):
                for cp in copies(t):
                    cp.start()
                return carry
            lax.fori_loop(0, NCH, body, 0)

        for k in range(NX0):
            x_piece(k).start()
        start_each(lambda t: [bwq_chunk(0, t)])
        start_each(lambda t: [row_chunk(1, t), row_chunk(2, t)])
        start_each(lambda t: [row_chunk(3, t)])
        for j in range(H // 2):
            wo_chunk(j).start()
            if j >= NX0:
                x_piece(j).start()
            if j > 0:
                bwq_chunk(1, j - 1).start()
        cp_m0.start()

        def u32(w):
            return pltpu.bitcast(w.astype(BF), jnp.uint32)

        def fold_pair(dst, p, lhs, rhs, scale, plan, sides):
            def put(lanes, val):
                val = val if scale is None else val * scale
                dst[pl.ds(pl.multiple_of(p * HD, 8), HD), lanes] = u32(val)

            zero = jnp.zeros((64, DH), BF)
            tails = jnp.concatenate(
                [jnp.concatenate([rhs[0][384:448, :], zero], axis=1),
                 jnp.concatenate([zero, rhs[1][384:448, :]], axis=1)], axis=0)
            sides = iter(sides)
            for step in plan:
                if step == 't':
                    put(slice(768, 896), _dot_nt(jnp.concatenate(lhs, axis=1), tails))
                elif step == 's':
                    next(sides)()
                else:
                    n, c0, c1 = step
                    put(slice(384 * n + c0 * T, 384 * n + c1 * T),
                        _dot_nt(lhs[n], rhs[n][c0 * T:c1 * T, :]))

        def transpose_x(n, width=256):
            cols = pl.ds(pl.multiple_of(n * width, width), width)
            x = xt_s[:, cols]
            rows = pl.ds(pl.multiple_of(XO + n * (width // 2), width // 2), width // 2)
            wy_s[rows, 0:512] = u32(jnp.concatenate([x, x[384:448, :]], axis=0).T)

        def x_rows(start, n, width):
            rows = pl.ds(pl.multiple_of(XO + start // 2, 8), n // 2)
            return pltpu.bitcast(wy_s[rows, 0:width], BF)

        def zero_body(n, carry):
            raw[pl.ds(4 * DM + n * 8, 8)] = jnp.zeros((8, H, DH), BF)
            return carry
        lax.fori_loop(0, RCH // 8, zero_body, 0)

        def x0_body(n, carry):
            @pl.when(lax.rem(n, XP // T) == 0)
            def _():
                x_piece(n // (XP // T), 0).wait()
            transpose_x(n, T)
            return carry
        lax.fori_loop(0, NX0 * XP // T, x0_body, 0)

        def pair_up(w):
            return [jnp.concatenate([w[2 * m], w[2 * m + 1]], axis=1) for m in range(H // 2)]

        def bwq_body(t, carry):
            @pl.when(lax.rem(t, 2) == 0)
            def _():
                bwq_chunk(0, t // 2).wait()
            rows = pl.ds(pl.multiple_of(t * (RCH // 2), RCH // 2), RCH // 2)
            for m, w in enumerate(pair_up(jnp.swapaxes(raw[rows, :, 0:T], 0, 1))):
                bwq_s[m, rows, :] = w
            return carry
        lax.fori_loop(0, 2 * NCH, bwq_body, 0)

        def chunk_rows(k, p, n, size, lanes=slice(None)):
            g = jnp.where(p > 0, k * NCH + p - 1, 4 * NCH)
            return raw[pl.ds(pl.multiple_of(g * RCH + n * size, size), size), :, lanes]

        def q_proj(m, half, start, n):
            w = bwq_s[m] if half == 0 else pltpu.bitcast(wy_s[wv_slot(m, 2, 0, HD)], BF)
            q = (_dot(x_rows(start, n, DM), w) * SCALE).astype(BF)
            rows = pl.ds(pl.multiple_of(start, 16), n)
            for odd in range(2):
                hm_s[2 * m + odd, rows, half * T:(half + 1) * T] = q[:, odd * T:(odd + 1) * T]

        def wv_slot(pair, odd, start, n):
            return (pl.ds(pl.multiple_of(XO + pair * HD + start, 8), n),
                    slice(odd * DH, (odd + 1) * DH))

        def pair_loop(unroll, waits, work):
            def body(i, carry):
                later = []
                for u in range(unroll):
                    p = i * unroll + u
                    for first, cp in waits(p, jnp.maximum(p - 1, 0)):
                        if u >= first:
                            cp.wait()
                        else:
                            assert first <= unroll
                            later.append(cp)

                @pl.when(i > 0)
                def _():
                    for cp in later:
                        cp.wait()

                for u in range(unroll):
                    p = i * unroll + u
                    work(p, jnp.maximum(p - 1, 0))
                return carry
            lax.fori_loop(0, H // 2 // unroll, body, 0)

        def q0_work(p, prev):
            def relayout(k):
                dst = pl.ds(pl.multiple_of(S + k * DM + prev * RCH, RCH), RCH)
                hm_s[:, dst, :] = jnp.swapaxes(chunk_rows(1 + k, p, 0, RCH), 0, 1)

            q_proj(p, 0, 0, R0 // 2)
            relayout(0)
            q_proj(p, 0, R0 // 2, R0 // 4)
            relayout(1)
            q_proj(p, 0, 3 * R0 // 4, R0 // 4)
        pair_loop(1, lambda p, prev: [(1, row_chunk(1, prev)), (1, row_chunk(2, prev))], q0_work)

        def ck_work(p, prev):
            def relayout(n):
                w = jnp.swapaxes(chunk_rows(3, p, n, RCH // 2), 0, 1)
                for h in range(H):
                    start = prev * (RCH // 2) + n * (RCH // 4)
                    wx_s[wv_slot(h // 2, h % 2, start, RCH // 4)] = u32(w[h])

            fold_pair(wx_s, p, [hm_s[2 * p + n, S + DM:S + 2 * DM, :] for n in range(2)],
                      [hm_s[2 * p + n, S:S + DM, :] for n in range(2)], SCALE,
                      CPLAN, [lambda: relayout(0), lambda: relayout(1)])
        pair_loop(1, lambda p, prev: [(1, row_chunk(3, prev))], ck_work)

        for s0 in range(UCH):
            for cp in stage_copies(s0, s0):
                cp.start()

        def cv_work(p, prev):
            def relayout_bwq():
                w = jnp.swapaxes(chunk_rows(0, p, 0, RCH, slice(T, 2 * T)), 0, 1)
                for m, wm in enumerate(pair_up(w)):
                    wy_s[wv_slot(m, 2, prev * (RCH // 2), RCH // 2)] = u32(wm)

            sides = [relayout_bwq, lambda: transpose_x(2 * p), lambda: transpose_x(2 * p + 1)]
            fold_pair(wy_s, p, [pltpu.bitcast(wx_s[wv_slot(p, n, 0, HD)], BF) for n in range(2)],
                      [wo_s[2 * p + n] for n in range(2)], None,
                      DPLAN, sides)
        pair_loop(2, lambda p, prev: [(0, wo_chunk(p)), (NX0, x_piece(p, 0)),
                                       (1, bwq_chunk(1, prev))], cv_work)

        cp_c.start()
        cp_bwo.start()
        cp_m0.wait()

        m0 = mem0_s[...].astype(F32)
        mem_init = jnp.concatenate([m0, m0[:, 384:448]], axis=1)

        def chain_body(b, mem):
            for u in range(UCH):
                i = b * UCH + u
                for cp in stage_copies(i, lax.rem(i, NSLOT)):
                    cp.wait()

            @pl.when(b + 1 < NPAIR // UCH)
            def _():
                for u in range(UCH):
                    nxt = (b + 1) * UCH + u
                    for cp in stage_copies(nxt, lax.rem(nxt, NSLOT)):
                        cp.start()

            for u in range(UCH):
                mem = pair_body(b, u, mem)
            return mem

        def pair_body(b, u, mem):
            i = b * UCH + u
            slot = lax.rem(i, NSLOT)

            def relayout_piece(n):
                part, src = n % 2, (stage_k, stage_v)[n // 2]
                wrows = pl.ds(pl.multiple_of(S + (n // 2) * DC + i * WCH + part * 16, 16), 16)
                hm_s[:, wrows, :] = jnp.swapaxes(src[slot, part * 16:(part + 1) * 16], 0, 1)

            def q_fill(k):
                def run():
                    n = 6 * u + k
                    same = [f for f, c in zip(FILL, HALF) if c == HALF[n]]
                    done = sum(f for f, c in zip(FILL[:n], HALF) if c == HALF[n])
                    start = (R0 if HALF[n] == 0 else 0) + lax.rem(b, 2) * sum(same) + done
                    for piece in PIECES[k]:
                        relayout_piece(piece)
                    q_proj(b // 2, HALF[n], start, FILL[n])
                return run

            lane = lax.broadcasted_iota(jnp.int32, (G, T), 1)
            r = lax.broadcasted_iota(jnp.int32, (G, H * L), 0)
            col = lax.broadcasted_iota(jnp.int32, (G, H * L), 1)
            kk = col - L * ((col * 1639) >> 16)
            keep_e = (r >= 32) | (kk >= 32) | (kk <= r)
            kpos = jnp.where(kk < 24, kk + 8, kk - 32)
            qpos = jnp.where(r < 24, r + 8, r - 32)
            q_any = ((r >= 24) & (r < 32)) | (r >= 40)
            keep_o = q_any | ((kk >= 24) & (kk < 32)) | (kpos <= qpos)

            base = pl.multiple_of(i * 64, 64)
            xs = x_rows(S + base, 64, 512)
            xs32 = xs[32:64, :].astype(F32)

            def proj(lhs, w_s, j):
                return _dot(lhs, pltpu.bitcast(w_s[j * HD:(j + 1) * HD, :], BF))

            def own(x):
                return jnp.concatenate([x[0:32, :], x[40:48, :]], axis=0)

            l1 = jnp.concatenate(
                [xs[0:32, :], jnp.concatenate([xs32[0:8, :], mem], axis=0).astype(BF)], axis=0)
            l1p = l1[:, 0:DM]
            k1 = [proj(l1p, wx_s, j) for j in range(H // 2)]
            v1 = []

            def v1_fn(j):
                v1.append(proj(l1p, wy_s, j))
                return own(v1[j])

            o1 = _rec_attention(l1, [own(k) for k in k1], v1_fn, q_fill(0), q_fill(1), keep_e, lane)
            q_fill(2)()

            l2 = jnp.concatenate([xs32[8:32, :], o1[40:48, :]], axis=0).astype(BF)
            l2p = l2[:, 0:DM]
            k2 = [jnp.concatenate([proj(l2p, wx_s, j), k1[j][32:40, :]], axis=0)
                  for j in range(H // 2)]
            o2 = _rec_attention(
                jnp.concatenate([l2, l1[32:48, :]], axis=0), k2,
                lambda j: jnp.concatenate([proj(l2p, wy_s, j), v1[j][32:40, :]], axis=0),
                q_fill(3), q_fill(4), keep_o, lane)
            q_fill(5)()

            res = jnp.concatenate([o1[0:32, :], o2[32:40, :], o2[0:24, :]], axis=0)
            out_s[pl.ds(base, 64), 0:512] = res.astype(BF)
            return o2[24:32, :]

        lax.fori_loop(0, NPAIR // UCH, chain_body, mem_init)

    pl.run_scoped(
        phase_a,
        pltpu.VMEM((DM, 2 * S), BF), pltpu.VMEM((MEM, DM), BF),
        pltpu.VMEM((4 * DM + RCH, H, DH), BF),
        pltpu.VMEM((H, DM, DH), BF), pltpu.VMEM((H // 2, DM, DH), BF),
        pltpu.VMEM((2 * XO, PAIR), jnp.uint32),
        pltpu.VMEM((XO + S, PAIR), jnp.uint32),
    )

    def phase_b(k_s, v_s, o_s, bt_s):
        cp_a = pltpu.make_async_copy(out_s.at[:, 0:384], out_hbm.at[:, 0:384], sems.at[0])
        cp_a.start()
        cp_c.wait()
        cp_bwo.wait()

        def head(h, carry):
            k_s[...] = _dot(c_s[...], hm_s[h, S:S + DC, :]).astype(BF)
            v_s[...] = _dot(c_s[...], hm_s[h, S + DC:S + 2 * DC, :]).astype(BF)
            row = lax.broadcasted_iota(jnp.int32, (T, T), 0)
            col = lax.broadcasted_iota(jnp.int32, (T, T), 1)
            tri = row >= col

            def qk(r0):
                q = hm_s[h, r0:r0 + BQ, :]
                return _b_qk(q, k_s, r0, tri)

            starts = list(reversed(range(0, S, BQ)))
            scores = qk(starts[0])
            for n, r0 in enumerate(starts):
                nxt = qk(starts[n + 1]) if n + 1 < len(starts) else None
                o_s[h, r0:r0 + BQ, :] = _b_pv(scores, v_s, h < 0).astype(BF)
                scores = nxt
            return carry
        lax.fori_loop(0, H, head, 0)

        def out_copy(t):
            rows = pl.ds(pl.multiple_of(t * BO, BO), BO)
            return pltpu.make_async_copy(
                out_s.at[rows, 384:2 * DM], out_hbm.at[rows, 384:2 * DM], out_sems.at[t])

        def project(t, after, never):
            rows = pl.ds(pl.multiple_of(t * BO, BO), BO)
            ctx = [o_s[h, rows, :] for h in range(H)]
            for n in range(2):
                ctx[8 + n] = jnp.where(never, after[:, n * DH:(n + 1) * DH], ctx[8 + n])
            wo = jnp.concatenate([bwo_s[h] for h in range(H)], axis=1)
            return _dot_nt(wo, jnp.concatenate(ctx, axis=1))

        def emit(t, bt):
            rows = pl.ds(pl.multiple_of(t * BO, BO), BO)
            b = jnp.concatenate([jnp.zeros((64, BO), F32), bt], axis=0).T.astype(BF)
            lo = lax.broadcasted_iota(jnp.int32, (BO, T), 1) < 64
            out_s[rows, 384:512] = jnp.where(lo, out_s[rows, 384:512], b[:, 0:T])
            out_s[rows, 512:896] = b[:, T:]
            return b

        bt_s[...] = jnp.zeros((DM, BO), F32)

        def oproj(i, carry):
            prev = jnp.maximum(UOP * i - 1, 0)
            b = emit(prev, bt_s[...])

            @pl.when(i > 0)
            def _():
                out_copy(prev).start()

            for u in range(UOP - 1):
                b = emit(UOP * i + u, project(UOP * i + u, b, i < 0))
                out_copy(UOP * i + u).start()
            bt_s[...] = project(UOP * i + UOP - 1, b, i < 0)
            return carry
        lax.fori_loop(0, S // BO // UOP, oproj, 0)
        emit(S // BO - 1, bt_s[...])
        out_copy(S // BO - 1).start()
        cp_a.wait()
        for t in range(S // BO):
            out_copy(t).wait()

    pl.run_scoped(
        phase_b,
        pltpu.VMEM((S, DH), BF), pltpu.VMEM((S, DH), BF),
        pltpu.VMEM((H, S, DH), BF), pltpu.VMEM((DM, BO), F32),
    )


@jax.jit
def pallas_concat_heads__memory_aug_recurrent_mem_tr__compressed_kv_cla__prompt_kernel(
    A_x: jax.Array,
    A_mem0: jax.Array,
    A_Wq: jax.Array,
    A_Wk: jax.Array,
    A_Wv: jax.Array,
    A_Wo: jax.Array,
    A_seg_len: jax.Array,
    B_x: jax.Array,
    B_c_kv: jax.Array,
    B_w_q: jax.Array,
    B_w_uk: jax.Array,
    B_w_uv: jax.Array,
    B_w_o: jax.Array,
):
    del A_seg_len
    assert A_x.shape == (1, S, DM) and A_mem0.shape == (1, MEM, DM)
    assert A_Wq.shape == (DM, H, DH) and A_Wo.shape == (H, DH, DM)
    assert B_x.shape == (1, S, DM) and B_c_kv.shape == (1, S, DC)
    assert B_w_uk.shape == (DC, H, DH) and B_w_o.shape == (H, DH, DM)

    any_spec = pl.BlockSpec(memory_space=pl.ANY)
    out = pl.pallas_call(
        _kernel,
        out_shape=jax.ShapeDtypeStruct((S, 2 * DM), BF),
        in_specs=[any_spec] * 12,
        out_specs=any_spec,
        scratch_shapes=[
            pltpu.VMEM((S, DC), BF),
            pltpu.VMEM((H, S + 2 * DC, DH), BF),
            pltpu.VMEM((H, DM, DH), BF),
            pltpu.VMEM((NSLOT, WCH, H, DH), BF),
            pltpu.VMEM((NSLOT, WCH, H, DH), BF),
            pltpu.VMEM((S, 2 * DM), BF),
            pltpu.SemaphoreType.DMA((4,)),
            pltpu.SemaphoreType.DMA((7, 8)),
            pltpu.SemaphoreType.DMA((2, NSLOT)),
            pltpu.SemaphoreType.DMA((S // BO,)),
        ],
        compiler_params=pltpu.CompilerParams(
            vmem_limit_bytes=120 * 1024 * 1024,
            disable_bounds_checks=True,
            disable_semaphore_checks=True),
    )(jnp.swapaxes(A_x, 1, 2).reshape(DM, S), A_mem0.reshape(MEM, DM), A_Wq, A_Wk, A_Wv,
      jnp.swapaxes(A_Wo, 1, 2),
      jnp.swapaxes(B_x, 1, 2).reshape(DM, S), B_c_kv.reshape(S, DC), B_w_q, B_w_uk, B_w_uv,
      jnp.swapaxes(B_w_o, 1, 2))
    return out.reshape(1, S, 2 * DM)
```

```python
import jax
import jax.numpy as jnp
from jax import lax
import jax.experimental.pallas as pl
import jax.experimental.pallas.tpu as pltpu

BF = jnp.bfloat16
F32 = jnp.float32

S = 2048
DM = 448
H = 16
DH = 256
MEM = 8
SEG = 32
DC = 1024
LOG2E = 1.4426950408889634
SCALE = DH ** -0.5 * LOG2E
NEG = -1000000000.0 * LOG2E
T = 128
L = MEM + SEG
G = 48
PAIR = 2 * DM
BQ = 512
KC = 256
BO = 128
UOP = 2
UCH = 2
NPAIR = S // (2 * SEG)
WCH = DC // NPAIR
NSLOT = 2 * UCH
RCH = 64
LAG = 2
FILL = (144, 96, 176, 144, 80, 176, 144, 96, 176, 144, 80, 112)
HALF = (0, 1, 1, 0, 1, 1, 0, 1, 1, 1, 1, 0)
PIECES = ((0,), (), (1,), (2,), (), (3,))
R0 = S - 2 * sum(f for f, c in zip(FILL, HALF) if c == 0)
assert sum(f for f, c in zip(FILL, HALF) if c == 1) * 2 == S and UCH == 2
NCH = DM // RCH
HD = DM // 2
XO = (H // 2) * HD
XP = 512
NX0 = -(-R0 // XP)
CPLAN = ((0, 0, 3), 's', 't', (1, 0, 1), 's', (1, 1, 3))
DPLAN = ((0, 0, 2), 's', (0, 2, 3), 's', 't', (1, 0, 1), 's', (1, 1, 3))


def _dot(a, b):
    return jnp.dot(a, b, preferred_element_type=F32)


def _dot_nt(a, b):
    return lax.dot_general(a, b, (((1,), (1,)), ((), ())), preferred_element_type=F32)


def _seg_reduce_bcast(x, lane, fill, combine, reduce_fn):
    nt = H * L // T
    tiles = [x[:, t * T:(t + 1) * T] for t in range(nt)]
    outs = [None] * nt
    for g in range(H):
        parts = []
        for t in range(nt):
            lo = max(L * g - T * t, 0)
            hi = min(L * g + L - T * t, T)
            if lo < hi:
                parts.append((t, (lane >= lo) & (lane < hi)))
        acc = None
        for t, msk in parts:
            sel = jnp.where(msk, tiles[t], fill)
            acc = sel if acc is None else combine(acc, sel)
        red = reduce_fn(acc, axis=1, keepdims=True)
        for t, msk in parts:
            if outs[t] is None:
                outs[t] = jnp.broadcast_to(red, tiles[t].shape)
            else:
                outs[t] = jnp.where(msk, red, outs[t])
    return jnp.concatenate(outs, axis=1)


def _seg_softmax(s, keep, lane):
    s = jnp.where(keep, s, NEG)
    m = _seg_reduce_bcast(s, lane, -jnp.inf, jnp.maximum, jnp.max)
    p = jnp.exp2(s - m)
    l = _seg_reduce_bcast(p, lane, 0.0, jnp.add, jnp.sum)
    return (p * (1.0 / l)).astype(BF)


def _stack(slabs):
    lo = lax.broadcasted_iota(jnp.int32, (L, T), 1) < 64
    blocks = []
    for r in slabs:
        tail = r[:, 768:896]
        blocks.append(jnp.concatenate([r[:, 0:384], jnp.where(lo, tail, 0.0)], axis=1))
        blocks.append(jnp.concatenate([r[:, 384:768], jnp.where(lo, 0.0, tail)], axis=1))
    return jnp.concatenate(blocks, axis=0).astype(BF)


def _rec_attention(qrows, kslabs, vslab_fn, filler0, filler, keep, lane):
    filler0()
    s = _dot_nt(qrows, _stack(kslabs))
    vslabs = [vslab_fn(j) for j in range(H // 2)]
    filler()
    p = _seg_softmax(s, keep, lane)
    o = _dot(p, _stack(vslabs))
    t = o[:, 384:512]
    return jnp.concatenate([o[:, 0:384], t + pltpu.roll(t, 64, 1)], axis=1)


def _b_qk(q, k_s, r0, tri):
    nt = BQ // T

    def mask_top(blk):
        top = jnp.where(tri, blk[0:T, :], NEG)
        return jnp.concatenate([top, blk[T:, :]], axis=0) if blk.shape[0] > T else top

    s_main = _dot_nt(q, k_s[0:r0 + T, :])
    chunks = [(0, c0, s_main[:, c0:min(c0 + KC, r0)]) for c0 in range(0, r0, KC)]
    chunks.append((0, r0, mask_top(s_main[:, r0:r0 + T])))
    for t in range(1, nt):
        chunks.append((t * T, r0 + t * T, mask_top(
            _dot_nt(q[t * T:, :], k_s[r0 + t * T:r0 + (t + 1) * T, :]))))
    ms = []
    for u in range(nt):
        row = [c[u * T - f:(u + 1) * T - f, :] for f, _, c in chunks if f <= u * T]
        row = jnp.concatenate(row, axis=1) if len(row) > 1 else row[0]
        ms.append(jnp.max(row, axis=1, keepdims=True))
    return chunks, jnp.concatenate(ms, axis=0)


def _b_pv(scores, v_s, never):
    chunks, m = scores
    nt = BQ // T
    o = [None] * nt
    l = None
    ocs = []
    mb = jnp.broadcast_to(m, (BQ, T))
    for f, k0, c in chunks:
        mc = mb[f:, :]
        if len(ocs) >= LAG:
            pf, prev = ocs[-LAG]
            mc = jnp.where(never, prev[f - pf:, 0:T], mc)
        ps = [jnp.exp2(c[:, j * T:(j + 1) * T] - mc) for j in range(c.shape[1] // T)]
        p = jnp.concatenate(ps, axis=1) if len(ps) > 1 else ps[0]
        oc = _dot(p.astype(BF), v_s[k0:k0 + c.shape[1], :])
        ocs.append((f, oc))
        lc = ps[0]
        for x in ps[1:]:
            lc = lc + x
        if l is None:
            l = lc
        elif f == 0:
            l = l + lc
        else:
            l = jnp.concatenate([l[0:f, :], l[f:, :] + lc], axis=0)
        for u in range(f // T, nt):
            rows = slice(u * T - f, (u + 1) * T - f)
            o[u] = oc[rows] if o[u] is None else o[u] + oc[rows]
    return jnp.concatenate(o, axis=0) * (1.0 / jnp.sum(l, axis=1, keepdims=True))


def _kernel(xa_hbm, mem0_hbm, wq_hbm, wk_hbm, wv_hbm, wo_hbm,
            xb_hbm, c_hbm, bwq_hbm, bwk_hbm, bwv_hbm, bwo_hbm,
            out_hbm,
            c_s, hm_s, bwo_s, stage_k, stage_v, out_s,
            sems, w_sems, stage_sems, out_sems):

    def stage_copies(chunk, slot):
        rows = pl.ds(chunk * WCH, WCH)
        return (pltpu.make_async_copy(bwk_hbm.at[rows], stage_k.at[slot], stage_sems.at[0, slot]),
                pltpu.make_async_copy(bwv_hbm.at[rows], stage_v.at[slot], stage_sems.at[1, slot]))

    cp_c = pltpu.make_async_copy(c_hbm, c_s, sems.at[2])
    cp_bwo = pltpu.make_async_copy(bwo_hbm, bwo_s, sems.at[3])

    def phase_a(xt_s, mem0_s, raw, wo_s, bwq_s, wx_s, wy_s):
        srcs = (bwq_hbm, wq_hbm, wk_hbm, wv_hbm)

        def row_chunk(k, t):
            return pltpu.make_async_copy(
                srcs[k].at[pl.ds(t * RCH, RCH)], raw.at[pl.ds((k * NCH + t) * RCH, RCH)],
                w_sems.at[k, t])

        def bwq_chunk(c, t):
            rows, lanes = pl.ds(t * RCH, RCH), pl.ds(c * T, T)
            return pltpu.make_async_copy(
                bwq_hbm.at[rows, :, lanes], raw.at[rows, :, lanes], w_sems.at[6 * c, t])

        def wo_chunk(j):
            heads = pl.ds(2 * j, 2)
            return pltpu.make_async_copy(wo_hbm.at[heads], wo_s.at[heads], w_sems.at[4, j])

        def x_piece(k, src_k=None):
            sk = k if src_k is None else src_k
            src = (xb_hbm, xa_hbm)[sk // 4].at[:, pl.ds((sk % 4) * XP, XP)]
            return pltpu.make_async_copy(
                src, xt_s.at[:, pl.ds(pl.multiple_of(k * XP, XP), XP)], w_sems.at[5, k])

        cp_m0 = pltpu.make_async_copy(mem0_hbm, mem0_s, sems.at[1])

        def start_each(copies):
            def body(t, carry):
                for cp in copies(t):
                    cp.start()
                return carry
            lax.fori_loop(0, NCH, body, 0)

        for k in range(NX0):
            x_piece(k).start()
        start_each(lambda t: [bwq_chunk(0, t)])
        start_each(lambda t: [row_chunk(1, t), row_chunk(2, t)])
        start_each(lambda t: [row_chunk(3, t)])
        for j in range(H // 2):
            wo_chunk(j).start()
            if j >= NX0:
                x_piece(j).start()
            if j > 0:
                bwq_chunk(1, j - 1).start()
        cp_m0.start()

        def u32(w):
            return pltpu.bitcast(w.astype(BF), jnp.uint32)

        def fold_pair(dst, p, lhs, rhs, scale, plan, sides):
            def put(lanes, val):
                val = val if scale is None else val * scale
                dst[pl.ds(pl.multiple_of(p * HD, 8), HD), lanes] = u32(val)

            zero = jnp.zeros((64, DH), BF)
            tails = jnp.concatenate(
                [jnp.concatenate([rhs[0][384:448, :], zero], axis=1),
                 jnp.concatenate([zero, rhs[1][384:448, :]], axis=1)], axis=0)
            sides = iter(sides)
            for step in plan:
                if step == 't':
                    put(slice(768, 896), _dot_nt(jnp.concatenate(lhs, axis=1), tails))
                elif step == 's':
                    next(sides)()
                else:
                    n, c0, c1 = step
                    put(slice(384 * n + c0 * T, 384 * n + c1 * T),
                        _dot_nt(lhs[n], rhs[n][c0 * T:c1 * T, :]))

        def transpose_x(n, width=256):
            cols = pl.ds(pl.multiple_of(n * width, width), width)
            x = xt_s[:, cols]
            rows = pl.ds(pl.multiple_of(XO + n * (width // 2), width // 2), width // 2)
            wy_s[rows, 0:512] = u32(jnp.concatenate([x, x[384:448, :]], axis=0).T)

        def x_rows(start, n, width):
            rows = pl.ds(pl.multiple_of(XO + start // 2, 8), n // 2)
            return pltpu.bitcast(wy_s[rows, 0:width], BF)

        def zero_body(n, carry):
            raw[pl.ds(4 * DM + n * 8, 8)] = jnp.zeros((8, H, DH), BF)
            return carry
        lax.fori_loop(0, RCH // 8, zero_body, 0)

        def x0_body(n, carry):
            @pl.when(lax.rem(n, XP // T) == 0)
            def _():
                x_piece(n // (XP // T), 0).wait()
            transpose_x(n, T)
            return carry
        lax.fori_loop(0, NX0 * XP // T, x0_body, 0)

        def pair_up(w):
            return [jnp.concatenate([w[2 * m], w[2 * m + 1]], axis=1) for m in range(H // 2)]

        def bwq_body(t, carry):
            @pl.when(lax.rem(t, 2) == 0)
            def _():
                bwq_chunk(0, t // 2).wait()
            rows = pl.ds(pl.multiple_of(t * (RCH // 2), RCH // 2), RCH // 2)
            for m, w in enumerate(pair_up(jnp.swapaxes(raw[rows, :, 0:T], 0, 1))):
                bwq_s[m, rows, :] = w
            return carry
        lax.fori_loop(0, 2 * NCH, bwq_body, 0)

        def chunk_rows(k, p, n, size, lanes=slice(None)):
            g = jnp.where(p > 0, k * NCH + p - 1, 4 * NCH)
            return raw[pl.ds(pl.multiple_of(g * RCH + n * size, size), size), :, lanes]

        def q_proj(m, half, start, n):
            w = bwq_s[m] if half == 0 else pltpu.bitcast(wy_s[wv_slot(m, 2, 0, HD)], BF)
            q = (_dot(x_rows(start, n, DM), w) * SCALE).astype(BF)
            rows = pl.ds(pl.multiple_of(start, 16), n)
            for odd in range(2):
                hm_s[2 * m + odd, rows, half * T:(half + 1) * T] = q[:, odd * T:(odd + 1) * T]

        def wv_slot(pair, odd, start, n):
            return (pl.ds(pl.multiple_of(XO + pair * HD + start, 8), n),
                    slice(odd * DH, (odd + 1) * DH))

        def pair_loop(unroll, waits, work):
            def body(i, carry):
                later = []
                for u in range(unroll):
                    p = i * unroll + u
                    for first, cp in waits(p, jnp.maximum(p - 1, 0)):
                        if u >= first:
                            cp.wait()
                        else:
                            assert first <= unroll
                            later.append(cp)

                @pl.when(i > 0)
                def _():
                    for cp in later:
                        cp.wait()

                for u in range(unroll):
                    p = i * unroll + u
                    work(p, jnp.maximum(p - 1, 0))
                return carry
            lax.fori_loop(0, H // 2 // unroll, body, 0)

        def q0_work(p, prev):
            def relayout(k):
                dst = pl.ds(pl.multiple_of(S + k * DM + prev * RCH, RCH), RCH)
                hm_s[:, dst, :] = jnp.swapaxes(chunk_rows(1 + k, p, 0, RCH), 0, 1)

            q_proj(p, 0, 0, R0 // 2)
            relayout(0)
            q_proj(p, 0, R0 // 2, R0 // 4)
            relayout(1)
            q_proj(p, 0, 3 * R0 // 4, R0 // 4)
        pair_loop(1, lambda p, prev: [(1, row_chunk(1, prev)), (1, row_chunk(2, prev))], q0_work)

        def ck_work(p, prev):
            def relayout(n):
                w = jnp.swapaxes(chunk_rows(3, p, n, RCH // 2), 0, 1)
                for h in range(H):
                    start = prev * (RCH // 2) + n * (RCH // 4)
                    wx_s[wv_slot(h // 2, h % 2, start, RCH // 4)] = u32(w[h])

            fold_pair(wx_s, p, [hm_s[2 * p + n, S + DM:S + 2 * DM, :] for n in range(2)],
                      [hm_s[2 * p + n, S:S + DM, :] for n in range(2)], SCALE,
                      CPLAN, [lambda: relayout(0), lambda: relayout(1)])
        pair_loop(1, lambda p, prev: [(1, row_chunk(3, prev))], ck_work)

        for s0 in range(UCH):
            for cp in stage_copies(s0, s0):
                cp.start()

        def cv_work(p, prev):
            def relayout_bwq():
                w = jnp.swapaxes(chunk_rows(0, p, 0, RCH, slice(T, 2 * T)), 0, 1)
                for m, wm in enumerate(pair_up(w)):
                    wy_s[wv_slot(m, 2, prev * (RCH // 2), RCH // 2)] = u32(wm)

            sides = [relayout_bwq, lambda: transpose_x(2 * p), lambda: transpose_x(2 * p + 1)]
            fold_pair(wy_s, p, [pltpu.bitcast(wx_s[wv_slot(p, n, 0, HD)], BF) for n in range(2)],
                      [wo_s[2 * p + n] for n in range(2)], None,
                      DPLAN, sides)
        pair_loop(2, lambda p, prev: [(0, wo_chunk(p)), (NX0, x_piece(p, 0)),
                                       (1, bwq_chunk(1, prev))], cv_work)

        cp_c.start()
        cp_bwo.start()
        cp_m0.wait()

        m0 = mem0_s[...].astype(F32)
        mem_init = jnp.concatenate([m0, m0[:, 384:448]], axis=1)

        def chain_body(b, mem):
            for u in range(UCH):
                i = b * UCH + u
                for cp in stage_copies(i, lax.rem(i, NSLOT)):
                    cp.wait()

            @pl.when(b + 1 < NPAIR // UCH)
            def _():
                for u in range(UCH):
                    nxt = (b + 1) * UCH + u
                    for cp in stage_copies(nxt, lax.rem(nxt, NSLOT)):
                        cp.start()

            for u in range(UCH):
                mem = pair_body(b, u, mem)
            return mem

        def pair_body(b, u, mem):
            i = b * UCH + u
            slot = lax.rem(i, NSLOT)

            def relayout_piece(n):
                part, src = n % 2, (stage_k, stage_v)[n // 2]
                wrows = pl.ds(pl.multiple_of(S + (n // 2) * DC + i * WCH + part * 16, 16), 16)
                hm_s[:, wrows, :] = jnp.swapaxes(src[slot, part * 16:(part + 1) * 16], 0, 1)

            def q_fill(k):
                def run():
                    n = 6 * u + k
                    same = [f for f, c in zip(FILL, HALF) if c == HALF[n]]
                    done = sum(f for f, c in zip(FILL[:n], HALF) if c == HALF[n])
                    start = (R0 if HALF[n] == 0 else 0) + lax.rem(b, 2) * sum(same) + done
                    for piece in PIECES[k]:
                        relayout_piece(piece)
                    q_proj(b // 2, HALF[n], start, FILL[n])
                return run

            lane = lax.broadcasted_iota(jnp.int32, (G, T), 1)
            r = lax.broadcasted_iota(jnp.int32, (G, H * L), 0)
            col = lax.broadcasted_iota(jnp.int32, (G, H * L), 1)
            kk = col - L * ((col * 1639) >> 16)
            keep_e = (r >= 32) | (kk >= 32) | (kk <= r)
            kpos = jnp.where(kk < 24, kk + 8, kk - 32)
            qpos = jnp.where(r < 24, r + 8, r - 32)
            q_any = ((r >= 24) & (r < 32)) | (r >= 40)
            keep_o = q_any | ((kk >= 24) & (kk < 32)) | (kpos <= qpos)

            base = pl.multiple_of(i * 64, 64)
            xs = x_rows(S + base, 64, 512)
            xs32 = xs[32:64, :].astype(F32)

            def proj(lhs, w_s, j):
                return _dot(lhs, pltpu.bitcast(w_s[j * HD:(j + 1) * HD, :], BF))

            def own(x):
                return jnp.concatenate([x[0:32, :], x[40:48, :]], axis=0)

            l1 = jnp.concatenate(
                [xs[0:32, :], jnp.concatenate([xs32[0:8, :], mem], axis=0).astype(BF)], axis=0)
            l1p = l1[:, 0:DM]
            k1 = [proj(l1p, wx_s, j) for j in range(H // 2)]
            v1 = []

            def v1_fn(j):
                v1.append(proj(l1p, wy_s, j))
                return own(v1[j])

            o1 = _rec_attention(l1, [own(k) for k in k1], v1_fn, q_fill(0), q_fill(1), keep_e, lane)
            q_fill(2)()

            l2 = jnp.concatenate([xs32[8:32, :], o1[40:48, :]], axis=0).astype(BF)
            l2p = l2[:, 0:DM]
            k2 = [jnp.concatenate([proj(l2p, wx_s, j), k1[j][32:40, :]], axis=0)
                  for j in range(H // 2)]
            o2 = _rec_attention(
                jnp.concatenate([l2, l1[32:48, :]], axis=0), k2,
                lambda j: jnp.concatenate([proj(l2p, wy_s, j), v1[j][32:40, :]], axis=0),
                q_fill(3), q_fill(4), keep_o, lane)
            q_fill(5)()

            res = jnp.concatenate([o1[0:32, :], o2[32:40, :], o2[0:24, :]], axis=0)
            out_s[pl.ds(base, 64), 0:512] = res.astype(BF)
            return o2[24:32, :]

        lax.fori_loop(0, NPAIR // UCH, chain_body, mem_init)

    pl.run_scoped(
        phase_a,
        pltpu.VMEM((DM, 2 * S), BF), pltpu.VMEM((MEM, DM), BF),
        pltpu.VMEM((4 * DM + RCH, H, DH), BF),
        pltpu.VMEM((H, DM, DH), BF), pltpu.VMEM((H // 2, DM, DH), BF),
        pltpu.VMEM((2 * XO, PAIR), jnp.uint32),
        pltpu.VMEM((XO + S, PAIR), jnp.uint32),
    )

    def phase_b(k_s, v_s, o_s, bt_s):
        cp_a = pltpu.make_async_copy(out_s.at[:, 0:384], out_hbm.at[:, 0:384], sems.at[0])
        cp_a.start()
        cp_c.wait()
        cp_bwo.wait()

        def head(h, carry):
            w = jnp.concatenate([hm_s[h, S:S + DC, :], hm_s[h, S + DC:S + 2 * DC, :]], axis=1)
            kv = _dot(c_s[...], w).astype(BF)
            k_s[...] = kv[:, 0:DH]
            v_s[...] = kv[:, DH:]
            row = lax.broadcasted_iota(jnp.int32, (T, T), 0)
            col = lax.broadcasted_iota(jnp.int32, (T, T), 1)
            tri = row >= col

            def qk(r0):
                q = hm_s[h, r0:r0 + BQ, :]
                return _b_qk(q, k_s, r0, tri)

            starts = list(reversed(range(0, S, BQ)))
            scores = qk(starts[0])
            for n, r0 in enumerate(starts):
                nxt = qk(starts[n + 1]) if n + 1 < len(starts) else None
                o_s[h, r0:r0 + BQ, :] = _b_pv(scores, v_s, h < 0).astype(BF)
                scores = nxt
            return carry
        lax.fori_loop(0, H, head, 0)

        def out_copy(t):
            rows = pl.ds(pl.multiple_of(t * BO, BO), BO)
            return pltpu.make_async_copy(
                out_s.at[rows, 384:2 * DM], out_hbm.at[rows, 384:2 * DM], out_sems.at[t])

        def project(t, after, never):
            rows = pl.ds(pl.multiple_of(t * BO, BO), BO)
            ctx = [o_s[h, rows, :] for h in range(H)]
            for n in range(2):
                ctx[8 + n] = jnp.where(never, after[:, n * DH:(n + 1) * DH], ctx[8 + n])
            wo = jnp.concatenate([bwo_s[h] for h in range(H)], axis=1)
            return _dot_nt(wo, jnp.concatenate(ctx, axis=1))

        def emit(t, bt):
            rows = pl.ds(pl.multiple_of(t * BO, BO), BO)
            b = jnp.concatenate([jnp.zeros((64, BO), F32), bt], axis=0).T.astype(BF)
            lo = lax.broadcasted_iota(jnp.int32, (BO, T), 1) < 64
            out_s[rows, 384:512] = jnp.where(lo, out_s[rows, 384:512], b[:, 0:T])
            out_s[rows, 512:896] = b[:, T:]
            return b

        bt_s[...] = jnp.zeros((DM, BO), F32)

        def oproj(i, carry):
            prev = jnp.maximum(UOP * i - 1, 0)
            b = emit(prev, bt_s[...])

            @pl.when(i > 0)
            def _():
                out_copy(prev).start()

            for u in range(UOP - 1):
                b = emit(UOP * i + u, project(UOP * i + u, b, i < 0))
                out_copy(UOP * i + u).start()
            bt_s[...] = project(UOP * i + UOP - 1, b, i < 0)
            return carry
        lax.fori_loop(0, S // BO // UOP, oproj, 0)
        emit(S // BO - 1, bt_s[...])
        out_copy(S // BO - 1).start()
        cp_a.wait()
        for t in range(S // BO):
            out_copy(t).wait()

    pl.run_scoped(
        phase_b,
        pltpu.VMEM((S, DH), BF), pltpu.VMEM((S, DH), BF),
        pltpu.VMEM((H, S, DH), BF), pltpu.VMEM((DM, BO), F32),
    )


@jax.jit
def pallas_concat_heads__memory_aug_recurrent_mem_tr__compressed_kv_cla__prompt_kernel(
    A_x: jax.Array,
    A_mem0: jax.Array,
    A_Wq: jax.Array,
    A_Wk: jax.Array,
    A_Wv: jax.Array,
    A_Wo: jax.Array,
    A_seg_len: jax.Array,
    B_x: jax.Array,
    B_c_kv: jax.Array,
    B_w_q: jax.Array,
    B_w_uk: jax.Array,
    B_w_uv: jax.Array,
    B_w_o: jax.Array,
):
    del A_seg_len
    assert A_x.shape == (1, S, DM) and A_mem0.shape == (1, MEM, DM)
    assert A_Wq.shape == (DM, H, DH) and A_Wo.shape == (H, DH, DM)
    assert B_x.shape == (1, S, DM) and B_c_kv.shape == (1, S, DC)
    assert B_w_uk.shape == (DC, H, DH) and B_w_o.shape == (H, DH, DM)

    any_spec = pl.BlockSpec(memory_space=pl.ANY)
    out = pl.pallas_call(
        _kernel,
        out_shape=jax.ShapeDtypeStruct((S, 2 * DM), BF),
        in_specs=[any_spec] * 12,
        out_specs=any_spec,
        scratch_shapes=[
            pltpu.VMEM((S, DC), BF),
            pltpu.VMEM((H, S + 2 * DC, DH), BF),
            pltpu.VMEM((H, DM, DH), BF),
            pltpu.VMEM((NSLOT, WCH, H, DH), BF),
            pltpu.VMEM((NSLOT, WCH, H, DH), BF),
            pltpu.VMEM((S, 2 * DM), BF),
            pltpu.SemaphoreType.DMA((4,)),
            pltpu.SemaphoreType.DMA((7, 8)),
            pltpu.SemaphoreType.DMA((2, NSLOT)),
            pltpu.SemaphoreType.DMA((S // BO,)),
        ],
        compiler_params=pltpu.CompilerParams(
            vmem_limit_bytes=120 * 1024 * 1024,
            disable_bounds_checks=True,
            disable_semaphore_checks=True),
    )(jnp.swapaxes(A_x, 1, 2).reshape(DM, S), A_mem0.reshape(MEM, DM), A_Wq, A_Wk, A_Wv,
      jnp.swapaxes(A_Wo, 1, 2),
      jnp.swapaxes(B_x, 1, 2).reshape(DM, S), B_c_kv.reshape(S, DC), B_w_q, B_w_uk, B_w_uv,
      jnp.swapaxes(B_w_o, 1, 2))
    return out.reshape(1, S, 2 * DM)
```
